```python
import jax
import jax.numpy as jnp

def _softmax(x, axis=-1):
    return jax.nn.softmax(x, axis=axis)
def _gelu(x):
    return jax.nn.gelu(x, approximate=True)
def _silu(x):
    return jax.nn.silu(x)
def _sigmoid(x):
    return jax.nn.sigmoid(x)
def _layernorm(x, axis=-1, eps=1e-5):
    m = jnp.mean(x, axis=axis, keepdims=True)
    v = jnp.var(x, axis=axis, keepdims=True)
    return (x - m) / jnp.sqrt(v + eps)
def _scatter_add(tgt, idx, src, axis=0):
    return tgt.at[idx].add(src)
def _segment_sum(src, seg, n):
    return jax.ops.segment_sum(src, seg, n)
class _Rng:
    def __init__(self, key):
        self._k = key
    def _next(self):
        self._k, sub = jax.random.split(self._k)
        return sub
    def normal(self, shape):
        return jax.random.normal(self._next(), shape, dtype=jnp.bfloat16)
    def randint(self, lo, hi, shape):
        return jax.random.randint(self._next(), shape, lo, hi, dtype=jnp.int32)
    def uniform(self, shape, lo=0.0, hi=1.0):
        return jax.random.uniform(self._next(), shape, jnp.bfloat16, lo, hi)
    def permutation(self, n):
        return jax.random.permutation(self._next(), n)


kernel_name = 'gated_mix__ssm_conv_h3__compressed_kv_cla__prompt'

def setup_inputs():
    _rng = _Rng(jax.random.key(int.from_bytes(__import__("os").urandom(4), "little")))
    _w = (lambda a: (lambda t: t.astype(jnp.bfloat16) if jnp.issubdtype(t.dtype, jnp.floating) else t)(jnp.asarray(a)))
    def _A_setup():
        B, S, D = 1, 2048, 1024
        ks = 4
        return {
            "q": _w((lambda *s: _rng.normal(s) * 0.05)(B, S, D)),
            "k": _w((lambda *s: _rng.normal(s) * 0.05)(B, S, D)),
            "v": _w((lambda *s: _rng.normal(s) * 0.05)(B, S, D)),
            "shift_k": _w((lambda *s: _rng.normal(s) * 0.05)(D, ks) * 0.5),
            "ssm_k": _w((lambda *s: _rng.normal(s) * 0.05)(D, S) * (1.0 / S ** 0.5)),
            "ssm_D": _w((lambda *s: _rng.normal(s) * 0.05)(D)),
        }
    _A_in = _A_setup()

    def _B_setup():
        B, H, Sq, Sk, D, M = 1, 32, 2048, 2048, 128, 1024
        Dc = 4 * D
        return {
            "x": _w((lambda *s: _rng.normal(s) * 0.05)(B, Sq, M)),
            "c_kv": _w((lambda *s: _rng.normal(s) * 0.05)(B, Sk, Dc)),
            "w_q": _w((lambda *s: _rng.normal(s) * 0.05)(M, H, D) * (M ** -0.5)),
            "w_uk": _w((lambda *s: _rng.normal(s) * 0.05)(Dc, H, D) * (Dc ** -0.5)),
            "w_uv": _w((lambda *s: _rng.normal(s) * 0.05)(Dc, H, D) * (Dc ** -0.5)),
            "w_o": _w((lambda *s: _rng.normal(s) * 0.05)(H, D, M) * ((H * D) ** -0.5)),
        }
    _B_in = _B_setup()

    return {
        "A_q": _A_in["q"],
        "A_k": _A_in["k"],
        "A_v": _A_in["v"],
        "A_shift_k": _A_in["shift_k"],
        "A_ssm_k": _A_in["ssm_k"],
        "A_ssm_D": _A_in["ssm_D"],
        "B_x": _B_in["x"],
        "B_c_kv": _B_in["c_kv"],
        "B_w_q": _B_in["w_q"],
        "B_w_uk": _B_in["w_uk"],
        "B_w_uv": _B_in["w_uv"],
        "B_w_o": _B_in["w_o"],
        "gate_w": _w((lambda *s: _rng.normal(s) * 0.05)(1024)),
    }

def reference(A_q, A_k, A_v, A_shift_k, A_ssm_k, A_ssm_D, B_x, B_c_kv, B_w_q, B_w_uk, B_w_uv, B_w_o, gate_w):
    def _A_ref(q, k, v, shift_k, ssm_k, ssm_D):
        B, S, D = q.shape
        ks = shift_k.shape[-1]
        k_pad = jnp.pad(k, ((0, 0), (ks - 1, 0), (0, 0)))
        k_shift = jnp.zeros_like(k)
        for t in range(ks):
            k_shift = k_shift + k_pad[:, t:t + S, :] * shift_k[:, ks - 1 - t][None, None, :]
        kv = k_shift * v
        L = 2 * S
        kv_pad = jnp.pad(kv, ((0, 0), (0, S), (0, 0)))
        kf_pad = jnp.pad(ssm_k, ((0, 0), (0, S)))
        kv_f = (lambda x, axes=(-2,-1): jnp.fft.rfft2(x.astype(jnp.float32), axes=axes))(kv_pad[:, None, :, :], axes=(1, 2))
        kf_f = (lambda x, axes=(-2,-1): jnp.fft.rfft2(x.astype(jnp.float32), axes=axes))(kf_pad[:, None, :], axes=(1, 2))
        kf_f = (lambda x, *d: x.transpose(*d))(kf_f, 1, 2, 0)
        y_f = kv_f * kf_f[None, :, :, :]
        y = (lambda x, s, axes=(-2,-1): jnp.fft.irfft2(x, s=s, axes=axes).astype(jnp.bfloat16))(y_f, (1, L), axes=(1, 2))[:, 0, :S, :]
        y = y + kv * ssm_D[None, None, :]
        return q * y

    def _B_ref(x, c_kv, w_q, w_uk, w_uv, w_o):
        B, Sq, M = x.shape[0], x.shape[1], x.shape[2]
        Sk = c_kv.shape[1]
        H, D = w_q.shape[1], w_q.shape[2]
        q = jnp.einsum("bqm,mhd->bhqd", x, w_q)
        k = jnp.einsum("bkc,chd->bhkd", c_kv, w_uk)
        v = jnp.einsum("bkc,chd->bhkd", c_kv, w_uv)
        scores = jnp.einsum("bhqd,bhkd->bhqk", q, k) * (D ** -0.5)
        off = Sk - Sq
        qi = jnp.arange(Sq)[:, None]
        kj = jnp.arange(Sk)[None, :]
        cmask = kj <= (qi + off)
        scores = jnp.where(cmask[None, None], scores, -1e9)
        p = _softmax(scores, axis=-1)
        ctx = jnp.einsum("bhqk,bhkd->bhqd", p, v)
        return jnp.einsum("bhqd,hdm->bqm", ctx, w_o)

    x = A_q
    g = _sigmoid((x * gate_w).sum(-1, keepdims=True))
    a = _A_ref(x, A_k, A_v, A_shift_k, A_ssm_k, A_ssm_D)
    b = _B_ref(x, B_c_kv, B_w_q, B_w_uk, B_w_uv, B_w_o)
    return g * a + (1 - g) * b
```

```python
import numpy as np
import jax
import jax.numpy as jnp
from jax import lax
import jax.experimental.pallas as pl
import jax.experimental.pallas.tpu as pltpu

_BF = jnp.bfloat16
_F32 = jnp.float32
_NT = (((1,), (1,)), ((), ()))
_T = 128
_BQ = 256
_NEG = -1e30
_LOG2E = 1.4426950408889634


def _dft_tables(c):
    f = np.concatenate([np.arange(0, c, 2), np.arange(1, c, 2)]).astype(np.float64)
    b = np.arange(c, dtype=np.float64)
    ang = np.pi * (f[:, None] + 0.5) * b[None, :] / c
    fwd = np.concatenate([np.cos(ang), -np.sin(ang)], axis=0)
    inv = np.concatenate([np.cos(ang).T, -np.sin(ang).T], axis=1) / c
    return fwd.astype(np.float32), inv.astype(np.float32)


_FWD_NP, _INV_NP = _dft_tables(_T)


def _dot(a, b):
    return jnp.dot(a, b, preferred_element_type=_F32)


def _dot_nt(a, b):
    return lax.dot_general(a, b, _NT, preferred_element_type=_F32)


def _unpack_head(w32, odd):
    bits = (w32 & jnp.uint32(0xFFFF0000)) if odd else (w32 << 16)
    return pltpu.bitcast(bits, _F32).astype(_BF)


def _kernel(x_hbm, k_hbm, v_hbm, shift_ref, ssmk_hbm, ssmd_ref, c_hbm, wq_hbm, wuk_hbm,
            wuv_hbm, wo_hbm, gate_ref, fwd_ref, inv_ref, out_hbm,
            x_v, c_v, wq_v, wuk_v, wuv_v, wo_v, ak_v, av_v, sk_v, ctx_v,
            wq_b, wkv_b, q0, k0, v0, q1, k1, v1, g_v, kf32, kv_v, uf_v, kf_v, yf_v, o_v,
            sem_in, sem_w, sem_o, *, S, M, H, D):
    NP = H // 2
    NQ = S // _BQ
    qscale = float(D ** -0.5 * _LOG2E)

    def w_copies(p):
        return [pltpu.make_async_copy(src.bitcast(jnp.uint32).at[:, p, :], dst.at[p],
                                      sem_w.at[3 * p + n])
                for n, (src, dst) in enumerate(((wuk_hbm, wuk_v), (wuv_hbm, wuv_v),
                                                (wq_hbm, wq_v)))]

    in_copies = [pltpu.make_async_copy(src, dst, sem_in.at[n])
                 for n, (src, dst) in enumerate(((c_hbm, c_v), (x_hbm, x_v), (wo_hbm, wo_v),
                                                 (k_hbm, ak_v), (v_hbm, av_v),
                                                 (ssmk_hbm, sk_v)))]
    in_copies[0].start()
    for cp in w_copies(0):
        cp.start()
    in_copies[1].start()
    for p in range(1, NP):
        for cp in w_copies(p):
            cp.start()
    for cp in in_copies[2:]:
        cp.start()

    tri = (lax.broadcasted_iota(jnp.int32, (_T, _T), 1)
           <= lax.broadcasted_iota(jnp.int32, (_T, _T), 0))

    def prep_weights(p, odd):
        wq_b[...] = _unpack_head(wq_v[p], odd)
        wkv_b[:, 0:D] = _unpack_head(wuk_v[p], odd)
        wkv_b[:, D:2 * D] = _unpack_head(wuv_v[p], odd)

    def proj(i, dst):
        qd, kd, vd = dst
        rows = pl.ds(i * _BQ, _BQ)
        qd[rows, :] = (_dot(x_v[rows, :], wq_b[...]) * qscale).astype(_BF)
        kv = _dot(c_v[rows, :], wkv_b[...])
        kd[rows, :] = kv[:, 0:D].astype(_BF)
        vd[rows, :] = kv[:, D:2 * D].astype(_BF)

    def qk(i, src):
        qs, ks, _ = src
        r0 = i * _BQ
        nfull = 2 * i
        q = qs[pl.ds(r0, _BQ), :]
        tiles = [_dot_nt(q, ks[pl.ds(j * _T, _T), :]) for j in range(nfull + 1)]
        d = tiles[nfull]
        d0 = jnp.where(tri, d[0:_T], _NEG)
        d1 = d[_T:]
        tiles[nfull] = jnp.concatenate([d0, d1], axis=0)
        last = jnp.where(tri, _dot_nt(q[_T:], ks[pl.ds((nfull + 1) * _T, _T), :]), _NEG)
        m = tiles[0]
        for t in tiles[1:]:
            m = jnp.maximum(m, t)
        m = jnp.concatenate([m[0:_T], jnp.maximum(m[_T:], last)], axis=0)
        m = jnp.broadcast_to(jnp.max(m, axis=1, keepdims=True), (_BQ, _T))
        return tiles, last, m

    def pv(i, src, h, state):
        _, _, vs = src
        tiles, last, m = state
        l = None
        acc = None
        for j, t in enumerate(tiles):
            p = jnp.exp2(t - m)
            l = p if l is None else l + p
            o = _dot(p.astype(_BF), vs[pl.ds(j * _T, _T), :])
            acc = o if acc is None else acc + o
        p = jnp.exp2(last - m[_T:])
        o = _dot(p.astype(_BF), vs[pl.ds(len(tiles) * _T, _T), :])
        l = jnp.concatenate([l[0:_T], l[_T:] + p], axis=0)
        acc = jnp.concatenate([acc[0:_T], acc[_T:] + o], axis=0)
        l = jnp.broadcast_to(jnp.sum(l, axis=1, keepdims=True), (_BQ, _T))
        r = pl.reciprocal(l, approx=True)
        r = r * (2.0 - l * r)
        ctx_v[h, pl.ds(i * _BQ, _BQ), :] = (acc * r).astype(_BF)

    def head(h, src, dst, wp, odd):
        if dst is not None:
            prep_weights(wp, odd)
        state = qk(0, src)
        for i in range(NQ):
            nxt = qk(i + 1, src) if i + 1 < NQ else None
            if dst is not None and i + 1 < NQ:
                proj(i, dst)
            pv(i, src, h, state)
            if dst is not None and i + 1 == NQ:
                proj(i, dst)
            state = nxt

    buf0, buf1 = (q0, k0, v0), (q1, k1, v1)

    in_copies[0].wait()
    for cp in w_copies(0):
        cp.wait()
    in_copies[1].wait()
    prep_weights(0, False)
    gw = gate_ref[...].astype(_F32)
    for i in range(NQ):
        proj(i, buf0)
        rows = pl.ds(i * _BQ, _BQ)
        z = jnp.sum(x_v[rows, :].astype(_F32) * gw, axis=1, keepdims=True)
        g_v[rows, :] = jnp.broadcast_to(1.0 / (1.0 + jnp.exp(-z)), (_BQ, _T))

    def pair_body(p, carry):
        head(2 * p, buf0, buf1, p, True)
        for cp in w_copies(p + 1):
            cp.wait()
        head(2 * p + 1, buf1, buf0, p + 1, False)
        return carry

    lax.fori_loop(0, NP - 1, pair_body, 0)
    head(H - 2, buf0, buf1, NP - 1, True)
    head(H - 1, buf1, None, None, None)

    for cp in in_copies[2:]:
        cp.wait()
    NC = S // _T
    NB = M // _T
    HF = _T // 2

    def out_copy(cb, slot):
        cols = pl.ds(pl.multiple_of(cb * _T, _T), _T)
        return pltpu.make_async_copy(o_v.at[slot], out_hbm.at[:, cols], sem_o.at[slot])

    kf32[0:8, :] = jnp.zeros((8, _T), _F32)

    def col_body(cb, carry):
        cols = pl.ds(pl.multiple_of(cb * _T, _T), _T)
        slot = cb % 2

        @pl.when(cb >= 2)
        def _():
            out_copy(cb - 2, slot).wait()

        kf32[pl.ds(8, S), :] = ak_v[:, cols].astype(_F32)
        sh = shift_ref[:, cols].astype(_F32)
        fwd = fwd_ref[...]
        for j in range(NC):
            acc = kf32[pl.ds(8 + j * _T, _T), :] * sh[0:1, :]
            for s in range(1, sh.shape[0]):
                acc = acc + kf32[pl.ds(8 + j * _T - s, _T), :] * sh[s:s + 1, :]
            kv = (acc * av_v[pl.ds(j * _T, _T), cols].astype(_F32)).astype(_BF)
            kv_v[pl.ds(j * _T, _T), :] = kv
            uf_v[j] = _dot(fwd, kv)
            kf_v[j] = _dot_nt(fwd, sk_v[cols, pl.ds(j * _T, _T)])

        for fg in range(_T // 8):
            re = pl.ds(fg * 8, 8)
            im = pl.ds(_T + fg * 8, 8)
            even = fg * 8 < HF
            prev = None
            for i in range(NC):
                yr = yi = None
                for j in range(i + 1):
                    kr, ki = kf_v[i - j, re, :], kf_v[i - j, im, :]
                    ur, ui = uf_v[j, re, :], uf_v[j, im, :]
                    tr = kr * ur - ki * ui
                    ti = kr * ui + ki * ur
                    yr = tr if yr is None else yr + tr
                    yi = ti if yi is None else yi + ti
                if prev is None:
                    zr, zi = yr, yi
                elif even:
                    zr, zi = yr - prev[1], yi + prev[0]
                else:
                    zr, zi = yr + prev[1], yi - prev[0]
                prev = (yr, yi)
                yf_v[i, re, :] = zr
                yf_v[i, im, :] = zi

        dvec = ssmd_ref[:, cols].astype(_F32)
        inv = inv_ref[...]
        for i in range(NQ):
            rows = pl.ds(i * _BQ, _BQ)
            b = None
            for h in range(H):
                t = _dot(ctx_v[h, rows, :], wo_v[h, :, cols])
                b = t if b is None else b + t
            y = jnp.concatenate([_dot(inv, yf_v[2 * i].astype(_BF)),
                                 _dot(inv, yf_v[2 * i + 1].astype(_BF))], axis=0)
            y = y + kv_v[rows, :].astype(_F32) * dvec
            a = x_v[rows, cols].astype(_F32) * y
            g = g_v[rows, :]
            o_v[slot, rows, :] = (g * a + (1.0 - g) * b).astype(_BF)
        out_copy(cb, slot).start()
        return carry

    lax.fori_loop(0, NB, col_body, 0)
    out_copy(NB - 2, 0).wait()
    out_copy(NB - 1, 1).wait()


@jax.jit
def pallas_gated_mix__ssm_conv_h3__compressed_kv_cla__prompt_kernel(
    A_q: jax.Array,
    A_k: jax.Array,
    A_v: jax.Array,
    A_shift_k: jax.Array,
    A_ssm_k: jax.Array,
    A_ssm_D: jax.Array,
    B_x: jax.Array,
    B_c_kv: jax.Array,
    B_w_q: jax.Array,
    B_w_uk: jax.Array,
    B_w_uv: jax.Array,
    B_w_o: jax.Array,
    gate_w: jax.Array,
):
    del B_x
    B, S, M = A_q.shape
    _, H, D = B_w_q.shape
    DC = B_c_kv.shape[-1]
    assert B == 1 and D == _T and H % 2 == 0 and S % _BQ == 0 and B_c_kv.shape[1] == S
    NP, NC = H // 2, S // _T

    def body(*refs):
        _kernel(*refs, S=S, M=M, H=H, D=D)

    hbm = pl.BlockSpec(memory_space=pl.ANY)
    vmem = pl.BlockSpec(memory_space=pltpu.VMEM)
    scratch = [
        pltpu.VMEM((S, M), _BF),
        pltpu.VMEM((S, DC), _BF),
        pltpu.VMEM((NP, M, D), jnp.uint32),
        pltpu.VMEM((NP, DC, D), jnp.uint32),
        pltpu.VMEM((NP, DC, D), jnp.uint32),
        pltpu.VMEM((H, D, M), _BF),
        pltpu.VMEM((S, M), _BF),
        pltpu.VMEM((S, M), _BF),
        pltpu.VMEM((M, S), _BF),
        pltpu.VMEM((H, S, D), _BF),
        pltpu.VMEM((M, D), _BF),
        pltpu.VMEM((DC, 2 * D), _BF),
    ] + [pltpu.VMEM((S, D), _BF)] * 6 + [
        pltpu.VMEM((S, _T), _F32),
        pltpu.VMEM((S + 8, _T), _F32),
        pltpu.VMEM((S, _T), _BF),
        pltpu.VMEM((NC, 2 * _T, _T), _F32),
        pltpu.VMEM((NC, 2 * _T, _T), _F32),
        pltpu.VMEM((NC, 2 * _T, _T), _F32),
        pltpu.VMEM((2, S, _T), _BF),
        pltpu.SemaphoreType.DMA((6,)),
        pltpu.SemaphoreType.DMA((3 * NP,)),
        pltpu.SemaphoreType.DMA((2,)),
    ]
    out = pl.pallas_call(
        body,
        out_shape=jax.ShapeDtypeStruct((S, M), _BF),
        in_specs=[hbm, hbm, hbm, vmem, hbm, vmem, hbm, hbm, hbm, hbm, hbm, vmem, vmem, vmem],
        out_specs=hbm,
        scratch_shapes=scratch,
        compiler_params=pltpu.CompilerParams(vmem_limit_bytes=112 * 2 ** 20),
    )(
        A_q.reshape(S, M), A_k.reshape(S, M), A_v.reshape(S, M), A_shift_k.T, A_ssm_k,
        A_ssm_D.reshape(1, M), B_c_kv.reshape(S, DC), B_w_q, B_w_uk, B_w_uv, B_w_o,
        gate_w.reshape(1, M), jnp.asarray(_FWD_NP, _BF), jnp.asarray(_INV_NP, _BF),
    )
    return out.reshape(B, S, M)
```

```python
import numpy as np
import jax
import jax.numpy as jnp
from jax import lax
import jax.experimental.pallas as pl
import jax.experimental.pallas.tpu as pltpu

_BF = jnp.bfloat16
_F32 = jnp.float32
_NT = (((1,), (1,)), ((), ()))
_T = 128
_BQ = 256
_NEG = -1e30
_LOG2E = 1.4426950408889634


def _dft_tables(c):
    f = np.concatenate([np.arange(0, c, 2), np.arange(1, c, 2)]).astype(np.float64)
    b = np.arange(c, dtype=np.float64)
    ang = np.pi * (f[:, None] + 0.5) * b[None, :] / c
    fwd = np.concatenate([np.cos(ang), -np.sin(ang)], axis=0)
    inv = np.concatenate([np.cos(ang).T, -np.sin(ang).T], axis=1) / c
    return fwd.astype(np.float32), inv.astype(np.float32)


_FWD_NP, _INV_NP = _dft_tables(_T)


def _dot(a, b):
    return jnp.dot(a, b, preferred_element_type=_F32)


def _dot_nt(a, b):
    return lax.dot_general(a, b, _NT, preferred_element_type=_F32)


def _unpack_head(w32, odd):
    bits = (w32 & jnp.uint32(0xFFFF0000)) if odd else (w32 << 16)
    return pltpu.bitcast(bits, _F32).astype(_BF)


def _merge(a, b):
    out, ia, ib = [], 0, 0
    while ia < len(a) or ib < len(b):
        if ib >= len(b) or (ia < len(a) and ia * len(b) <= ib * len(a)):
            out.append(a[ia])
            ia += 1
        else:
            out.append(b[ib])
            ib += 1
    return out


def _kernel(x_hbm, k_hbm, v_hbm, shift_ref, ssmk_hbm, ssmd_ref, c_hbm, wq_hbm, wuk_hbm,
            wuv_hbm, wo_hbm, gate_ref, fwd_ref, inv_ref, out_hbm,
            x_v, c_v, wq_v, wuk_v, wuv_v, wo_v, ak_v, av_v, sk_v, ctx_v,
            wq_b, wkv_b, q0, k0, v0, q1, k1, v1, g_v, kf32, o_v,
            sem_in, sem_w, sem_o, *, S, M, H, D):
    NP = H // 2
    NQ = S // _BQ
    TPB = _BQ // _T
    qscale = float(D ** -0.5 * _LOG2E)

    def w_copies(p):
        return [pltpu.make_async_copy(src.bitcast(jnp.uint32).at[:, p, :], dst.at[p],
                                      sem_w.at[3 * p + n])
                for n, (src, dst) in enumerate(((wuk_hbm, wuk_v), (wuv_hbm, wuv_v),
                                                (wq_hbm, wq_v)))]

    cp_c, cp_x, cp_wo, cp_k, cp_v, cp_s = [
        pltpu.make_async_copy(src, dst, sem_in.at[n])
        for n, (src, dst) in enumerate(((c_hbm, c_v), (x_hbm, x_v), (wo_hbm, wo_v),
                                        (k_hbm, ak_v), (v_hbm, av_v), (ssmk_hbm, sk_v)))]

    tri = (lax.broadcasted_iota(jnp.int32, (_T, _T), 1)
           <= lax.broadcasted_iota(jnp.int32, (_T, _T), 0))

    def prep_kv(p, odd):
        wkv_b[:, 0:D] = _unpack_head(wuk_v[p], odd)
        wkv_b[:, D:2 * D] = _unpack_head(wuv_v[p], odd)

    def prep_q(p, odd):
        wq_b[...] = _unpack_head(wq_v[p], odd)

    def proj_q(r, dst):
        rows = pl.ds(r * _BQ, _BQ)
        dst[0][rows, :] = (_dot(x_v[rows, :], wq_b[...]) * qscale).astype(_BF)

    def proj_kv(r, dst):
        rows = pl.ds(r * _BQ, _BQ)
        kv = _dot(c_v[rows, :], wkv_b[...])
        dst[1][rows, :] = kv[:, 0:D].astype(_BF)
        dst[2][rows, :] = kv[:, D:2 * D].astype(_BF)

    def head(h, src, dst):
        qs, ks, vs = src
        st = {}

        def first_row(i, j):
            return max(0, j - TPB * i) * _T

        def accum(old, new, lo, op):
            if old is None:
                return new
            if lo == 0:
                return op(old, new)
            return jnp.concatenate([old[:lo], op(old[lo:], new)], axis=0)

        def qk(i, js):
            s = st.setdefault(i, dict(t={}, m=None, l=None, acc=None))
            q = qs[pl.ds(i * _BQ, _BQ), :]
            for j in js:
                lo = first_row(i, j)
                t = _dot_nt(q[lo:], ks[pl.ds(j * _T, _T), :])
                if j >= TPB * i:
                    top = jnp.where(tri, t[0:_T], _NEG)
                    t = top if t.shape[0] == _T else jnp.concatenate([top, t[_T:]], axis=0)
                s["t"][j] = t
                s["m"] = accum(s["m"], t, lo, jnp.maximum)
            if js[-1] == TPB * (i + 1) - 1:
                s["m"] = jnp.broadcast_to(jnp.max(s["m"], axis=1, keepdims=True), (_BQ, _T))

        def pv(i, js):
            s = st[i]
            for j in js:
                lo = first_row(i, j)
                p = jnp.exp2(s["t"][j] - s["m"][lo:])
                s["l"] = accum(s["l"], p, lo, jnp.add)
                s["acc"] = accum(s["acc"], _dot(p.astype(_BF), vs[pl.ds(j * _T, _T), :]),
                                 lo, jnp.add)
            if js[-1] == TPB * (i + 1) - 1:
                l = jnp.broadcast_to(jnp.sum(s["l"], axis=1, keepdims=True), (_BQ, _T))
                r = pl.reciprocal(l, approx=True)
                r = r * (2.0 - l * r)
                ctx_v[h, pl.ds(i * _BQ, _BQ), :] = (s["acc"] * r).astype(_BF)

        def groups(fn, i):
            n = TPB * (i + 1)
            return [(fn, i, list(range(a, min(a + 4, n)))) for a in range(0, n, 4)]

        att = groups(qk, NQ - 1)
        for i in range(NQ - 1, -1, -1):
            att += _merge(groups(qk, i - 1) if i > 0 else [], groups(pv, i))
        side = [] if dst is None else [(f, r) for r in range(NQ) for f in (proj_q, proj_kv)]
        cost = [sum(_BQ - first_row(i, j) for j in js) for _, i, js in att]
        done, k = 0, 0
        for (fn, i, js), c in zip(att, cost):
            fn(i, js)
            done += c
            while k < len(side) - 1 and (k + 0.5) * sum(cost) <= (len(side) - 1) * done:
                side[k][0](side[k][1], dst)
                k += 1
        for f, r in side[k:]:
            f(r, dst)

    buf0, buf1 = (q0, k0, v0), (q1, k1, v1)

    w0 = w_copies(0)
    cp_c.start()
    w0[0].start()
    w0[1].start()
    cp_c.wait()
    w0[2].start()
    cp_x.start()
    w0[0].wait()
    w0[1].wait()
    prep_kv(0, False)
    for r in range(NQ):
        proj_kv(r, buf0)
    w0[2].wait()
    cp_x.wait()
    for cp in w_copies(1):
        cp.start()
    for cp in (cp_wo, cp_k, cp_v, cp_s):
        cp.start()
    prep_q(0, False)
    gw = gate_ref[...].astype(_F32)
    for r in range(NQ):
        proj_q(r, buf0)
        rows = pl.ds(r * _BQ, _BQ)
        z = jnp.sum(x_v[rows, :].astype(_F32) * gw, axis=1, keepdims=True)
        g_v[rows, :] = jnp.broadcast_to(1.0 / (1.0 + jnp.exp(-z)), (_BQ, _T))

    def pair_body(p, carry):
        for cp in w_copies(p + 1):
            cp.wait()

        @pl.when(p + 2 < NP)
        def _():
            for cp in w_copies(p + 2):
                cp.start()

        prep_q(p, True)
        prep_kv(p, True)
        head(2 * p, buf0, buf1)
        prep_q(p + 1, False)
        prep_kv(p + 1, False)
        head(2 * p + 1, buf1, buf0)
        return carry

    lax.fori_loop(0, NP - 1, pair_body, 0)
    prep_q(NP - 1, True)
    prep_kv(NP - 1, True)
    head(H - 2, buf0, buf1)
    head(H - 1, buf1, None)

    for cp in (cp_wo, cp_k, cp_v, cp_s):
        cp.wait()
    NC = S // _T
    NB = M // _T
    HF = _T // 2

    def out_copy(cb, slot):
        cols = pl.ds(pl.multiple_of(cb * _T, _T), _T)
        return pltpu.make_async_copy(o_v.at[slot], out_hbm.at[:, cols], sem_o.at[slot])

    kf32[0:8, :] = jnp.zeros((8, _T), _F32)

    def col_body(cb, carry):
        cols = pl.ds(pl.multiple_of(cb * _T, _T), _T)
        slot = cb % 2

        @pl.when(cb >= 2)
        def _():
            out_copy(cb - 2, slot).wait()

        sh = shift_ref[:, cols].astype(_F32)
        dvec = ssmd_ref[:, cols].astype(_F32)
        bacc, kvs, uf, kf, yf, yt = {}, {}, {}, {}, {}, {}

        def out_proj(i, g):
            rows = pl.ds(i * _BQ, _BQ)
            for h in range(4 * g, 4 * g + 4):
                t = _dot(ctx_v[h, rows, :], wo_v[h, :, cols])
                bacc[i] = t if h == 0 else bacc[i] + t

        def dft_u(j):
            kf32[pl.ds(8 + j * _T, _T), :] = ak_v[pl.ds(j * _T, _T), cols].astype(_F32)
            acc = kf32[pl.ds(8 + j * _T, _T), :] * sh[0:1, :]
            for s in range(1, sh.shape[0]):
                acc = acc + kf32[pl.ds(8 + j * _T - s, _T), :] * sh[s:s + 1, :]
            kv = (acc * av_v[pl.ds(j * _T, _T), cols].astype(_F32)).astype(_BF)
            kvs[j] = kv
            uf[j] = _dot(fwd_ref[...], kv)

        def dft_k(j):
            s = _dot_nt(fwd_ref[...], sk_v[cols, pl.ds(j * _T, _T)])
            if j == 0:
                kf[j] = s
            else:
                p = kf["prev"]
                kf[j] = jnp.concatenate(
                    [s[0:HF] - p[_T:_T + HF], s[HF:_T] + p[_T + HF:],
                     s[_T:_T + HF] + p[0:HF], s[_T + HF:] - p[HF:_T]], axis=0)
            kf["prev"] = s

        def mac(fg):
            re, im = slice(fg * 8, fg * 8 + 8), slice(_T + fg * 8, _T + fg * 8 + 8)
            for i in range(NC):
                yr = yi = None
                for j in range(i + 1):
                    kr, ki, ur, ui = kf[i - j][re], kf[i - j][im], uf[j][re], uf[j][im]
                    tr, ti = kr * ur - ki * ui, kr * ui + ki * ur
                    yr, yi = (tr, ti) if j == 0 else (yr + tr, yi + ti)
                yf[i, fg] = (yr, yi)

        def idft(c):
            spec = jnp.concatenate([yf[c, fg][part] for part in range(2)
                                    for fg in range(_T // 8)], axis=0)
            yt[c] = _dot(inv_ref[...], spec.astype(_BF))

        def combine(c):
            rows = pl.ds(c * _T, _T)
            off = (c % TPB) * _T
            y = yt[c] + kvs[c].astype(_F32) * dvec
            a = x_v[rows, cols].astype(_F32) * y
            g = g_v[rows, :]
            o_v[slot, rows, :] = (g * a + (1.0 - g) * bacc[c // TPB][off:off + _T]).astype(_BF)

        main = [(i, g) for i in range(NQ) for g in range(H // 4)]
        f0, f1, f2, f3 = 0.05, 0.25, 0.75, 0.85
        stage1 = [(dft_k, j) for j in range(NC)] + [(dft_u, j) for j in range(NC)]
        side = [(f0 + (f1 - f0) * n / len(stage1), f, a) for n, (f, a) in enumerate(stage1)]
        side += [(f1 + (f2 - f1) * fg * 8 / _T, mac, fg) for fg in range(_T // 8)]
        side += [(f2 + (f3 - f2) * c / NC, idft, c) for c in range(NC)]
        side += [(max(f2 + (f3 - f2) * (c + 0.5) / NC, (c // TPB + 1) / NQ), combine, c)
                 for c in range(NC)]
        side.sort(key=lambda t: t[0])
        k = 0
        for n, (i, g) in enumerate(main):
            while k < len(side) and side[k][0] <= n / len(main) + 1e-9:
                side[k][1](side[k][2])
                k += 1
            out_proj(i, g)
        for _, f, a in side[k:]:
            f(a)
        out_copy(cb, slot).start()
        return carry

    lax.fori_loop(0, NB, col_body, 0)
    out_copy(NB - 2, 0).wait()
    out_copy(NB - 1, 1).wait()


@jax.jit
def pallas_gated_mix__ssm_conv_h3__compressed_kv_cla__prompt_kernel(
    A_q: jax.Array,
    A_k: jax.Array,
    A_v: jax.Array,
    A_shift_k: jax.Array,
    A_ssm_k: jax.Array,
    A_ssm_D: jax.Array,
    B_x: jax.Array,
    B_c_kv: jax.Array,
    B_w_q: jax.Array,
    B_w_uk: jax.Array,
    B_w_uv: jax.Array,
    B_w_o: jax.Array,
    gate_w: jax.Array,
):
    del B_x
    B, S, M = A_q.shape
    _, H, D = B_w_q.shape
    DC = B_c_kv.shape[-1]
    assert B == 1 and D == _T and H % 2 == 0 and S % _BQ == 0 and B_c_kv.shape[1] == S
    NP = H // 2

    def body(*refs):
        _kernel(*refs, S=S, M=M, H=H, D=D)

    hbm = pl.BlockSpec(memory_space=pl.ANY)
    vmem = pl.BlockSpec(memory_space=pltpu.VMEM)
    scratch = [
        pltpu.VMEM((S, M), _BF),
        pltpu.VMEM((S, DC), _BF),
        pltpu.VMEM((NP, M, D), jnp.uint32),
        pltpu.VMEM((NP, DC, D), jnp.uint32),
        pltpu.VMEM((NP, DC, D), jnp.uint32),
        pltpu.VMEM((H, D, M), _BF),
        pltpu.VMEM((S, M), _BF),
        pltpu.VMEM((S, M), _BF),
        pltpu.VMEM((M, S), _BF),
        pltpu.VMEM((H, S, D), _BF),
        pltpu.VMEM((M, D), _BF),
        pltpu.VMEM((DC, 2 * D), _BF),
    ] + [pltpu.VMEM((S, D), _BF)] * 6 + [
        pltpu.VMEM((S, _T), _F32),
        pltpu.VMEM((S + 8, _T), _F32),
        pltpu.VMEM((2, S, _T), _BF),
        pltpu.SemaphoreType.DMA((6,)),
        pltpu.SemaphoreType.DMA((3 * NP,)),
        pltpu.SemaphoreType.DMA((2,)),
    ]
    out = pl.pallas_call(
        body,
        out_shape=jax.ShapeDtypeStruct((S, M), _BF),
        in_specs=[hbm, hbm, hbm, vmem, hbm, vmem, hbm, hbm, hbm, hbm, hbm, vmem, vmem, vmem],
        out_specs=hbm,
        scratch_shapes=scratch,
        compiler_params=pltpu.CompilerParams(vmem_limit_bytes=112 * 2 ** 20),
    )(
        A_q.reshape(S, M), A_k.reshape(S, M), A_v.reshape(S, M), A_shift_k.T, A_ssm_k,
        A_ssm_D.reshape(1, M), B_c_kv.reshape(S, DC), B_w_q, B_w_uk, B_w_uv, B_w_o,
        gate_w.reshape(1, M), jnp.asarray(_FWD_NP, _BF), jnp.asarray(_INV_NP, _BF),
    )
    return out.reshape(B, S, M)
```

```python
import numpy as np
import jax
import jax.numpy as jnp
from jax import lax
import jax.experimental.pallas as pl
import jax.experimental.pallas.tpu as pltpu

_BF = jnp.bfloat16
_F32 = jnp.float32
_NT = (((1,), (1,)), ((), ()))
_T = 128
_BQ = 256
_NCHUNK = 4
_NEG = -1e30
_LOG2E = 1.4426950408889634


def _dft_tables(c):
    f = np.concatenate([np.arange(0, c, 2), np.arange(1, c, 2)]).astype(np.float64)
    b = np.arange(c, dtype=np.float64)
    ang = np.pi * (f[:, None] + 0.5) * b[None, :] / c
    fwd = np.concatenate([np.cos(ang), -np.sin(ang)], axis=0)
    inv = np.concatenate([np.cos(ang).T, -np.sin(ang).T], axis=1) / c
    return fwd.astype(np.float32), inv.astype(np.float32)


_FWD_NP, _INV_NP = _dft_tables(_T)


def _dot(a, b):
    return jnp.dot(a, b, preferred_element_type=_F32)


def _dot_nt(a, b):
    return lax.dot_general(a, b, _NT, preferred_element_type=_F32)


def _unpack_head(w32, odd):
    bits = (w32 & jnp.uint32(0xFFFF0000)) if odd else (w32 << 16)
    return pltpu.bitcast(bits, _F32).astype(_BF)


def _merge(a, b):
    out, ia, ib = [], 0, 0
    while ia < len(a) or ib < len(b):
        if ib >= len(b) or (ia < len(a) and ia * len(b) <= ib * len(a)):
            out.append(a[ia])
            ia += 1
        else:
            out.append(b[ib])
            ib += 1
    return out


def _kernel(x_hbm, k_hbm, v_hbm, shift_hbm, ssmk_hbm, ssmd_hbm, c_hbm, wq_hbm, wuk_hbm,
            wuv_hbm, wo_hbm, gate_hbm, fwd_hbm, inv_hbm, out_hbm,
            x_v, c_v, wq_v, wuk_v, wuv_v, wo_v, ak_v, av_v, sk_v, ctx_v,
            wq_b, wkv_b, q0, k0, v0, q1, k1, v1, g_v, kf32, spec_v, o_v,
            shift_v, ssmd_v, gate_v, fwd_v, inv_v, ssmd_f, zero_s,
            sem_in, sem_w, sem_o, *, S, M, H, D):
    NP = H // 2
    NQ = S // _BQ
    TPB = _BQ // _T
    qscale = float(D ** -0.5 * _LOG2E)

    def w_copies(p):
        return [pltpu.make_async_copy(src.bitcast(jnp.uint32).at[:, p, :], dst.at[p],
                                      sem_w.at[3 * p + n])
                for n, (src, dst) in enumerate(((wuk_hbm, wuk_v), (wuv_hbm, wuv_v),
                                                (wq_hbm, wq_v)))]

    cp_gate, *cp_late = [
        pltpu.make_async_copy(src, dst, sem_in.at[n])
        for n, (src, dst) in enumerate((
            (gate_hbm, gate_v), (wo_hbm, wo_v), (k_hbm, ak_v), (v_hbm, av_v), (ssmk_hbm, sk_v),
            (shift_hbm, shift_v), (ssmd_hbm, ssmd_v), (fwd_hbm, fwd_v), (inv_hbm, inv_v)))]

    def row_copies(src, dst, sem0, nchunk):
        rows = S // nchunk
        return [pltpu.make_async_copy(src.at[pl.ds(n * rows, rows)], dst.at[pl.ds(n * rows, rows)],
                                      sem_in.at[sem0 + n]) for n in range(nchunk)]

    cp_c = row_copies(c_hbm, c_v, 9, _NCHUNK)
    cp_x = row_copies(x_hbm, x_v, 9 + _NCHUNK, _NCHUNK)

    tri = (lax.broadcasted_iota(jnp.int32, (_T, _T), 1)
           <= lax.broadcasted_iota(jnp.int32, (_T, _T), 0))

    def prep_kv(p, odd):
        wkv_b[:, 0:D] = _unpack_head(wuk_v[p], odd)
        wkv_b[:, D:2 * D] = _unpack_head(wuv_v[p], odd)

    def prep_q(p, odd):
        wq_b[...] = _unpack_head(wq_v[p], odd)

    def proj_q(r, dst):
        rows = pl.ds(r * _BQ, _BQ)
        dst[0][rows, :] = (_dot(x_v[rows, :], wq_b[...]) * qscale).astype(_BF)

    def proj_kv(r, dst):
        rows = pl.ds(r * _BQ, _BQ)
        kv = _dot(c_v[rows, :], wkv_b[...])
        dst[1][rows, :] = kv[:, 0:D].astype(_BF)
        dst[2][rows, :] = kv[:, D:2 * D].astype(_BF)

    def head(h, src, dst):
        qs, ks, vs = src
        st = {}

        def first_row(i, j):
            return max(0, j - TPB * i) * _T

        def accum(old, new, lo, op):
            if old is None:
                return new
            if lo == 0:
                return op(old, new)
            return jnp.concatenate([old[:lo], op(old[lo:], new)], axis=0)

        def qk(i, js):
            s = st.setdefault(i, dict(t={}, m=None, l=None, acc=None))
            q = qs[pl.ds(i * _BQ, _BQ), :]
            for j in js:
                lo = first_row(i, j)
                t = _dot_nt(q[lo:], ks[pl.ds(j * _T, _T), :])
                if j >= TPB * i:
                    top = jnp.where(tri, t[0:_T], _NEG)
                    t = top if t.shape[0] == _T else jnp.concatenate([top, t[_T:]], axis=0)
                s["t"][j] = t
                s["m"] = accum(s["m"], t, lo, jnp.maximum)
            if js[-1] == TPB * (i + 1) - 1:
                s["m"] = jnp.broadcast_to(jnp.max(s["m"], axis=1, keepdims=True), (_BQ, _T))

        def pv(i, js):
            s = st[i]
            for j in js:
                lo = first_row(i, j)
                p = jnp.exp2(s["t"][j] - s["m"][lo:])
                s["l"] = accum(s["l"], p, lo, jnp.add)
                s["acc"] = accum(s["acc"], _dot(p.astype(_BF), vs[pl.ds(j * _T, _T), :]),
                                 lo, jnp.add)
            if js[-1] == TPB * (i + 1) - 1:
                l = jnp.broadcast_to(jnp.sum(s["l"], axis=1, keepdims=True), (_BQ, _T))
                r = pltpu.reciprocal(l, approx=True)
                r = r * (2.0 - l * r)
                ctx_v[h, pl.ds(i * _BQ, _BQ), :] = (s["acc"] * r).astype(_BF)

        def groups(fn, i):
            n = TPB * (i + 1)
            return [(fn, i, list(range(a, min(a + 4, n)))) for a in range(0, n, 4)]

        att = groups(qk, NQ - 1)
        for i in range(NQ - 1, -1, -1):
            att += _merge(groups(qk, i - 1) if i > 0 else [], groups(pv, i))
        side = [] if dst is None else [(f, r) for r in range(NQ) for f in (proj_q, proj_kv)]
        cost = [sum(_BQ - first_row(i, j) for j in js) for _, i, js in att]
        done, k = 0, 0
        for (fn, i, js), c in zip(att, cost):
            fn(i, js)
            done += c
            while k < len(side) - 1 and (k + 0.5) * sum(cost) <= (len(side) - 1) * done:
                side[k][0](side[k][1], dst)
                k += 1
        for f, r in side[k:]:
            f(r, dst)

    buf0, buf1 = (q0, k0, v0), (q1, k1, v1)

    w0 = w_copies(0)
    for cp in [w0[0], w0[1]] + cp_c:
        cp.start()

    def clear(i, carry):
        zero_s[i] = 0
        return carry

    lax.fori_loop(0, zero_s.shape[0], clear, 0)
    w0[0].wait()
    w0[1].wait()
    for cp in [w0[2], cp_gate] + cp_x + w_copies(1):
        cp.start()
    prep_kv(0, False)
    for r in range(NQ):
        if r % (NQ // _NCHUNK) == 0:
            cp_c[r // (NQ // _NCHUNK)].wait()
        proj_kv(r, buf0)
    w0[2].wait()
    prep_q(0, False)
    cp_gate.wait()
    gw = gate_v[...].astype(_F32)
    for r in range(NQ):
        if r % (NQ // _NCHUNK) == 0:
            cp_x[r // (NQ // _NCHUNK)].wait()
        proj_q(r, buf0)
        rows = pl.ds(r * _BQ, _BQ)
        z = None
        for n in range(M // _T):
            t = x_v[rows, pl.ds(n * _T, _T)].astype(_F32) * gw[n:n + 1, :]
            z = t if z is None else z + t
        z = jnp.sum(z, axis=1, keepdims=True)
        g_v[rows, :] = jnp.broadcast_to(1.0 / (1.0 + jnp.exp(-z)), (_BQ, _T))

    def pair_body(p, carry):
        for cp in w_copies(p + 1):
            cp.wait()

        @pl.when(p + 2 < NP)
        def _():
            for cp in w_copies(p + 2):
                cp.start()

        for n, cp in enumerate(cp_late):
            pl.when(p == min(n, 4))(cp.start)

        prep_q(p, True)
        prep_kv(p, True)
        head(2 * p, buf0, buf1)
        prep_q(p + 1, False)
        prep_kv(p + 1, False)
        head(2 * p + 1, buf1, buf0)
        return carry

    lax.fori_loop(0, NP - 1, pair_body, 0)
    prep_q(NP - 1, True)
    prep_kv(NP - 1, True)
    head(H - 2, buf0, buf1)
    head(H - 1, buf1, None)

    for cp in cp_late:
        cp.wait()
    ssmd_f[...] = ssmd_v[...].astype(_F32)
    NC = S // _T
    NB = M // _T
    HF = _T // 2

    def out_copy(cb, slot):
        cols = pl.ds(pl.multiple_of(cb * _T, _T), _T)
        return pltpu.make_async_copy(o_v.at[slot], out_hbm.at[:, cols], sem_o.at[slot])

    kf32[0:8, :] = jnp.zeros((8, _T), _F32)

    def col_body(cb, carry):
        cols = pl.ds(pl.multiple_of(cb * _T, _T), _T)
        slot = cb % 2

        @pl.when(cb >= 2)
        def _():
            out_copy(cb - 2, slot).wait()

        sh = shift_v[:, cols].astype(_F32)
        dvec = ssmd_f[pl.ds(cb, 1), :]
        bacc, kvs, yt, state = {}, {}, {}, {"n": 0}

        def new_step():
            state["z"] = pl.multiple_of(zero_s[state["n"]] * 8, 8)
            state["n"] += 1

        def spec_rows(kind, c, part, fg):
            return pl.ds(state["z"] + ((kind * NC + c) * 2 + part) * _T + fg * 8, 8)

        def spec_load(kind, c, fg):
            return spec_v[spec_rows(kind, c, 0, fg), :], spec_v[spec_rows(kind, c, 1, fg), :]

        def spec_store_all(kind, c, val):
            spec_v[pl.ds(state["z"] + (kind * NC + c) * 2 * _T, 2 * _T), :] = val

        def out_proj(i, g):
            rows = pl.ds(i * _BQ, _BQ)
            for h in range(4 * g, 4 * g + 4):
                t = _dot(ctx_v[h, rows, :], wo_v[h, :, cols])
                bacc[i] = t if h == 0 else bacc[i] + t

        def dft_u(j):
            kf32[pl.ds(8 + j * _T, _T), :] = ak_v[pl.ds(j * _T, _T), cols].astype(_F32)
            acc = kf32[pl.ds(8 + j * _T, _T), :] * sh[0:1, :]
            for s in range(1, sh.shape[0]):
                acc = acc + kf32[pl.ds(8 + j * _T - s, _T), :] * sh[s:s + 1, :]
            kv = (acc * av_v[pl.ds(j * _T, _T), cols].astype(_F32)).astype(_BF)
            kvs[j] = kv
            spec_store_all(0, j, _dot(fwd_v[...], kv))

        def dft_k(j):
            s = _dot_nt(fwd_v[...], sk_v[cols, pl.ds(j * _T, _T)])
            if j == 0:
                spec_store_all(1, j, s)
            else:
                p = state["prev"]
                spec_store_all(1, j, jnp.concatenate(
                    [s[0:HF] - p[_T:_T + HF], s[HF:_T] + p[_T + HF:],
                     s[_T:_T + HF] + p[0:HF], s[_T + HF:] - p[HF:_T]], axis=0))
            state["prev"] = s

        def mac(arg):
            fg, a, b = arg
            new_step()
            kc, y = {}, {}
            if b > 0:
                y = {i: spec_load(2, i, fg) for i in range(4 * a, 4 * a + 4)}
            for j in range(4 * b, 4 * b + 4):
                ur, ui = spec_load(0, j, fg)
                for i in range(max(4 * a, j), 4 * a + 4):
                    if i - j not in kc:
                        kc[i - j] = spec_load(1, i - j, fg)
                    kr, ki = kc[i - j]
                    tr, ti = kr * ur - ki * ui, kr * ui + ki * ur
                    y[i] = (tr, ti) if i not in y else (y[i][0] + tr, y[i][1] + ti)
            for i, (yr, yi) in y.items():
                spec_v[spec_rows(2, i, 0, fg), :] = yr
                spec_v[spec_rows(2, i, 1, fg), :] = yi

        def idft(c):
            new_step()
            spec = spec_v[pl.ds(state["z"] + (2 * NC + c) * 2 * _T, 2 * _T), :]
            yt[c] = _dot(inv_v[...], spec.astype(_BF))

        def combine(c):
            rows = pl.ds(c * _T, _T)
            off = (c % TPB) * _T
            y = yt[c] + kvs[c].astype(_F32) * dvec
            a = x_v[rows, cols].astype(_F32) * y
            g = g_v[rows, :]
            o_v[slot, rows, :] = (g * a + (1.0 - g) * bacc[c // TPB][off:off + _T]).astype(_BF)

        main = [(i, g) for i in range(NQ) for g in range(H // 4)]
        f0, f1, f2, f3 = 0.05, 0.25, 0.8, 0.9
        stage1 = [(dft_k, j) for j in range(NC)] + [(dft_u, j) for j in range(NC)]
        stage2 = [(fg, a, b) for fg in range(_T // 8) for a in range(NC // 4)
                  for b in range(a + 1)]
        side = [(f0 + (f1 - f0) * n / len(stage1), f, a) for n, (f, a) in enumerate(stage1)]
        side += [(f1 + (f2 - f1) * n / len(stage2), mac, a) for n, a in enumerate(stage2)]
        side += [(f2 + (f3 - f2) * c / NC, idft, c) for c in range(NC)]
        side += [(max(f2 + (f3 - f2) * (c + 0.5) / NC, (c // TPB + 1) / NQ), combine, c)
                 for c in range(NC)]
        side.sort(key=lambda t: t[0])
        new_step()
        k = 0
        for n, (i, g) in enumerate(main):
            while k < len(side) and side[k][0] <= n / len(main) + 1e-9:
                side[k][1](side[k][2])
                k += 1
            out_proj(i, g)
        for _, f, a in side[k:]:
            f(a)
        out_copy(cb, slot).start()
        return carry

    lax.fori_loop(0, NB, col_body, 0)
    out_copy(NB - 2, 0).wait()
    out_copy(NB - 1, 1).wait()


@jax.jit
def pallas_gated_mix__ssm_conv_h3__compressed_kv_cla__prompt_kernel(
    A_q: jax.Array,
    A_k: jax.Array,
    A_v: jax.Array,
    A_shift_k: jax.Array,
    A_ssm_k: jax.Array,
    A_ssm_D: jax.Array,
    B_x: jax.Array,
    B_c_kv: jax.Array,
    B_w_q: jax.Array,
    B_w_uk: jax.Array,
    B_w_uv: jax.Array,
    B_w_o: jax.Array,
    gate_w: jax.Array,
):
    del B_x
    B, S, M = A_q.shape
    _, H, D = B_w_q.shape
    DC = B_c_kv.shape[-1]
    assert B == 1 and D == _T and H % 2 == 0 and S % _BQ == 0 and B_c_kv.shape[1] == S
    NP, NC = H // 2, S // _T

    def body(*refs):
        _kernel(*refs, S=S, M=M, H=H, D=D)

    hbm = pl.BlockSpec(memory_space=pl.ANY)
    scratch = [
        pltpu.VMEM((S, M), _BF),
        pltpu.VMEM((S, DC), _BF),
        pltpu.VMEM((NP, M, D), jnp.uint32),
        pltpu.VMEM((NP, DC, D), jnp.uint32),
        pltpu.VMEM((NP, DC, D), jnp.uint32),
        pltpu.VMEM((H, D, M), _BF),
        pltpu.VMEM((S, M), _BF),
        pltpu.VMEM((S, M), _BF),
        pltpu.VMEM((M, S), _BF),
        pltpu.VMEM((H, S, D), _BF),
        pltpu.VMEM((M, D), _BF),
        pltpu.VMEM((DC, 2 * D), _BF),
    ] + [pltpu.VMEM((S, D), _BF)] * 6 + [
        pltpu.VMEM((S, _T), _F32),
        pltpu.VMEM((S + 8, _T), _F32),
        pltpu.VMEM((3 * 2 * S, _T), _F32),
        pltpu.VMEM((2, S, _T), _BF),
        pltpu.VMEM((A_shift_k.shape[1], M), _BF),
        pltpu.VMEM((M // _T, _T), _BF),
        pltpu.VMEM((M // _T, _T), _BF),
        pltpu.VMEM((2 * _T, _T), _BF),
        pltpu.VMEM((_T, 2 * _T), _BF),
        pltpu.VMEM((M // _T, _T), _F32),
        pltpu.SMEM((1 + (_T // 8) * (NC // 4) * (NC // 4 + 1) // 2 + NC,), jnp.int32),
        pltpu.SemaphoreType.DMA((9 + 2 * _NCHUNK,)),
        pltpu.SemaphoreType.DMA((3 * NP,)),
        pltpu.SemaphoreType.DMA((2,)),
    ]
    out = pl.pallas_call(
        body,
        out_shape=jax.ShapeDtypeStruct((S, M), _BF),
        in_specs=[hbm] * 14,
        out_specs=hbm,
        scratch_shapes=scratch,
        compiler_params=pltpu.CompilerParams(vmem_limit_bytes=112 * 2 ** 20),
    )(
        A_q.reshape(S, M), A_k.reshape(S, M), A_v.reshape(S, M), A_shift_k.T, A_ssm_k,
        A_ssm_D.reshape(M // _T, _T), B_c_kv.reshape(S, DC), B_w_q, B_w_uk, B_w_uv, B_w_o,
        gate_w.reshape(M // _T, _T), jnp.asarray(_FWD_NP, _BF), jnp.asarray(_INV_NP, _BF),
    )
    return out.reshape(B, S, M)
```

```python
import numpy as np
import jax
import jax.numpy as jnp
from jax import lax
import jax.experimental.pallas as pl
import jax.experimental.pallas.tpu as pltpu

_BF = jnp.bfloat16
_F32 = jnp.float32
_NT = (((1,), (1,)), ((), ()))
_T = 128
_BQ = 256
_G = 3
_AHEAD = 4
_NEG = -1e30
_LOG2E = 1.4426950408889634


def _dft_tables(c):
    f = np.concatenate([np.arange(0, c, 2), np.arange(1, c, 2)]).astype(np.float64)
    b = np.arange(c, dtype=np.float64)
    ang = np.pi * (f[:, None] + 0.5) * b[None, :] / c
    fwd = np.concatenate([np.cos(ang), -np.sin(ang)], axis=0)
    inv = np.concatenate([np.cos(ang).T, -np.sin(ang).T], axis=1) / c
    return fwd.astype(np.float32), inv.astype(np.float32)


_FWD_NP, _INV_NP = _dft_tables(_T)


def _dot(a, b):
    return jnp.dot(a, b, preferred_element_type=_F32)


def _dot_nt(a, b):
    return lax.dot_general(a, b, _NT, preferred_element_type=_F32)


def _unpack_head(w32, odd):
    bits = (w32 & jnp.uint32(0xFFFF0000)) if odd else (w32 << 16)
    return pltpu.bitcast(bits, _F32).astype(_BF)


def _merge(a, b):
    out, ia, ib = [], 0, 0
    while ia < len(a) or ib < len(b):
        if ib >= len(b) or (ia < len(a) and ia * len(b) <= ib * len(a)):
            out.append(a[ia])
            ia += 1
        else:
            out.append(b[ib])
            ib += 1
    return out


def _kernel(x_hbm, k_hbm, v_hbm, shift_hbm, ssmk_hbm, ssmd_hbm, c_hbm, wq_hbm, wuk_hbm,
            wuv_hbm, wo_hbm, gate_hbm, fwd_hbm, inv_hbm, out_hbm,
            x_v, c_v, wq_v, wuk_v, wuv_v, wo_v, ak_v, av_v, sk_v, ctx_v,
            wq0, wkv0, wq1, wkv1, q0, k0, v0, q1, k1, v1, g_v, kf32, spec_v, o_v,
            shift_v, ssmd_v, gate_v, fwd_v, inv_v, ssmd_f, zero_s,
            sem_in, sem_w, sem_o, *, S, M, H, D):
    NP = H // 2
    NQ = S // _BQ
    TPB = _BQ // _T
    qscale = float(D ** -0.5 * _LOG2E)

    def w_copies(p):
        return [pltpu.make_async_copy(src.bitcast(jnp.uint32).at[:, p, :], dst.at[p],
                                      sem_w.at[3 * p + n])
                for n, (src, dst) in enumerate(((wuk_hbm, wuk_v), (wuv_hbm, wuv_v),
                                                (wq_hbm, wq_v)))]

    cp_gate, *cp_late = [
        pltpu.make_async_copy(src, dst, sem_in.at[n])
        for n, (src, dst) in enumerate((
            (gate_hbm, gate_v), (wo_hbm, wo_v), (k_hbm, ak_v), (v_hbm, av_v), (ssmk_hbm, sk_v),
            (shift_hbm, shift_v), (ssmd_hbm, ssmd_v), (fwd_hbm, fwd_v), (inv_hbm, inv_v)))]

    def row_copies(src, dst, sem0, rows):
        return [pltpu.make_async_copy(src.at[pl.ds(n * rows, rows)], dst.at[pl.ds(n * rows, rows)],
                                      sem_in.at[sem0 + n]) for n in range(S // rows)]

    tri = (lax.broadcasted_iota(jnp.int32, (_T, _T), 1)
           <= lax.broadcasted_iota(jnp.int32, (_T, _T), 0))
    bufs = ((q0, k0, v0, wq0, wkv0), (q1, k1, v1, wq1, wkv1))

    def prep_kv(p, odd):
        wkv_b = bufs[odd][4]
        wkv_b[:, 0:D] = _unpack_head(wuk_v[p], odd)
        wkv_b[:, D:2 * D] = _unpack_head(wuv_v[p], odd)

    def prep_q(p, odd):
        bufs[odd][3][...] = _unpack_head(wq_v[p], odd)

    def prep(p, odd):
        prep_kv(p, odd)
        prep_q(p, odd)

    def proj_q(r, odd):
        q_b, _, _, wq_b, _ = bufs[odd]
        rows = pl.ds(r * _BQ, _BQ)
        q_b[rows, :] = (_dot(x_v[rows, :], wq_b[...]) * qscale).astype(_BF)

    def proj_kv(r, odd):
        _, k_b, v_b, _, wkv_b = bufs[odd]
        rows = pl.ds(r * _BQ, _BQ)
        kv = _dot(c_v[rows, :], wkv_b[...])
        k_b[rows, :] = kv[:, 0:D].astype(_BF)
        v_b[rows, :] = kv[:, D:2 * D].astype(_BF)

    def first_row(i, j):
        return max(0, j - TPB * i) * _T

    def accum(old, new, lo, op):
        if old is None:
            return new
        if lo == 0:
            return op(old, new)
        return jnp.concatenate([old[:lo], op(old[lo:], new)], axis=0)

    def attention(h, odd):
        q_b, k_b, v_b, _, _ = bufs[odd]
        st = {}

        def qk(i, js):
            s = st.setdefault(i, dict(t={}, m=None, l=None, acc=None))
            q = q_b[pl.ds(i * _BQ, _BQ), :]
            for j in js:
                lo = first_row(i, j)
                t = _dot_nt(q[lo:], k_b[pl.ds(j * _T, _T), :])
                if j >= TPB * i:
                    top = jnp.where(tri, t[0:_T], _NEG)
                    t = top if t.shape[0] == _T else jnp.concatenate([top, t[_T:]], axis=0)
                s["t"][j] = t
                s["m"] = accum(s["m"], t, lo, jnp.maximum)
            if js[-1] == TPB * (i + 1) - 1:
                s["m"] = jnp.broadcast_to(jnp.max(s["m"], axis=1, keepdims=True), (_BQ, _T))

        def pv(i, js):
            s = st[i]
            for j in js:
                lo = first_row(i, j)
                p = jnp.exp2(s["t"][j] - s["m"][lo:]).astype(_BF)
                s["l"] = accum(s["l"], p.astype(_F32), lo, jnp.add)
                s["acc"] = accum(s["acc"], _dot(p, v_b[pl.ds(j * _T, _T), :]), lo, jnp.add)
            if js[-1] == TPB * (i + 1) - 1:
                l = jnp.broadcast_to(jnp.sum(s["l"], axis=1, keepdims=True), (_BQ, _T))
                r = pltpu.reciprocal(l, approx=True)
                r = r * (2.0 - l * r)
                ctx_v[h, pl.ds(i * _BQ, _BQ), :] = (s["acc"] * r).astype(_BF)

        def groups(fn, i):
            n = TPB * (i + 1)
            return [(fn, i, list(range(a, min(a + _G, n)))) for a in range(0, n, _G)]

        return (lambda i: groups(qk, i)), (lambda i: groups(pv, i))

    def head(h, odd, project_next):
        qk, pv = attention(h, odd)
        att = qk(NQ - 1)
        for i in range(NQ - 1, -1, -1):
            att += _merge(qk(i - 1) if i > 0 else [], pv(i))
        side = [(f, r) for r in range(NQ) for f in (proj_q, proj_kv)] if project_next else []
        cost = [sum(_BQ - first_row(i, j) for j in js) for _, i, js in att]
        done, k = 0, 0
        for (fn, i, js), c in zip(att, cost):
            fn(i, js)
            done += c
            while k < len(side) - 1 and (k + 0.5) * sum(cost) <= (len(side) - 1) * done:
                side[k][0](side[k][1], 1 - odd)
                k += 1
        for f, r in side[k:]:
            f(r, 1 - odd)

    def prologue():
        cp_c = row_copies(c_hbm, c_v, 9, 2 * _BQ)
        cp_x = row_copies(x_hbm, x_v, 9 + NQ, _BQ)
        cp_uk, cp_uv, cp_q = w_copies(0)
        queue = [cp_uk, cp_uv] + cp_c + [cp_q, cp_gate] + cp_x + w_copies(1)
        for cp in queue[:_AHEAD]:
            cp.start()
        waited = []

        def wait(cp):
            cp.wait()
            waited.append(cp)
            if len(waited) + _AHEAD <= len(queue):
                queue[len(waited) + _AHEAD - 1].start()

        def clear(i, carry):
            zero_s[i] = 0
            return carry

        lax.fori_loop(0, zero_s.shape[0], clear, 0)
        wait(cp_uk)
        wait(cp_uv)
        prep_kv(0, 0)
        for r in range(NQ):
            if r % 2 == 0:
                wait(cp_c[r // 2])
            proj_kv(r, 0)
        wait(cp_q)
        wait(cp_gate)
        prep_q(0, 0)
        gw = gate_v[...].astype(_F32)
        for r in range(NQ):
            wait(cp_x[r])
            proj_q(r, 0)
            rows = pl.ds(r * _BQ, _BQ)
            z = None
            for n in range(M // _T):
                t = x_v[rows, pl.ds(n * _T, _T)].astype(_F32) * gw[n:n + 1, :]
                z = t if z is None else z + t
            g = lax.logistic(jnp.sum(z, axis=1, keepdims=True))
            g_v[rows, :] = jnp.broadcast_to(g, (_BQ, _T))
        for cp in queue[len(waited):]:
            wait(cp)

    def pair_body(p, carry):
        @pl.when(p == 0)
        def _():
            for n in range(2, NP):
                for cp in w_copies(n):
                    cp.start()

        @pl.when(p == 1)
        def _():
            for n in range(2, NP):
                for cp in w_copies(n):
                    cp.wait()
            for cp in cp_late:
                cp.start()

        prep(p, 1)
        head(2 * p, 0, True)
        prep(p + 1, 0)
        head(2 * p + 1, 1, True)
        return carry

    prologue()
    lax.fori_loop(0, NP - 1, pair_body, 0)
    prep(NP - 1, 1)
    head(H - 2, 0, True)
    head(H - 1, 1, False)

    for cp in cp_late:
        cp.wait()
    ssmd_f[...] = ssmd_v[...].astype(_F32)
    NC = S // _T
    NB = M // _T
    HF = _T // 2

    def out_copy(cb):
        cols = pl.ds(cb * _T if isinstance(cb, int) else pl.multiple_of(cb * _T, _T), _T)
        return pltpu.make_async_copy(o_v.at[cb], out_hbm.at[:, cols], sem_o.at[cb])

    kf32[0:8, :] = jnp.zeros((8, _T), _F32)

    def col_body(cb, carry):
        cols = pl.ds(pl.multiple_of(cb * _T, _T), _T)
        sh = shift_v[:, cols].astype(_F32)
        dvec = ssmd_f[pl.ds(cb, 1), :]
        bacc, kvs, yt, state = {}, {}, {}, {"n": 0}

        def new_step():
            state["z"] = pl.multiple_of(zero_s[state["n"]] * 8, 8)
            state["n"] += 1

        def spec_rows(kind, c, part, fg):
            return pl.ds(state["z"] + ((kind * NC + c) * 2 + part) * _T + fg * 8, 8)

        def spec_load(kind, c, fg):
            return spec_v[spec_rows(kind, c, 0, fg), :], spec_v[spec_rows(kind, c, 1, fg), :]

        def spec_store_all(kind, c, val):
            spec_v[pl.ds(state["z"] + (kind * NC + c) * 2 * _T, 2 * _T), :] = val

        def out_proj(i, g):
            rows = pl.ds(i * _BQ, _BQ)
            for h in range(4 * g, 4 * g + 4):
                t = _dot(ctx_v[h, rows, :], wo_v[h, :, cols])
                bacc[i] = t if h == 0 else bacc[i] + t

        def dft_u(j):
            kf32[pl.ds(8 + j * _T, _T), :] = ak_v[pl.ds(j * _T, _T), cols].astype(_F32)
            acc = kf32[pl.ds(8 + j * _T, _T), :] * sh[0:1, :]
            for s in range(1, sh.shape[0]):
                acc = acc + kf32[pl.ds(8 + j * _T - s, _T), :] * sh[s:s + 1, :]
            kv = (acc * av_v[pl.ds(j * _T, _T), cols].astype(_F32)).astype(_BF)
            kvs[j] = kv
            spec_store_all(0, j, _dot(fwd_v[...], kv))

        def dft_k(j):
            s = _dot_nt(fwd_v[...], sk_v[cols, pl.ds(j * _T, _T)])
            if j == 0:
                spec_store_all(1, j, s)
            else:
                p = state["prev"]
                spec_store_all(1, j, jnp.concatenate(
                    [s[0:HF] - p[_T:_T + HF], s[HF:_T] + p[_T + HF:],
                     s[_T:_T + HF] + p[0:HF], s[_T + HF:] - p[HF:_T]], axis=0))
            state["prev"] = s

        def mac(arg):
            fg, a, b = arg
            new_step()
            kc, y = {}, {}
            if b > 0:
                y = {i: spec_load(2, i, fg) for i in range(4 * a, 4 * a + 4)}
            for j in range(4 * b, 4 * b + 4):
                ur, ui = spec_load(0, j, fg)
                for i in range(max(4 * a, j), 4 * a + 4):
                    if i - j not in kc:
                        kc[i - j] = spec_load(1, i - j, fg)
                    kr, ki = kc[i - j]
                    tr, ti = kr * ur - ki * ui, kr * ui + ki * ur
                    y[i] = (tr, ti) if i not in y else (y[i][0] + tr, y[i][1] + ti)
            for i, (yr, yi) in y.items():
                spec_v[spec_rows(2, i, 0, fg), :] = yr
                spec_v[spec_rows(2, i, 1, fg), :] = yi

        def idft(c):
            new_step()
            spec = spec_v[pl.ds(state["z"] + (2 * NC + c) * 2 * _T, 2 * _T), :]
            yt[c] = _dot(inv_v[...], spec.astype(_BF))

        def combine(c):
            rows = pl.ds(c * _T, _T)
            off = (c % TPB) * _T
            y = yt[c] + kvs[c].astype(_F32) * dvec
            a = x_v[rows, cols].astype(_F32) * y
            g = g_v[rows, :]
            o_v[cb, rows, :] = (g * a + (1.0 - g) * bacc[c // TPB][off:off + _T]).astype(_BF)

        main = [(i, g) for i in range(NQ) for g in range(H // 4)]
        f0, f1, f2, f3 = 0.05, 0.25, 0.8, 0.9
        stage1 = [(dft_k, j) for j in range(NC)] + [(dft_u, j) for j in range(NC)]
        stage2 = [(fg, a, b) for fg in range(_T // 8) for a in range(NC // 4)
                  for b in range(a + 1)]
        side = [(f0 + (f1 - f0) * n / len(stage1), f, a) for n, (f, a) in enumerate(stage1)]
        side += [(f1 + (f2 - f1) * n / len(stage2), mac, a) for n, a in enumerate(stage2)]
        side += [(f2 + (f3 - f2) * c / NC, idft, c) for c in range(NC)]
        side += [(max(f2 + (f3 - f2) * (c + 0.5) / NC, (c // TPB + 1) / NQ), combine, c)
                 for c in range(NC)]
        side.sort(key=lambda t: t[0])
        new_step()
        k = 0
        for n, (i, g) in enumerate(main):
            while k < len(side) and side[k][0] <= n / len(main) + 1e-9:
                side[k][1](side[k][2])
                k += 1
            out_proj(i, g)
        for _, f, a in side[k:]:
            f(a)
        out_copy(cb).start()
        return carry

    lax.fori_loop(0, NB, col_body, 0)
    for cb in range(NB):
        out_copy(cb).wait()


@jax.jit
def pallas_gated_mix__ssm_conv_h3__compressed_kv_cla__prompt_kernel(
    A_q: jax.Array,
    A_k: jax.Array,
    A_v: jax.Array,
    A_shift_k: jax.Array,
    A_ssm_k: jax.Array,
    A_ssm_D: jax.Array,
    B_x: jax.Array,
    B_c_kv: jax.Array,
    B_w_q: jax.Array,
    B_w_uk: jax.Array,
    B_w_uv: jax.Array,
    B_w_o: jax.Array,
    gate_w: jax.Array,
):
    del B_x
    B, S, M = A_q.shape
    _, H, D = B_w_q.shape
    DC = B_c_kv.shape[-1]
    assert B == 1 and D == _T and H % 2 == 0 and S % _BQ == 0 and B_c_kv.shape[1] == S
    NP, NC = H // 2, S // _T

    def body(*refs):
        _kernel(*refs, S=S, M=M, H=H, D=D)

    hbm = pl.BlockSpec(memory_space=pl.ANY)
    scratch = [
        pltpu.VMEM((S, M), _BF),
        pltpu.VMEM((S, DC), _BF),
        pltpu.VMEM((NP, M, D), jnp.uint32),
        pltpu.VMEM((NP, DC, D), jnp.uint32),
        pltpu.VMEM((NP, DC, D), jnp.uint32),
        pltpu.VMEM((H, D, M), _BF),
        pltpu.VMEM((S, M), _BF),
        pltpu.VMEM((S, M), _BF),
        pltpu.VMEM((M, S), _BF),
        pltpu.VMEM((H, S, D), _BF),
    ] + [
        pltpu.VMEM((M, D), _BF),
        pltpu.VMEM((DC, 2 * D), _BF),
    ] * 2 + [pltpu.VMEM((S, D), _BF)] * 6 + [
        pltpu.VMEM((S, _T), _F32),
        pltpu.VMEM((S + 8, _T), _F32),
        pltpu.VMEM((3 * 2 * S, _T), _F32),
        pltpu.VMEM((M // _T, S, _T), _BF),
        pltpu.VMEM((A_shift_k.shape[1], M), _BF),
        pltpu.VMEM((M // _T, _T), _BF),
        pltpu.VMEM((M // _T, _T), _BF),
        pltpu.VMEM((2 * _T, _T), _BF),
        pltpu.VMEM((_T, 2 * _T), _BF),
        pltpu.VMEM((M // _T, _T), _F32),
        pltpu.SMEM((1 + (_T // 8) * (NC // 4) * (NC // 4 + 1) // 2 + NC,), jnp.int32),
        pltpu.SemaphoreType.DMA((9 + 2 * (S // _BQ),)),
        pltpu.SemaphoreType.DMA((3 * NP,)),
        pltpu.SemaphoreType.DMA((M // _T,)),
    ]
    out = pl.pallas_call(
        body,
        out_shape=jax.ShapeDtypeStruct((S, M), _BF),
        in_specs=[hbm] * 14,
        out_specs=hbm,
        scratch_shapes=scratch,
        compiler_params=pltpu.CompilerParams(vmem_limit_bytes=112 * 2 ** 20),
    )(
        A_q.reshape(S, M), A_k.reshape(S, M), A_v.reshape(S, M), A_shift_k.T, A_ssm_k,
        A_ssm_D.reshape(M // _T, _T), B_c_kv.reshape(S, DC), B_w_q, B_w_uk, B_w_uv, B_w_o,
        gate_w.reshape(M // _T, _T), jnp.asarray(_FWD_NP, _BF), jnp.asarray(_INV_NP, _BF),
    )
    return out.reshape(B, S, M)
```

```python
import numpy as np
import jax
import jax.numpy as jnp
from jax import lax
import jax.experimental.pallas as pl
import jax.experimental.pallas.tpu as pltpu

_BF = jnp.bfloat16
_F32 = jnp.float32
_NT = (((1,), (1,)), ((), ()))
_T = 128
_BQ = 256
_G = 3
_NEG = -1e30
_LOG2E = 1.4426950408889634


def _dft_tables(c):
    f = np.concatenate([np.arange(0, c, 2), np.arange(1, c, 2)]).astype(np.float64)
    b = np.arange(c, dtype=np.float64)
    ang = np.pi * (f[:, None] + 0.5) * b[None, :] / c
    fwd = np.concatenate([np.cos(ang), -np.sin(ang)], axis=0)
    inv = np.concatenate([np.cos(ang).T, -np.sin(ang).T], axis=1) / c
    return fwd.astype(np.float32), inv.astype(np.float32)


_FWD_NP, _INV_NP = _dft_tables(_T)


def _dot(a, b):
    return jnp.dot(a, b, preferred_element_type=_F32)


def _dot_nt(a, b):
    return lax.dot_general(a, b, _NT, preferred_element_type=_F32)


def _unpack_head(w32, odd):
    bits = (w32 & jnp.uint32(0xFFFF0000)) if odd else (w32 << 16)
    return pltpu.bitcast(bits, _F32).astype(_BF)


def _merge(a, b):
    out, ia, ib = [], 0, 0
    while ia < len(a) or ib < len(b):
        if ib >= len(b) or (ia < len(a) and ia * len(b) <= ib * len(a)):
            out.append(a[ia])
            ia += 1
        else:
            out.append(b[ib])
            ib += 1
    return out


def _kernel(x_hbm, k_hbm, v_hbm, shift_hbm, ssmk_hbm, ssmd_hbm, c_hbm, wq_hbm, wuk_hbm,
            wuv_hbm, wo_hbm, gate_hbm, fwd_hbm, inv_hbm, out_hbm,
            x_v, c_v, wq_v, wuk_v, wuv_v, wo_v, ak_v, av_v, sk_v, ctx_v,
            wq0, wkv0, wq1, wkv1, q0, k0, v0, q1, k1, v1, g_v, kf32, spec_v, o_v,
            shift_v, ssmd_v, gate_v, fwd_v, inv_v, ssmd_f, zero_s,
            sem_in, sem_w, sem_o, *, S, M, H, D):
    NP = H // 2
    NQ = S // _BQ
    TPB = _BQ // _T
    qscale = float(D ** -0.5 * _LOG2E)

    def w_copies(p):
        return [pltpu.make_async_copy(src.bitcast(jnp.uint32).at[:, p, :], dst.at[p],
                                      sem_w.at[3 * p + n])
                for n, (src, dst) in enumerate(((wuk_hbm, wuk_v), (wuv_hbm, wuv_v),
                                                (wq_hbm, wq_v)))]

    cp_gate, *cp_late = [
        pltpu.make_async_copy(src, dst, sem_in.at[n])
        for n, (src, dst) in enumerate((
            (gate_hbm, gate_v), (wo_hbm, wo_v), (k_hbm, ak_v), (v_hbm, av_v), (ssmk_hbm, sk_v),
            (shift_hbm, shift_v), (ssmd_hbm, ssmd_v), (fwd_hbm, fwd_v), (inv_hbm, inv_v)))]

    def aligned(n, size):
        return pl.ds(n * size if isinstance(n, int) else pl.multiple_of(n * size, size), size)

    def row_copy(src, dst, sem0, rows, n):
        return pltpu.make_async_copy(src.at[aligned(n, rows)], dst.at[aligned(n, rows)],
                                     sem_in.at[sem0 + n])

    tri = (lax.broadcasted_iota(jnp.int32, (_T, _T), 1)
           <= lax.broadcasted_iota(jnp.int32, (_T, _T), 0))
    bufs = ((q0, k0, v0, wq0, wkv0), (q1, k1, v1, wq1, wkv1))

    def prep_kv(p, odd):
        wkv_b = bufs[odd][4]
        wkv_b[:, 0:D] = _unpack_head(wuk_v[p], odd)
        wkv_b[:, D:2 * D] = _unpack_head(wuv_v[p], odd)

    def prep_q(p, odd):
        bufs[odd][3][...] = _unpack_head(wq_v[p], odd)

    def prep(p, odd):
        prep_kv(p, odd)
        prep_q(p, odd)

    def proj_q(r, odd):
        q_b, _, _, wq_b, _ = bufs[odd]
        rows = aligned(r, _BQ)
        q_b[rows, :] = (_dot(x_v[rows, :], wq_b[...]) * qscale).astype(_BF)

    def proj_kv(r, odd):
        _, k_b, v_b, _, wkv_b = bufs[odd]
        rows = aligned(r, _BQ)
        kv = _dot(c_v[rows, :], wkv_b[...])
        k_b[rows, :] = kv[:, 0:D].astype(_BF)
        v_b[rows, :] = kv[:, D:2 * D].astype(_BF)

    def first_row(i, j):
        return max(0, j - TPB * i) * _T

    def accum(old, new, lo, op):
        if old is None:
            return new
        if lo == 0:
            return op(old, new)
        return jnp.concatenate([old[:lo], op(old[lo:], new)], axis=0)

    def attention(h, odd):
        q_b, k_b, v_b, _, _ = bufs[odd]
        st = {}

        def qk(i, js):
            s = st.setdefault(i, dict(t={}, m=None, l=None, acc=None))
            q = q_b[pl.ds(i * _BQ, _BQ), :]
            for j in js:
                lo = first_row(i, j)
                t = _dot_nt(q[lo:], k_b[pl.ds(j * _T, _T), :])
                if j >= TPB * i:
                    top = jnp.where(tri, t[0:_T], _NEG)
                    t = top if t.shape[0] == _T else jnp.concatenate([top, t[_T:]], axis=0)
                s["t"][j] = t
                s["m"] = accum(s["m"], t, lo, jnp.maximum)
            if js[-1] == TPB * (i + 1) - 1:
                s["m"] = jnp.broadcast_to(jnp.max(s["m"], axis=1, keepdims=True), (_BQ, _T))

        def pv(i, js):
            s = st[i]
            for j in js:
                lo = first_row(i, j)
                p = jnp.exp2(s["t"][j] - s["m"][lo:]).astype(_BF)
                s["l"] = accum(s["l"], p.astype(_F32), lo, jnp.add)
                s["acc"] = accum(s["acc"], _dot(p, v_b[pl.ds(j * _T, _T), :]), lo, jnp.add)
            if js[-1] == TPB * (i + 1) - 1:
                l = jnp.broadcast_to(jnp.sum(s["l"], axis=1, keepdims=True), (_BQ, _T))
                r = pltpu.reciprocal(l, approx=True)
                r = r * (2.0 - l * r)
                ctx_v[h, pl.ds(i * _BQ, _BQ), :] = (s["acc"] * r).astype(_BF)

        def groups(fn, i):
            n = TPB * (i + 1)
            return [(fn, i, list(range(a, min(a + _G, n)))) for a in range(0, n, _G)]

        return (lambda i: groups(qk, i)), (lambda i: groups(pv, i))

    def head(h, odd, project_next):
        qk, pv = attention(h, odd)
        att = qk(NQ - 1)
        for i in range(NQ - 1, -1, -1):
            att += _merge(qk(i - 1) if i > 0 else [], pv(i))
        side = [(f, r) for r in range(NQ) for f in (proj_q, proj_kv)] if project_next else []
        cost = [sum(_BQ - first_row(i, j) for j in js) for _, i, js in att]
        done, k = 0, 0
        for (fn, i, js), c in zip(att, cost):
            fn(i, js)
            done += c
            while k < len(side) - 1 and (k + 0.5) * sum(cost) <= (len(side) - 1) * done:
                side[k][0](side[k][1], 1 - odd)
                k += 1
        for f, r in side[k:]:
            f(r, 1 - odd)

    def prologue():
        cp_c = [row_copy(c_hbm, c_v, 9, 2 * _BQ, n) for n in range(NQ // 2)]
        cp_x = [row_copy(x_hbm, x_v, 9 + NQ, _BQ, n) for n in range(NQ)]
        cp_uk, cp_uv, cp_q = w_copies(0)

        def clear(i, carry):
            zero_s[i] = 0
            return carry

        def kv_body(n, carry):
            row_copy(c_hbm, c_v, 9, 2 * _BQ, n).wait()
            row_copy(x_hbm, x_v, 9 + NQ, _BQ, 2 * n).start()
            row_copy(x_hbm, x_v, 9 + NQ, _BQ, 2 * n + 1).start()
            proj_kv(2 * n, 0)
            proj_kv(2 * n + 1, 0)
            return carry

        for cp in [cp_uk, cp_uv] + cp_c[:2]:
            cp.start()
        lax.fori_loop(0, zero_s.shape[0], clear, 0)
        cp_uk.wait()
        cp_uv.wait()
        for cp in cp_c[2:] + [cp_q, cp_gate]:
            cp.start()
        prep_kv(0, 0)
        lax.fori_loop(0, NQ // 2, kv_body, 0)
        for cp in w_copies(1):
            cp.start()
        cp_q.wait()
        cp_gate.wait()
        prep_q(0, 0)
        gw = gate_v[...].astype(_F32)
        waits = [0] + list(range(3, NQ, 2)) + [NQ]
        for lo, hi in zip(waits[:-1], waits[1:]):
            for r in range(lo, hi):
                cp_x[r].wait()
            for r in range(lo, hi):
                proj_q(r, 0)
                rows = pl.ds(r * _BQ, _BQ)
                z = None
                for n in range(M // _T):
                    t = x_v[rows, pl.ds(n * _T, _T)].astype(_F32) * gw[n:n + 1, :]
                    z = t if z is None else z + t
                g = lax.logistic(jnp.sum(z, axis=1, keepdims=True))
                g_v[rows, :] = jnp.broadcast_to(g, (_BQ, _T))
        for cp in w_copies(1):
            cp.wait()

    def pair_body(p, carry):
        @pl.when(p == 0)
        def _():
            for n in range(2, NP):
                for cp in w_copies(n):
                    cp.start()

        @pl.when(p == 1)
        def _():
            for n in range(2, NP):
                for cp in w_copies(n):
                    cp.wait()
            for cp in cp_late:
                cp.start()

        prep(p, 1)
        head(2 * p, 0, True)
        prep(p + 1, 0)
        head(2 * p + 1, 1, True)
        return carry

    prologue()
    lax.fori_loop(0, NP - 1, pair_body, 0)
    prep(NP - 1, 1)
    head(H - 2, 0, True)
    head(H - 1, 1, False)

    for cp in cp_late:
        cp.wait()
    ssmd_f[...] = ssmd_v[...].astype(_F32)
    NC = S // _T
    NB = M // _T
    HF = _T // 2

    def out_copy(cb):
        return pltpu.make_async_copy(o_v.at[cb], out_hbm.at[:, aligned(cb, _T)], sem_o.at[cb])

    kf32[0:8, :] = jnp.zeros((8, _T), _F32)

    def col_body(cb, carry):
        cols = aligned(cb, _T)
        sh = shift_v[:, cols].astype(_F32)
        dvec = ssmd_f[pl.ds(cb, 1), :]
        bacc, kvs, yt, state = {}, {}, {}, {"n": 0}

        def new_step():
            state["z"] = pl.multiple_of(zero_s[state["n"]] * 8, 8)
            state["n"] += 1

        def spec_rows(kind, c, part, fg):
            return pl.ds(state["z"] + ((kind * NC + c) * 2 + part) * _T + fg * 8, 8)

        def spec_load(kind, c, fg):
            return spec_v[spec_rows(kind, c, 0, fg), :], spec_v[spec_rows(kind, c, 1, fg), :]

        def spec_store_all(kind, c, val):
            spec_v[pl.ds(state["z"] + (kind * NC + c) * 2 * _T, 2 * _T), :] = val

        def out_proj(i, g):
            rows = pl.ds(i * _BQ, _BQ)
            for h in range(4 * g, 4 * g + 4):
                t = _dot(ctx_v[h, rows, :], wo_v[h, :, cols])
                bacc[i] = t if h == 0 else bacc[i] + t

        def dft_u(j):
            kf32[pl.ds(8 + j * _T, _T), :] = ak_v[pl.ds(j * _T, _T), cols].astype(_F32)
            acc = kf32[pl.ds(8 + j * _T, _T), :] * sh[0:1, :]
            for s in range(1, sh.shape[0]):
                acc = acc + kf32[pl.ds(8 + j * _T - s, _T), :] * sh[s:s + 1, :]
            kv = (acc * av_v[pl.ds(j * _T, _T), cols].astype(_F32)).astype(_BF)
            kvs[j] = kv
            spec_store_all(0, j, _dot(fwd_v[...], kv))

        def dft_k(j):
            s = _dot_nt(fwd_v[...], sk_v[cols, pl.ds(j * _T, _T)])
            if j == 0:
                spec_store_all(1, j, s)
            else:
                p = state["prev"]
                spec_store_all(1, j, jnp.concatenate(
                    [s[0:HF] - p[_T:_T + HF], s[HF:_T] + p[_T + HF:],
                     s[_T:_T + HF] + p[0:HF], s[_T + HF:] - p[HF:_T]], axis=0))
            state["prev"] = s

        def mac(arg):
            fg, a, b = arg
            new_step()
            kc, y = {}, {}
            if b > 0:
                y = {i: spec_load(2, i, fg) for i in range(4 * a, 4 * a + 4)}
            for j in range(4 * b, 4 * b + 4):
                ur, ui = spec_load(0, j, fg)
                for i in range(max(4 * a, j), 4 * a + 4):
                    if i - j not in kc:
                        kc[i - j] = spec_load(1, i - j, fg)
                    kr, ki = kc[i - j]
                    tr, ti = kr * ur - ki * ui, kr * ui + ki * ur
                    y[i] = (tr, ti) if i not in y else (y[i][0] + tr, y[i][1] + ti)
            for i, (yr, yi) in y.items():
                spec_v[spec_rows(2, i, 0, fg), :] = yr
                spec_v[spec_rows(2, i, 1, fg), :] = yi

        def idft(c):
            new_step()
            spec = spec_v[pl.ds(state["z"] + (2 * NC + c) * 2 * _T, 2 * _T), :]
            yt[c] = _dot(inv_v[...], spec.astype(_BF))

        def combine(c):
            rows = pl.ds(c * _T, _T)
            off = (c % TPB) * _T
            y = yt[c] + kvs[c].astype(_F32) * dvec
            a = x_v[rows, cols].astype(_F32) * y
            g = g_v[rows, :]
            o_v[cb, rows, :] = (g * a + (1.0 - g) * bacc[c // TPB][off:off + _T]).astype(_BF)

        main = [(i, g) for i in range(NQ) for g in range(H // 4)]
        f0, f1, f2, f3 = 0.05, 0.25, 0.8, 0.9
        stage1 = [(dft_k, j) for j in range(NC)] + [(dft_u, j) for j in range(NC)]
        stage2 = [(fg, a, b) for fg in range(_T // 8) for a in range(NC // 4)
                  for b in range(a + 1)]
        side = [(f0 + (f1 - f0) * n / len(stage1), f, a) for n, (f, a) in enumerate(stage1)]
        side += [(f1 + (f2 - f1) * n / len(stage2), mac, a) for n, a in enumerate(stage2)]
        side += [(f2 + (f3 - f2) * c / NC, idft, c) for c in range(NC)]
        side += [(max(f2 + (f3 - f2) * (c + 0.5) / NC, (c // TPB + 1) / NQ), combine, c)
                 for c in range(NC)]
        side.sort(key=lambda t: t[0])
        new_step()
        k = 0
        for n, (i, g) in enumerate(main):
            while k < len(side) and side[k][0] <= n / len(main) + 1e-9:
                side[k][1](side[k][2])
                k += 1
            out_proj(i, g)
        for _, f, a in side[k:]:
            f(a)
        out_copy(cb).start()
        return carry

    lax.fori_loop(0, NB, col_body, 0)
    for cb in range(NB):
        out_copy(cb).wait()


@jax.jit
def pallas_gated_mix__ssm_conv_h3__compressed_kv_cla__prompt_kernel(
    A_q: jax.Array,
    A_k: jax.Array,
    A_v: jax.Array,
    A_shift_k: jax.Array,
    A_ssm_k: jax.Array,
    A_ssm_D: jax.Array,
    B_x: jax.Array,
    B_c_kv: jax.Array,
    B_w_q: jax.Array,
    B_w_uk: jax.Array,
    B_w_uv: jax.Array,
    B_w_o: jax.Array,
    gate_w: jax.Array,
):
    del B_x
    B, S, M = A_q.shape
    _, H, D = B_w_q.shape
    DC = B_c_kv.shape[-1]
    assert B == 1 and D == _T and H % 2 == 0 and S % (2 * _BQ) == 0 and B_c_kv.shape[1] == S
    NP, NC = H // 2, S // _T

    def body(*refs):
        _kernel(*refs, S=S, M=M, H=H, D=D)

    hbm = pl.BlockSpec(memory_space=pl.ANY)
    scratch = [
        pltpu.VMEM((S, M), _BF),
        pltpu.VMEM((S, DC), _BF),
        pltpu.VMEM((NP, M, D), jnp.uint32),
        pltpu.VMEM((NP, DC, D), jnp.uint32),
        pltpu.VMEM((NP, DC, D), jnp.uint32),
        pltpu.VMEM((H, D, M), _BF),
        pltpu.VMEM((S, M), _BF),
        pltpu.VMEM((S, M), _BF),
        pltpu.VMEM((M, S), _BF),
        pltpu.VMEM((H, S, D), _BF),
    ] + [
        pltpu.VMEM((M, D), _BF),
        pltpu.VMEM((DC, 2 * D), _BF),
    ] * 2 + [pltpu.VMEM((S, D), _BF)] * 6 + [
        pltpu.VMEM((S, _T), _F32),
        pltpu.VMEM((S + 8, _T), _F32),
        pltpu.VMEM((3 * 2 * S, _T), _F32),
        pltpu.VMEM((M // _T, S, _T), _BF),
        pltpu.VMEM((A_shift_k.shape[1], M), _BF),
        pltpu.VMEM((M // _T, _T), _BF),
        pltpu.VMEM((M // _T, _T), _BF),
        pltpu.VMEM((2 * _T, _T), _BF),
        pltpu.VMEM((_T, 2 * _T), _BF),
        pltpu.VMEM((M // _T, _T), _F32),
        pltpu.SMEM((1 + (_T // 8) * (NC // 4) * (NC // 4 + 1) // 2 + NC,), jnp.int32),
        pltpu.SemaphoreType.DMA((9 + 2 * (S // _BQ),)),
        pltpu.SemaphoreType.DMA((3 * NP,)),
        pltpu.SemaphoreType.DMA((M // _T,)),
    ]
    out = pl.pallas_call(
        body,
        out_shape=jax.ShapeDtypeStruct((S, M), _BF),
        in_specs=[hbm] * 14,
        out_specs=hbm,
        scratch_shapes=scratch,
        compiler_params=pltpu.CompilerParams(vmem_limit_bytes=112 * 2 ** 20),
    )(
        A_q.reshape(S, M), A_k.reshape(S, M), A_v.reshape(S, M), A_shift_k.T, A_ssm_k,
        A_ssm_D.reshape(M // _T, _T), B_c_kv.reshape(S, DC), B_w_q, B_w_uk, B_w_uv, B_w_o,
        gate_w.reshape(M // _T, _T), jnp.asarray(_FWD_NP, _BF), jnp.asarray(_INV_NP, _BF),
    )
    return out.reshape(B, S, M)
```

```python
import numpy as np
import jax
import jax.numpy as jnp
from jax import lax
import jax.experimental.pallas as pl
import jax.experimental.pallas.tpu as pltpu

_BF = jnp.bfloat16
_F32 = jnp.float32
_NT = (((1,), (1,)), ((), ()))
_T = 128
_BQ = 256
_G = 3
_SPEC_STRIDE = _T + 8
_NEG = -1e30
_LOG2E = 1.4426950408889634


def _dft_tables(c):
    f = np.concatenate([np.arange(0, c, 2), np.arange(1, c, 2)]).astype(np.float64)
    w = np.pi * (f + 0.5) / c
    b = np.arange(c, dtype=np.float64)
    n = np.arange(c // 2, dtype=np.float64) + 0.5

    def forward(origin):
        ang = w[:, None] * (b[None, :] - origin)
        return np.concatenate([np.cos(ang), -np.sin(ang)], axis=0)

    inverse = np.concatenate([np.cos(n[:, None] * w[None, :]),
                              np.sin(n[:, None] * w[None, :])], axis=0) / c
    return np.concatenate([forward(0.0), forward((c - 1) / 2), inverse]).astype(np.float32)


_DFT_NP = _dft_tables(_T)


def _dot(a, b):
    return jnp.dot(a, b, preferred_element_type=_F32)


def _dot_nt(a, b):
    return lax.dot_general(a, b, _NT, preferred_element_type=_F32)


def _unpack_head(w32, odd):
    bits = (w32 & jnp.uint32(0xFFFF0000)) if odd else (w32 << 16)
    return pltpu.bitcast(bits, _F32).astype(_BF)


def _merge(a, b):
    out, ia, ib = [], 0, 0
    while ia < len(a) or ib < len(b):
        if ib >= len(b) or (ia < len(a) and ia * len(b) <= ib * len(a)):
            out.append(a[ia])
            ia += 1
        else:
            out.append(b[ib])
            ib += 1
    return out


def _kernel(x_hbm, k_hbm, v_hbm, shift_hbm, ssmk_hbm, ssmd_hbm, c_hbm, wq_hbm, wuk_hbm,
            wuv_hbm, wo_hbm, gate_hbm, dft_hbm, out_hbm,
            x_v, c_v, wq_v, wuk_v, wuv_v, wo_v, ak_v, av_v, sk_v, ctx_v,
            wq0, wkv0, wq1, wkv1, q0, k0, v0, q1, k1, v1, g_v, kf32, spec_v, o_v,
            shift_v, ssmd_v, gate_v, dft_v, ssmd_f, zero_s,
            sem_in, sem_w, sem_o, *, S, M, H, D):
    NP = H // 2
    NQ = S // _BQ
    TPB = _BQ // _T
    qscale = float(D ** -0.5 * _LOG2E)

    def w_copies(p):
        return [pltpu.make_async_copy(src.bitcast(jnp.uint32).at[:, p, :], dst.at[p],
                                      sem_w.at[3 * p + n])
                for n, (src, dst) in enumerate(((wuk_hbm, wuk_v), (wuv_hbm, wuv_v),
                                                (wq_hbm, wq_v)))]

    cp_gate, *cp_late = [
        pltpu.make_async_copy(src, dst, sem_in.at[n])
        for n, (src, dst) in enumerate((
            (gate_hbm, gate_v), (wo_hbm, wo_v.at[:, :, pl.ds(0, M)]), (k_hbm, ak_v),
            (v_hbm, av_v), (ssmk_hbm, sk_v), (shift_hbm, shift_v), (ssmd_hbm, ssmd_v),
            (dft_hbm, dft_v)))]

    def aligned(n, size):
        return pl.ds(n * size if isinstance(n, int) else pl.multiple_of(n * size, size), size)

    def row_copy(src, dst, sem0, rows, n):
        return pltpu.make_async_copy(src.at[aligned(n, rows)], dst.at[aligned(n, rows)],
                                     sem_in.at[sem0 + n])

    tri = (lax.broadcasted_iota(jnp.int32, (_T, _T), 1)
           <= lax.broadcasted_iota(jnp.int32, (_T, _T), 0))
    bufs = ((q0, k0, v0, wq0, wkv0), (q1, k1, v1, wq1, wkv1))

    def prep_kv(p, odd):
        wkv_b = bufs[odd][4]
        wkv_b[:, 0:D] = _unpack_head(wuk_v[p], odd)
        wkv_b[:, D:2 * D] = _unpack_head(wuv_v[p], odd)

    def prep_q(p, odd):
        bufs[odd][3][...] = _unpack_head(wq_v[p], odd)

    def prep(p, odd):
        prep_kv(p, odd)
        prep_q(p, odd)

    def proj_q(r, odd):
        q_b, _, _, wq_b, _ = bufs[odd]
        rows = aligned(r, _BQ)
        q_b[rows, :] = (_dot(x_v[rows, :], wq_b[...]) * qscale).astype(_BF)

    def proj_kv(r, odd):
        _, k_b, v_b, _, wkv_b = bufs[odd]
        rows = aligned(r, _BQ)
        kv = _dot(c_v[rows, :], wkv_b[...])
        k_b[rows, :] = kv[:, 0:D].astype(_BF)
        v_b[rows, :] = kv[:, D:2 * D].astype(_BF)

    def first_row(i, j):
        return max(0, j - TPB * i) * _T

    def accum(old, new, lo, op):
        if old is None:
            return new
        if lo == 0:
            return op(old, new)
        return jnp.concatenate([old[:lo], op(old[lo:], new)], axis=0)

    def attention(h, odd):
        q_b, k_b, v_b, _, _ = bufs[odd]
        st = {}

        def qk(i, js):
            s = st.setdefault(i, dict(t={}, m=None, l=None, acc=None))
            q = q_b[pl.ds(i * _BQ, _BQ), :]
            for j in js:
                lo = first_row(i, j)
                t = _dot_nt(q[lo:], k_b[pl.ds(j * _T, _T), :])
                if j >= TPB * i:
                    top = jnp.where(tri, t[0:_T], _NEG)
                    t = top if t.shape[0] == _T else jnp.concatenate([top, t[_T:]], axis=0)
                s["t"][j] = t
                s["m"] = accum(s["m"], t, lo, jnp.maximum)
            if js[-1] == TPB * (i + 1) - 1:
                s["m"] = jnp.broadcast_to(jnp.max(s["m"], axis=1, keepdims=True), (_BQ, _T))

        def pv(i, js):
            s = st[i]
            for j in js:
                lo = first_row(i, j)
                p = jnp.exp2(s["t"][j] - s["m"][lo:]).astype(_BF)
                s["l"] = accum(s["l"], p.astype(_F32), lo, jnp.add)
                s["acc"] = accum(s["acc"], _dot(p, v_b[pl.ds(j * _T, _T), :]), lo, jnp.add)
            if js[-1] == TPB * (i + 1) - 1:
                l = jnp.broadcast_to(jnp.sum(s["l"], axis=1, keepdims=True), (_BQ, _T))
                r = pltpu.reciprocal(l, approx=True)
                r = r * (2.0 - l * r)
                ctx_v[h, pl.ds(i * _BQ, _BQ), :] = (s["acc"] * r).astype(_BF)

        def groups(fn, i):
            n = TPB * (i + 1)
            return [(fn, i, list(range(a, min(a + _G, n)))) for a in range(0, n, _G)]

        return (lambda i: groups(qk, i)), (lambda i: groups(pv, i))

    def head(h, odd, project_next):
        qk, pv = attention(h, odd)
        att = qk(NQ - 1)
        for i in range(NQ - 1, -1, -1):
            att += _merge(qk(i - 1) if i > 0 else [], pv(i))
        side = [(f, r) for r in range(NQ) for f in (proj_q, proj_kv)] if project_next else []
        cost = [sum(_BQ - first_row(i, j) for j in js) for _, i, js in att]
        done, k = 0, 0
        for (fn, i, js), c in zip(att, cost):
            fn(i, js)
            done += c
            while k < len(side) - 1 and (k + 0.5) * sum(cost) <= (len(side) - 1) * done:
                side[k][0](side[k][1], 1 - odd)
                k += 1
        for f, r in side[k:]:
            f(r, 1 - odd)

    def prologue():
        cp_c = [row_copy(c_hbm, c_v, 9, 2 * _BQ, n) for n in range(NQ // 2)]
        cp_x = [row_copy(x_hbm, x_v, 9 + NQ, _BQ, n) for n in range(NQ)]
        cp_uk, cp_uv, cp_q = w_copies(0)

        def clear(i, carry):
            zero_s[i] = 0
            return carry

        def kv_body(n, carry):
            row_copy(c_hbm, c_v, 9, 2 * _BQ, n).wait()
            row_copy(x_hbm, x_v, 9 + NQ, _BQ, 2 * n).start()
            row_copy(x_hbm, x_v, 9 + NQ, _BQ, 2 * n + 1).start()
            proj_kv(2 * n, 0)
            proj_kv(2 * n + 1, 0)
            return carry

        for cp in [cp_uk, cp_uv] + cp_c[:2]:
            cp.start()
        lax.fori_loop(0, zero_s.shape[0], clear, 0)
        cp_uk.wait()
        cp_uv.wait()
        for cp in cp_c[2:] + [cp_q, cp_gate]:
            cp.start()
        prep_kv(0, 0)
        lax.fori_loop(0, NQ // 2, kv_body, 0)
        for cp in w_copies(1):
            cp.start()
        cp_q.wait()
        cp_gate.wait()
        prep_q(0, 0)
        gw = gate_v[...].astype(_F32)
        waits = [0] + list(range(3, NQ, 2)) + [NQ]
        for lo, hi in zip(waits[:-1], waits[1:]):
            for r in range(lo, hi):
                cp_x[r].wait()
            for r in range(lo, hi):
                proj_q(r, 0)
                rows = pl.ds(r * _BQ, _BQ)
                z = None
                for n in range(M // _T):
                    t = x_v[rows, pl.ds(n * _T, _T)].astype(_F32) * gw[n:n + 1, :]
                    z = t if z is None else z + t
                g = lax.logistic(jnp.sum(z, axis=1, keepdims=True))
                g_v[rows, :] = jnp.broadcast_to(g, (_BQ, _T))
        for cp in w_copies(1):
            cp.wait()

    def pair_body(p, carry):
        @pl.when(p == 0)
        def _():
            for n in range(2, NP):
                for cp in w_copies(n):
                    cp.start()

        @pl.when(p == 1)
        def _():
            for n in range(2, NP):
                for cp in w_copies(n):
                    cp.wait()
            for cp in cp_late:
                cp.start()

        prep(p, 1)
        head(2 * p, 0, True)
        prep(p + 1, 0)
        head(2 * p + 1, 1, True)
        return carry

    prologue()
    lax.fori_loop(0, NP - 1, pair_body, 0)
    prep(NP - 1, 1)
    head(H - 2, 0, True)
    head(H - 1, 1, False)

    for cp in cp_late:
        cp.wait()
    ssmd_f[...] = ssmd_v[...].astype(_F32)
    NC = S // _T
    NB = M // _T
    HF = _T // 2

    def out_copy(cb):
        return pltpu.make_async_copy(o_v.at[cb], out_hbm.at[:, aligned(cb, _T)], sem_o.at[cb])

    kf32[0:8, :] = jnp.zeros((8, _T), _F32)

    def col_body(cb, carry):
        cols = aligned(cb, _T)
        sh = shift_v[:, cols].astype(_F32)
        dvec = ssmd_f[pl.ds(cb, 1), :]
        flip = 7 - lax.broadcasted_iota(jnp.int32, (8, _T), 0)
        bacc, kvs, yt, state = {}, {}, {}, {"n": 0}

        def new_step():
            state["z"] = pl.multiple_of(zero_s[state["n"]] * 8, 8)
            state["n"] += 1

        def spec_rows(kind, c, part, lo=0, n=_T):
            return pl.ds(state["z"] + ((kind * NC + c) * 2 + part) * _SPEC_STRIDE + lo, n)

        def spec_load(kind, c, fg):
            return tuple(spec_v[spec_rows(kind, c, part, fg * 8, 8), :] for part in range(2))

        def spec_store(kind, c, val):
            for part in range(2):
                spec_v[spec_rows(kind, c, part), :] = val[part * _T:(part + 1) * _T]

        def out_proj(i, g):
            rows = pl.ds(i * _BQ, _BQ)
            for h in range(4 * g, 4 * g + 4):
                t = _dot(ctx_v[h, rows, :], wo_v[h, :, cols])
                bacc[i] = t if h == 0 else bacc[i] + t

        def dft_u(j):
            kf32[pl.ds(8 + j * _T, _T), :] = ak_v[pl.ds(j * _T, _T), cols].astype(_F32)
            acc = kf32[pl.ds(8 + j * _T, _T), :] * sh[0:1, :]
            for s in range(1, sh.shape[0]):
                acc = acc + kf32[pl.ds(8 + j * _T - s, _T), :] * sh[s:s + 1, :]
            kv = (acc * av_v[pl.ds(j * _T, _T), cols].astype(_F32)).astype(_BF)
            kvs[j] = kv
            spec_store(0, j, _dot(dft_v[0:2 * _T, :], kv))

        def dft_k(j):
            s = _dot_nt(dft_v[2 * _T:4 * _T, :], sk_v[cols, pl.ds(j * _T, _T)])
            if j == 0:
                spec_store(1, j, s)
            else:
                p = state["prev"]
                spec_store(1, j, jnp.concatenate(
                    [s[0:HF] - p[_T:_T + HF], s[HF:_T] + p[_T + HF:],
                     s[_T:_T + HF] + p[0:HF], s[_T + HF:] - p[HF:_T]], axis=0))
            state["prev"] = s

        def mac(arg):
            fg, a = arg
            new_step()
            kc, y = {}, {}
            for j in range(4 * a + 4):
                ur, ui = spec_load(0, j, fg)
                for i in range(max(4 * a, j), 4 * a + 4):
                    if i - j not in kc:
                        kc[i - j] = spec_load(1, i - j, fg)
                    kr, ki = kc[i - j]
                    tr, ti = kr * ur - ki * ui, kr * ui + ki * ur
                    y[i] = (tr, ti) if i not in y else (y[i][0] + tr, y[i][1] + ti)
            for i, parts in y.items():
                for part in range(2):
                    spec_v[spec_rows(2, i, part, fg * 8, 8), :] = parts[part]

        def idft(c):
            new_step()
            even, odd = [_dot(dft_v[4 * _T + part * HF:4 * _T + (part + 1) * HF, :],
                              spec_v[spec_rows(2, c, part), :].astype(_BF))
                         for part in range(2)]
            mirrored = even + odd
            yt[c] = jnp.concatenate(
                [jnp.take_along_axis(mirrored[lo:lo + 8], flip, axis=0)
                 for lo in range(HF - 8, -8, -8)] + [even - odd], axis=0)

        def combine(c):
            rows = pl.ds(c * _T, _T)
            off = (c % TPB) * _T
            y = yt[c] + kvs[c].astype(_F32) * dvec
            a = x_v[rows, cols].astype(_F32) * y
            g = g_v[rows, :]
            o_v[cb, rows, :] = (g * a + (1.0 - g) * bacc[c // TPB][off:off + _T]).astype(_BF)

        main = [(i, g) for i in range(NQ) for g in range(H // 4)]
        f0, f1, f2, f3 = 0.02, 0.2, 0.85, 0.92
        stage1 = [(dft_k, j) for j in range(NC)] + [(dft_u, j) for j in range(NC)]
        stage2 = [(fg, a) for fg in range(_T // 8) for a in range(NC // 4)]
        side = [(f0 + (f1 - f0) * n / len(stage1), f, a) for n, (f, a) in enumerate(stage1)]
        side += [(f1 + (f2 - f1) * n / len(stage2), mac, a) for n, a in enumerate(stage2)]
        side += [(f2 + (f3 - f2) * c / NC, idft, c) for c in range(NC)]
        side += [(max(f2 + (f3 - f2) * (c + 0.5) / NC, (c // TPB + 1) / NQ), combine, c)
                 for c in range(NC)]
        side.sort(key=lambda t: t[0])
        new_step()
        k = 0
        for n, (i, g) in enumerate(main):
            while k < len(side) and side[k][0] <= n / len(main) + 1e-9:
                side[k][1](side[k][2])
                k += 1
            out_proj(i, g)
        for _, f, a in side[k:]:
            f(a)
        out_copy(cb).start()
        return carry

    lax.fori_loop(0, NB, col_body, 0)
    for cb in range(NB):
        out_copy(cb).wait()


@jax.jit
def pallas_gated_mix__ssm_conv_h3__compressed_kv_cla__prompt_kernel(
    A_q: jax.Array,
    A_k: jax.Array,
    A_v: jax.Array,
    A_shift_k: jax.Array,
    A_ssm_k: jax.Array,
    A_ssm_D: jax.Array,
    B_x: jax.Array,
    B_c_kv: jax.Array,
    B_w_q: jax.Array,
    B_w_uk: jax.Array,
    B_w_uv: jax.Array,
    B_w_o: jax.Array,
    gate_w: jax.Array,
):
    del B_x
    B, S, M = A_q.shape
    _, H, D = B_w_q.shape
    DC = B_c_kv.shape[-1]
    assert B == 1 and D == _T and H % 2 == 0 and S % (2 * _BQ) == 0 and B_c_kv.shape[1] == S
    NP, NC = H // 2, S // _T

    def body(*refs):
        _kernel(*refs, S=S, M=M, H=H, D=D)

    hbm = pl.BlockSpec(memory_space=pl.ANY)
    scratch = [
        pltpu.VMEM((S, M), _BF),
        pltpu.VMEM((S, DC), _BF),
        pltpu.VMEM((NP, M, D), jnp.uint32),
        pltpu.VMEM((NP, DC, D), jnp.uint32),
        pltpu.VMEM((NP, DC, D), jnp.uint32),
        pltpu.VMEM((H, D, M + _T), _BF),
        pltpu.VMEM((S, M), _BF),
        pltpu.VMEM((S, M), _BF),
        pltpu.VMEM((M, S), _BF),
        pltpu.VMEM((H, S, D), _BF),
    ] + [
        pltpu.VMEM((M, D), _BF),
        pltpu.VMEM((DC, 2 * D), _BF),
    ] * 2 + [pltpu.VMEM((S, D), _BF)] * 6 + [
        pltpu.VMEM((S, _T), _F32),
        pltpu.VMEM((S + 8, _T), _F32),
        pltpu.VMEM((3 * 2 * NC * _SPEC_STRIDE, _T), _F32),
        pltpu.VMEM((M // _T, S, _T), _BF),
        pltpu.VMEM((A_shift_k.shape[1], M), _BF),
        pltpu.VMEM((M // _T, _T), _BF),
        pltpu.VMEM((M // _T, _T), _BF),
        pltpu.VMEM(_DFT_NP.shape, _BF),
        pltpu.VMEM((M // _T, _T), _F32),
        pltpu.SMEM((1 + (_T // 8) * (NC // 4) + NC,), jnp.int32),
        pltpu.SemaphoreType.DMA((9 + 2 * (S // _BQ),)),
        pltpu.SemaphoreType.DMA((3 * NP,)),
        pltpu.SemaphoreType.DMA((M // _T,)),
    ]
    out = pl.pallas_call(
        body,
        out_shape=jax.ShapeDtypeStruct((S, M), _BF),
        in_specs=[hbm] * 13,
        out_specs=hbm,
        scratch_shapes=scratch,
        compiler_params=pltpu.CompilerParams(vmem_limit_bytes=112 * 2 ** 20),
    )(
        A_q.reshape(S, M), A_k.reshape(S, M), A_v.reshape(S, M), A_shift_k.T, A_ssm_k,
        A_ssm_D.reshape(M // _T, _T), B_c_kv.reshape(S, DC), B_w_q, B_w_uk, B_w_uv, B_w_o,
        gate_w.reshape(M // _T, _T), jnp.asarray(_DFT_NP, _BF),
    )
    return out.reshape(B, S, M)
```

```python
import numpy as np
import jax
import jax.numpy as jnp
from jax import lax
import jax.experimental.pallas as pl
import jax.experimental.pallas.tpu as pltpu

_BF = jnp.bfloat16
_F32 = jnp.float32
_NT = (((1,), (1,)), ((), ()))
_T = 128
_BQ = 256
_SPEC_STRIDE = _T + 8
_NEG = -1e30
_LOG2E = 1.4426950408889634


def _dft_tables(c):
    f = np.concatenate([np.arange(0, c, 2), np.arange(1, c, 2)]).astype(np.float64)
    w = np.pi * (f + 0.5) / c
    b = np.arange(c, dtype=np.float64)
    n = np.arange(c // 2, dtype=np.float64) + 0.5

    def forward(origin):
        ang = w[:, None] * (b[None, :] - origin)
        return np.concatenate([np.cos(ang), -np.sin(ang)], axis=0)

    inverse = np.concatenate([np.cos(n[:, None] * w[None, :]),
                              np.sin(n[:, None] * w[None, :])], axis=0) / c
    return np.concatenate([forward(0.0), forward((c - 1) / 2), inverse]).astype(np.float32)


_DFT_NP = _dft_tables(_T)


def _dot(a, b):
    return jnp.dot(a, b, preferred_element_type=_F32)


def _dot_nt(a, b):
    return lax.dot_general(a, b, _NT, preferred_element_type=_F32)


def _unpack_head(w32, odd):
    bits = (w32 & jnp.uint32(0xFFFF0000)) if odd else (w32 << 16)
    return pltpu.bitcast(bits, _F32).astype(_BF)


def _merge(a, b):
    out, ia, ib = [], 0, 0
    while ia < len(a) or ib < len(b):
        if ib >= len(b) or (ia < len(a) and ia * len(b) <= ib * len(a)):
            out.append(a[ia])
            ia += 1
        else:
            out.append(b[ib])
            ib += 1
    return out


def _kernel(x_hbm, k_hbm, v_hbm, shift_hbm, ssmk_hbm, ssmd_hbm, c_hbm, wq_hbm, wuk_hbm,
            wuv_hbm, wo_hbm, gate_hbm, dft_hbm, out_hbm,
            x_v, c_v, wq_v, wuk_v, wuv_v, wo_v, ak_v, av_v, sk_v, ctx_v,
            wq0, wkv0, wq1, wkv1, q0, k0, v0, q1, k1, v1, g_v, kf32, spec_v, o_v,
            shift_v, ssmd_v, gate_v, dft_v, ssmd_f, zero_s,
            sem_in, sem_w, sem_o, *, S, M, H, D):
    NP = H // 2
    NQ = S // _BQ
    TPB = _BQ // _T
    qscale = float(D ** -0.5 * _LOG2E)

    def w_copies(p):
        return [pltpu.make_async_copy(src.bitcast(jnp.uint32).at[:, p, :], dst.at[p],
                                      sem_w.at[3 * p + n])
                for n, (src, dst) in enumerate(((wuk_hbm, wuk_v), (wuv_hbm, wuv_v),
                                                (wq_hbm, wq_v)))]

    cp_gate, *cp_late = [
        pltpu.make_async_copy(src, dst, sem_in.at[n])
        for n, (src, dst) in enumerate((
            (gate_hbm, gate_v), (wo_hbm, wo_v.at[:, :, pl.ds(0, M)]), (k_hbm, ak_v),
            (v_hbm, av_v), (ssmk_hbm, sk_v), (shift_hbm, shift_v), (ssmd_hbm, ssmd_v),
            (dft_hbm, dft_v)))]

    def aligned(n, size):
        return pl.ds(n * size if isinstance(n, int) else pl.multiple_of(n * size, size), size)

    def row_copy(src, dst, sem0, rows, n):
        return pltpu.make_async_copy(src.at[aligned(n, rows)], dst.at[aligned(n, rows)],
                                     sem_in.at[sem0 + n])

    tri = (lax.broadcasted_iota(jnp.int32, (_T, _T), 1)
           <= lax.broadcasted_iota(jnp.int32, (_T, _T), 0))
    bufs = ((q0, k0, v0, wq0, wkv0), (q1, k1, v1, wq1, wkv1))

    def prep_kv(p, odd):
        wkv_b = bufs[odd][4]
        wkv_b[:, 0:D] = _unpack_head(wuk_v[p], odd)
        wkv_b[:, D:2 * D] = _unpack_head(wuv_v[p], odd)

    def prep_q(p, odd):
        bufs[odd][3][...] = _unpack_head(wq_v[p], odd)

    def prep(p, odd):
        prep_kv(p, odd)
        prep_q(p, odd)

    def proj_q(r, odd):
        rows = aligned(r, _BQ)
        q = _dot(x_v[rows, :], bufs[odd][3][...]) * qscale
        bufs[odd][0][rows, :] = q.astype(_BF)

    def proj_k(r, odd):
        rows = aligned(r, _BQ)
        bufs[odd][1][rows, :] = _dot(c_v[rows, :], bufs[odd][4][:, 0:D]).astype(_BF)

    def proj_v(r, odd):
        rows = aligned(r, _BQ)
        bufs[odd][2][rows, :] = _dot(c_v[rows, :], bufs[odd][4][:, D:2 * D]).astype(_BF)

    def first_row(i, j):
        return max(0, j - TPB * i) * _T

    def accum(old, new, lo, op):
        if old is None:
            return new
        if lo == 0:
            return op(old, new)
        return jnp.concatenate([old[:lo], op(old[lo:], new)], axis=0)

    def head(h, odd, project_next):
        q_b, k_b, v_b, _, _ = bufs[odd]
        st = {}

        def qk(i, js):
            s = st.setdefault(i, dict(t={}, m=None, l=None, acc=None))
            q = q_b[pl.ds(i * _BQ, _BQ), :]
            for j in js:
                lo = first_row(i, j)
                t = _dot_nt(q[lo:], k_b[pl.ds(j * _T, _T), :])
                if j >= TPB * i:
                    top = jnp.where(tri, t[0:_T], _NEG)
                    t = top if t.shape[0] == _T else jnp.concatenate([top, t[_T:]], axis=0)
                s["t"][j] = t
                s["m"] = accum(s["m"], t, lo, jnp.maximum)
            if js[-1] == TPB * (i + 1) - 1:
                s["m"] = jnp.broadcast_to(jnp.max(s["m"], axis=1, keepdims=True), (_BQ, _T))

        def pv(i, js):
            s = st[i]
            for j in js:
                lo = first_row(i, j)
                p = jnp.exp2(s["t"][j] - s["m"][lo:]).astype(_BF)
                p32 = p.astype(_F32)
                o = _dot(p, v_b[pl.ds(j * _T, _T), :])
                s["l"] = accum(s["l"], p32, lo, jnp.add)
                s["acc"] = accum(s["acc"], o, lo, jnp.add)
            if js[-1] == TPB * (i + 1) - 1:
                l = jnp.broadcast_to(jnp.sum(s["l"], axis=1, keepdims=True), (_BQ, _T))
                r = pltpu.reciprocal(l, approx=True)
                r = r * (2.0 - l * r)
                ctx_v[h, pl.ds(i * _BQ, _BQ), :] = (s["acc"] * r).astype(_BF)

        def groups(fn, i, size):
            n = TPB * (i + 1)
            return [(fn, i, list(range(a, min(a + size, n)))) for a in range(0, n, size)]

        order = list(range(NQ - 1, -1, -1))
        if NQ >= 4:
            order[2], order[3] = order[3], order[2]
        att = groups(qk, order[0], 5)
        for n, i in enumerate(order):
            att += _merge(groups(qk, order[n + 1], 5) if n + 1 < NQ else [], groups(pv, i, 4))
        cost = [sum(_BQ - first_row(i, j) for j in js) * (1.5 if fn is qk else 1.0)
                for fn, i, js in att]

        side = [(f, r, c) for f, c in ((proj_q, 8), (proj_k, 4), (proj_v, 4))
                for r in range(NQ)] if project_next else []
        lead, tail = side[:1], side[len(side) - 3:]
        side = side[1:len(side) - 3]
        budget = sum(c for _, _, c in side)
        for f, r, _ in lead:
            f(r, 1 - odd)
        done = spent = 0
        for (fn, i, js), c in zip(att, cost):
            fn(i, js)
            done += c
            while side and spent + 0.8 * side[0][2] <= budget * (done / sum(cost)):
                f, r, c2 = side.pop(0)
                f(r, 1 - odd)
                spent += c2
        for f, r, _ in side + tail:
            f(r, 1 - odd)

    def prologue():
        cp_c = [row_copy(c_hbm, c_v, 9, 2 * _BQ, n) for n in range(NQ // 2)]
        cp_x = [row_copy(x_hbm, x_v, 9 + NQ, _BQ, n) for n in range(NQ)]
        cp_uk, cp_uv, cp_q = w_copies(0)

        def clear(i, carry):
            zero_s[i] = 0
            return carry

        def kv_body(n, carry):
            row_copy(c_hbm, c_v, 9, 2 * _BQ, n).wait()
            row_copy(x_hbm, x_v, 9 + NQ, _BQ, 2 * n).start()
            row_copy(x_hbm, x_v, 9 + NQ, _BQ, 2 * n + 1).start()
            for r in (2 * n, 2 * n + 1):
                proj_k(r, 0)
                proj_v(r, 0)
            return carry

        for cp in [cp_uk, cp_uv] + cp_c[:2]:
            cp.start()
        lax.fori_loop(0, zero_s.shape[0], clear, 0)
        cp_uk.wait()
        cp_uv.wait()
        for cp in cp_c[2:] + [cp_q, cp_gate]:
            cp.start()
        prep_kv(0, 0)
        lax.fori_loop(0, NQ // 2, kv_body, 0)
        cp_q.wait()
        cp_gate.wait()
        prep_q(0, 0)
        prep(0, 1)
        gw = gate_v[...].astype(_F32)
        waits = [0] + list(range(3, NQ, 2)) + [NQ]
        for lo, hi in zip(waits[:-1], waits[1:]):
            for r in range(lo, hi):
                cp_x[r].wait()
            if lo == waits[1]:
                for cp in w_copies(1):
                    cp.start()
            for r in range(lo, hi):
                proj_q(r, 0)
                rows = pl.ds(r * _BQ, _BQ)
                z = None
                for n in range(M // _T):
                    t = x_v[rows, pl.ds(n * _T, _T)].astype(_F32) * gw[n:n + 1, :]
                    z = t if z is None else z + t
                g = lax.logistic(jnp.sum(z, axis=1, keepdims=True))
                g_v[rows, :] = jnp.broadcast_to(g, (_BQ, _T))
        for cp in w_copies(1):
            cp.wait()

    def pair_body(p, carry):
        @pl.when(p == 0)
        def _():
            for n in range(2, NP):
                for cp in w_copies(n):
                    cp.start()

        @pl.when(p == 1)
        def _():
            for n in range(2, NP):
                for cp in w_copies(n):
                    cp.wait()
            for cp in cp_late:
                cp.start()

        prep(p + 1, 0)
        head(2 * p, 0, True)
        prep(p + 1, 1)
        head(2 * p + 1, 1, True)
        return carry

    prologue()
    lax.fori_loop(0, NP - 1, pair_body, 0)
    head(H - 2, 0, True)
    head(H - 1, 1, False)

    for cp in cp_late:
        cp.wait()
    ssmd_f[...] = ssmd_v[...].astype(_F32)
    NC = S // _T
    NB = M // _T
    HF = _T // 2

    def out_copy(cb):
        return pltpu.make_async_copy(o_v.at[cb], out_hbm.at[:, aligned(cb, _T)], sem_o.at[cb])

    kf32[0:8, :] = jnp.zeros((8, _T), _F32)

    def col_body(cb, carry):
        cols = aligned(cb, _T)
        sh = shift_v[:, cols].astype(_F32)
        dvec = ssmd_f[pl.ds(cb, 1), :]
        flip = 7 - lax.broadcasted_iota(jnp.int32, (8, _T), 0)
        bacc, kvs, yt, state = {}, {}, {}, {"n": 0}

        def new_step():
            state["z"] = pl.multiple_of(zero_s[state["n"]] * 8, 8)
            state["n"] += 1

        def spec_rows(kind, c, part, lo=0, n=_T):
            return pl.ds(state["z"] + ((kind * NC + c) * 2 + part) * _SPEC_STRIDE + lo, n)

        def spec_load(kind, c, fg):
            return tuple(spec_v[spec_rows(kind, c, part, fg * 8, 8), :] for part in range(2))

        def spec_store(kind, c, val):
            for part in range(2):
                spec_v[spec_rows(kind, c, part), :] = val[part * _T:(part + 1) * _T]

        def out_proj(i, g):
            rows = pl.ds(i * _BQ, _BQ)
            for h in range(4 * g, 4 * g + 4):
                t = _dot(ctx_v[h, rows, :], wo_v[h, :, cols])
                bacc[i] = t if h == 0 else bacc[i] + t

        def dft_u(j):
            kf32[pl.ds(8 + j * _T, _T), :] = ak_v[pl.ds(j * _T, _T), cols].astype(_F32)
            acc = kf32[pl.ds(8 + j * _T, _T), :] * sh[0:1, :]
            for s in range(1, sh.shape[0]):
                acc = acc + kf32[pl.ds(8 + j * _T - s, _T), :] * sh[s:s + 1, :]
            kv = (acc * av_v[pl.ds(j * _T, _T), cols].astype(_F32)).astype(_BF)
            kvs[j] = kv
            spec_store(0, j, _dot(dft_v[0:2 * _T, :], kv))

        def dft_k(j):
            s = _dot_nt(dft_v[2 * _T:4 * _T, :], sk_v[cols, pl.ds(j * _T, _T)])
            if j == 0:
                spec_store(1, j, s)
            else:
                p = state["prev"]
                spec_store(1, j, jnp.concatenate(
                    [s[0:HF] - p[_T:_T + HF], s[HF:_T] + p[_T + HF:],
                     s[_T:_T + HF] + p[0:HF], s[_T + HF:] - p[HF:_T]], axis=0))
            state["prev"] = s

        def mac(arg):
            fg, a = arg
            new_step()
            kc, y = {}, {}
            for j in range(4 * a + 4):
                ur, ui = spec_load(0, j, fg)
                for i in range(max(4 * a, j), 4 * a + 4):
                    if i - j not in kc:
                        kc[i - j] = spec_load(1, i - j, fg)
                    kr, ki = kc[i - j]
                    tr, ti = kr * ur - ki * ui, kr * ui + ki * ur
                    y[i] = (tr, ti) if i not in y else (y[i][0] + tr, y[i][1] + ti)
            for i, parts in y.items():
                for part in range(2):
                    spec_v[spec_rows(2, i, part, fg * 8, 8), :] = parts[part]

        def idft(c):
            new_step()
            even, odd = [_dot(dft_v[4 * _T + part * HF:4 * _T + (part + 1) * HF, :],
                              spec_v[spec_rows(2, c, part), :].astype(_BF))
                         for part in range(2)]
            mirrored = even + odd
            yt[c] = jnp.concatenate(
                [jnp.take_along_axis(mirrored[lo:lo + 8], flip, axis=0)
                 for lo in range(HF - 8, -8, -8)] + [even - odd], axis=0)

        def combine(c):
            rows = pl.ds(c * _T, _T)
            off = (c % TPB) * _T
            y = yt[c] + kvs[c].astype(_F32) * dvec
            a = x_v[rows, cols].astype(_F32) * y
            g = g_v[rows, :]
            o_v[cb, rows, :] = (g * a + (1.0 - g) * bacc[c // TPB][off:off + _T]).astype(_BF)

        main = [(i, g) for i in range(NQ) for g in range(H // 4)]
        f0, f1, f2, f3 = 0.02, 0.2, 0.85, 0.92
        stage1 = [(dft_k, j) for j in range(NC)] + [(dft_u, j) for j in range(NC)]
        stage2 = [(fg, a) for fg in range(_T // 8) for a in range(NC // 4)]
        side = [(f0 + (f1 - f0) * n / len(stage1), f, a) for n, (f, a) in enumerate(stage1)]
        side += [(f1 + (f2 - f1) * n / len(stage2), mac, a) for n, a in enumerate(stage2)]
        side += [(f2 + (f3 - f2) * c / NC, idft, c) for c in range(NC)]
        side += [(max(f2 + (f3 - f2) * (c + 0.5) / NC, (c // TPB + 1) / NQ), combine, c)
                 for c in range(NC)]
        side.sort(key=lambda t: t[0])
        new_step()
        k = 0
        for n, (i, g) in enumerate(main):
            while k < len(side) and side[k][0] <= n / len(main) + 1e-9:
                side[k][1](side[k][2])
                k += 1
            out_proj(i, g)
        for _, f, a in side[k:]:
            f(a)
        out_copy(cb).start()
        return carry

    lax.fori_loop(0, NB, col_body, 0)
    for cb in range(NB):
        out_copy(cb).wait()


@jax.jit
def pallas_gated_mix__ssm_conv_h3__compressed_kv_cla__prompt_kernel(
    A_q: jax.Array,
    A_k: jax.Array,
    A_v: jax.Array,
    A_shift_k: jax.Array,
    A_ssm_k: jax.Array,
    A_ssm_D: jax.Array,
    B_x: jax.Array,
    B_c_kv: jax.Array,
    B_w_q: jax.Array,
    B_w_uk: jax.Array,
    B_w_uv: jax.Array,
    B_w_o: jax.Array,
    gate_w: jax.Array,
):
    del B_x
    B, S, M = A_q.shape
    _, H, D = B_w_q.shape
    DC = B_c_kv.shape[-1]
    assert B == 1 and D == _T and H % 2 == 0 and S % (2 * _BQ) == 0 and B_c_kv.shape[1] == S
    NP, NC = H // 2, S // _T

    def body(*refs):
        _kernel(*refs, S=S, M=M, H=H, D=D)

    hbm = pl.BlockSpec(memory_space=pl.ANY)
    scratch = [
        pltpu.VMEM((S, M), _BF),
        pltpu.VMEM((S, DC), _BF),
        pltpu.VMEM((NP, M, D), jnp.uint32),
        pltpu.VMEM((NP, DC, D), jnp.uint32),
        pltpu.VMEM((NP, DC, D), jnp.uint32),
        pltpu.VMEM((H, D, M + _T), _BF),
        pltpu.VMEM((S, M), _BF),
        pltpu.VMEM((S, M), _BF),
        pltpu.VMEM((M, S), _BF),
        pltpu.VMEM((H, S, D), _BF),
    ] + [
        pltpu.VMEM((M, D), _BF),
        pltpu.VMEM((DC, 2 * D), _BF),
    ] * 2 + [pltpu.VMEM((S, D), _BF)] * 6 + [
        pltpu.VMEM((S, _T), _F32),
        pltpu.VMEM((S + 8, _T), _F32),
        pltpu.VMEM((3 * 2 * NC * _SPEC_STRIDE, _T), _F32),
        pltpu.VMEM((M // _T, S, _T), _BF),
        pltpu.VMEM((A_shift_k.shape[1], M), _BF),
        pltpu.VMEM((M // _T, _T), _BF),
        pltpu.VMEM((M // _T, _T), _BF),
        pltpu.VMEM(_DFT_NP.shape, _BF),
        pltpu.VMEM((M // _T, _T), _F32),
        pltpu.SMEM((1 + (_T // 8) * (NC // 4) + NC,), jnp.int32),
        pltpu.SemaphoreType.DMA((9 + 2 * (S // _BQ),)),
        pltpu.SemaphoreType.DMA((3 * NP,)),
        pltpu.SemaphoreType.DMA((M // _T,)),
    ]
    out = pl.pallas_call(
        body,
        out_shape=jax.ShapeDtypeStruct((S, M), _BF),
        in_specs=[hbm] * 13,
        out_specs=hbm,
        scratch_shapes=scratch,
        compiler_params=pltpu.CompilerParams(vmem_limit_bytes=112 * 2 ** 20),
    )(
        A_q.reshape(S, M), A_k.reshape(S, M), A_v.reshape(S, M), A_shift_k.T, A_ssm_k,
        A_ssm_D.reshape(M // _T, _T), B_c_kv.reshape(S, DC), B_w_q, B_w_uk, B_w_uv, B_w_o,
        gate_w.reshape(M // _T, _T), jnp.asarray(_DFT_NP, _BF),
    )
    return out.reshape(B, S, M)
```

```python
import numpy as np
import jax
import jax.numpy as jnp
from jax import lax
import jax.experimental.pallas as pl
import jax.experimental.pallas.tpu as pltpu

_BF = jnp.bfloat16
_F32 = jnp.float32
_NT = (((1,), (1,)), ((), ()))
_T = 128
_BQ = 256
_SPEC_STRIDE = _T + 8
_NEG = -1e30
_LOG2E = 1.4426950408889634


def _dft_tables(c):
    f = np.concatenate([np.arange(0, c, 2), np.arange(1, c, 2)]).astype(np.float64)
    w = np.pi * (f + 0.5) / c
    b = np.arange(c, dtype=np.float64)
    n = np.arange(c // 2, dtype=np.float64) + 0.5

    def forward(origin):
        ang = w[:, None] * (b[None, :] - origin)
        return np.concatenate([np.cos(ang), -np.sin(ang)], axis=0)

    inverse = np.concatenate([np.cos(n[:, None] * w[None, :]),
                              np.sin(n[:, None] * w[None, :])], axis=0) / c
    return np.concatenate([forward(0.0), forward((c - 1) / 2), inverse]).astype(np.float32)


_DFT_NP = _dft_tables(_T)


def _dot(a, b):
    return jnp.dot(a, b, preferred_element_type=_F32)


def _dot_nt(a, b):
    return lax.dot_general(a, b, _NT, preferred_element_type=_F32)


def _unpack_head(w32, odd):
    bits = (w32 & jnp.uint32(0xFFFF0000)) if odd else (w32 << 16)
    return pltpu.bitcast(bits, _F32).astype(_BF)


def _merge(a, b):
    out, ia, ib = [], 0, 0
    while ia < len(a) or ib < len(b):
        if ib >= len(b) or (ia < len(a) and ia * len(b) <= ib * len(a)):
            out.append(a[ia])
            ia += 1
        else:
            out.append(b[ib])
            ib += 1
    return out


def _kernel(x_hbm, k_hbm, v_hbm, shift_hbm, ssmk_hbm, ssmd_hbm, c_hbm, wq_hbm, wuk_hbm,
            wuv_hbm, wo_hbm, gate_hbm, dft_hbm, out_hbm,
            x_v, c_v, wq_v, wuk_v, wuv_v, wo_v, ak_v, av_v, sk_v, ctx_v,
            wq0, wkv0, wq1, wkv1, q0, k0, v0, q1, k1, v1, g_v, kf32, spec_v, o_v,
            shift_v, ssmd_v, gate_v, dft_v, ssmd_f, zero_s,
            sem, sem_c, sem_x, *, S, M, H, D):
    NP = H // 2
    NQ = S // _BQ
    TPB = _BQ // _T
    qscale = float(D ** -0.5 * _LOG2E)

    def w_copies(p, sems):
        return [pltpu.make_async_copy(src.bitcast(jnp.uint32).at[:, p, :], dst.at[p], sem.at[n])
                for n, (src, dst) in zip(sems, ((wuk_hbm, wuk_v), (wuv_hbm, wuv_v),
                                                (wq_hbm, wq_v)))]

    cp_gate = pltpu.make_async_copy(gate_hbm, gate_v, sem.at[1])
    cp_w1 = w_copies(1, (2, 2, 2))
    cp_w = [cp for n in range(2, NP) for cp in w_copies(n, (3, 3, 3))]
    cp_late = [pltpu.make_async_copy(src, dst, sem.at[4]) for src, dst in (
        (wo_hbm, wo_v.at[:, :, pl.ds(0, M)]), (k_hbm, ak_v), (v_hbm, av_v), (ssmk_hbm, sk_v),
        (shift_hbm, shift_v), (ssmd_hbm, ssmd_v), (dft_hbm, dft_v))]

    def aligned(n, size):
        return pl.ds(n * size if isinstance(n, int) else pl.multiple_of(n * size, size), size)

    def c_copy(n):
        rows = aligned(n, 2 * _BQ)
        return pltpu.make_async_copy(c_hbm.at[rows], c_v.at[rows], sem_c.at[n])

    def x_copy(n):
        rows = aligned(n, _BQ)
        return pltpu.make_async_copy(x_hbm.at[rows], x_v.at[rows], sem_x.at[n])

    def out_copy(cb):
        return pltpu.make_async_copy(o_v.at[cb], out_hbm.at[:, aligned(cb, _T)], sem.at[5])

    tri = (lax.broadcasted_iota(jnp.int32, (_T, _T), 1)
           <= lax.broadcasted_iota(jnp.int32, (_T, _T), 0))
    bufs = ((q0, k0, v0, wq0, wkv0), (q1, k1, v1, wq1, wkv1))

    def prep_kv(p, odd):
        wkv_b = bufs[odd][4]
        wkv_b[:, 0:D] = _unpack_head(wuk_v[p], odd)
        wkv_b[:, D:2 * D] = _unpack_head(wuv_v[p], odd)

    def prep_q(p, odd):
        bufs[odd][3][...] = _unpack_head(wq_v[p], odd)

    def prep(p, odd):
        prep_kv(p, odd)
        prep_q(p, odd)

    def proj_q(r, odd):
        rows = aligned(r, _BQ)
        q = _dot(x_v[rows, :], bufs[odd][3][...]) * qscale
        bufs[odd][0][rows, :] = q.astype(_BF)

    def proj_k(r, odd):
        rows = aligned(r, _BQ)
        bufs[odd][1][rows, :] = _dot(c_v[rows, :], bufs[odd][4][:, 0:D]).astype(_BF)

    def proj_v(r, odd):
        rows = aligned(r, _BQ)
        bufs[odd][2][rows, :] = _dot(c_v[rows, :], bufs[odd][4][:, D:2 * D]).astype(_BF)

    def first_row(i, j):
        return max(0, j - TPB * i) * _T

    def accum(old, new, lo, op):
        if old is None:
            return new
        if lo == 0:
            return op(old, new)
        return jnp.concatenate([old[:lo], op(old[lo:], new)], axis=0)

    def head(h, odd, project_next):
        q_b, k_b, v_b, _, _ = bufs[odd]
        st = {}

        def qk(i, js):
            s = st.setdefault(i, dict(t={}, m=None, l=None, acc=None))
            q = q_b[pl.ds(i * _BQ, _BQ), :]
            for j in js:
                lo = first_row(i, j)
                t = _dot_nt(q[lo:], k_b[pl.ds(j * _T, _T), :])
                if j >= TPB * i:
                    top = jnp.where(tri, t[0:_T], _NEG)
                    t = top if t.shape[0] == _T else jnp.concatenate([top, t[_T:]], axis=0)
                s["t"][j] = t
                s["m"] = accum(s["m"], t, lo, jnp.maximum)
            if js[-1] == TPB * (i + 1) - 1:
                s["m"] = jnp.broadcast_to(jnp.max(s["m"], axis=1, keepdims=True), (_BQ, _T))

        def pv(i, js):
            s = st[i]
            for j in js:
                lo = first_row(i, j)
                p = jnp.exp2(s["t"][j] - s["m"][lo:]).astype(_BF)
                p32 = p.astype(_F32)
                o = _dot(p, v_b[pl.ds(j * _T, _T), :])
                s["l"] = accum(s["l"], p32, lo, jnp.add)
                s["acc"] = accum(s["acc"], o, lo, jnp.add)
            if js[-1] == TPB * (i + 1) - 1:
                l = jnp.broadcast_to(jnp.sum(s["l"], axis=1, keepdims=True), (_BQ, _T))
                r = pltpu.reciprocal(l, approx=True)
                r = r * (2.0 - l * r)
                ctx_v[h, pl.ds(i * _BQ, _BQ), :] = (s["acc"] * r).astype(_BF)

        def groups(fn, i, size):
            n = TPB * (i + 1)
            return [(fn, i, list(range(a, min(a + size, n)))) for a in range(0, n, size)]

        order = list(range(NQ - 1, -1, -1))
        if NQ >= 4:
            order[2], order[3] = order[3], order[2]
        att = groups(qk, order[0], 5)
        for n, i in enumerate(order):
            att += _merge(groups(qk, order[n + 1], 5) if n + 1 < NQ else [], groups(pv, i, 4))
        cost = [sum(_BQ - first_row(i, j) for j in js) * (1.5 if fn is qk else 1.0)
                for fn, i, js in att]

        side = [(f, r, c) for f, c in ((proj_q, 8), (proj_k, 4), (proj_v, 4))
                for r in range(NQ)] if project_next else []
        lead, tail = side[:1], side[len(side) - 3:]
        side = side[1:len(side) - 3]
        budget = sum(c for _, _, c in side)
        for f, r, _ in lead:
            f(r, 1 - odd)
        done = spent = 0
        for (fn, i, js), c in zip(att, cost):
            fn(i, js)
            done += c
            while side and spent + 0.8 * side[0][2] <= budget * (done / sum(cost)):
                f, r, c2 = side.pop(0)
                f(r, 1 - odd)
                spent += c2
        for f, r, _ in side + tail:
            f(r, 1 - odd)

    def prologue():
        cp_uk, cp_uv, cp_q = w_copies(0, (0, 0, 1))

        def clear(i, carry):
            zero_s[i] = 0
            return carry

        def kv_body(n, carry):
            c_copy(n).wait()
            x_copy(2 * n).start()
            x_copy(2 * n + 1).start()
            for r in (2 * n, 2 * n + 1):
                proj_k(r, 0)
                proj_v(r, 0)
            return carry

        for cp in (cp_uk, cp_uv, c_copy(0), c_copy(1)):
            cp.start()
        lax.fori_loop(0, zero_s.shape[0], clear, 0)
        cp_uk.wait()
        cp_uv.wait()
        for cp in [c_copy(n) for n in range(2, NQ // 2)] + [cp_q, cp_gate]:
            cp.start()
        prep_kv(0, 0)
        lax.fori_loop(0, NQ // 2, kv_body, 0)
        cp_q.wait()
        cp_gate.wait()
        prep_q(0, 0)
        prep(0, 1)
        gw = gate_v[...].astype(_F32)
        waits = [0] + list(range(3, NQ, 2)) + [NQ]
        for lo, hi in zip(waits[:-1], waits[1:]):
            for r in range(lo, hi):
                x_copy(r).wait()
            if lo == waits[1]:
                for cp in cp_w1:
                    cp.start()
            for r in range(lo, hi):
                proj_q(r, 0)
                rows = pl.ds(r * _BQ, _BQ)
                z = None
                for n in range(M // _T):
                    t = x_v[rows, pl.ds(n * _T, _T)].astype(_F32) * gw[n:n + 1, :]
                    z = t if z is None else z + t
                g = lax.logistic(jnp.sum(z, axis=1, keepdims=True))
                g_v[rows, :] = jnp.broadcast_to(g, (_BQ, _T))
        for cp in cp_w1:
            cp.wait()

    def pair_body(p, carry):
        @pl.when(p == 0)
        def _():
            for cp in cp_w:
                cp.start()

        @pl.when(p == 1)
        def _():
            for cp in cp_w:
                cp.wait()
            for cp in cp_late:
                cp.start()

        prep(p + 1, 0)
        head(2 * p, 0, True)
        prep(p + 1, 1)
        head(2 * p + 1, 1, True)
        return carry

    prologue()
    lax.fori_loop(0, NP - 1, pair_body, 0)
    head(H - 2, 0, True)
    head(H - 1, 1, False)

    for cp in cp_late:
        cp.wait()
    ssmd_f[...] = ssmd_v[...].astype(_F32)
    NC = S // _T
    NB = M // _T
    HF = _T // 2

    kf32[0:8, :] = jnp.zeros((8, _T), _F32)

    def col_body(cb, carry):
        cols = aligned(cb, _T)
        sh = shift_v[:, cols].astype(_F32)
        dvec = ssmd_f[pl.ds(cb, 1), :]
        flip = 7 - lax.broadcasted_iota(jnp.int32, (8, _T), 0)
        bacc, kvs, yt, state = {}, {}, {}, {"n": 0}

        def new_step():
            state["z"] = pl.multiple_of(zero_s[state["n"]] * 8, 8)
            state["n"] += 1

        def spec_rows(kind, c, part, lo=0, n=_T):
            return pl.ds(state["z"] + ((kind * NC + c) * 2 + part) * _SPEC_STRIDE + lo, n)

        def spec_load(kind, c, fg):
            return tuple(spec_v[spec_rows(kind, c, part, fg * 8, 8), :] for part in range(2))

        def spec_store(kind, c, val):
            for part in range(2):
                spec_v[spec_rows(kind, c, part), :] = val[part * _T:(part + 1) * _T]

        def out_proj(i, g):
            rows = pl.ds(i * _BQ, _BQ)
            for h in range(4 * g, 4 * g + 4):
                t = _dot(ctx_v[h, rows, :], wo_v[h, :, cols])
                bacc[i] = t if h == 0 else bacc[i] + t

        def dft_u(j):
            kf32[pl.ds(8 + j * _T, _T), :] = ak_v[pl.ds(j * _T, _T), cols].astype(_F32)
            acc = kf32[pl.ds(8 + j * _T, _T), :] * sh[0:1, :]
            for s in range(1, sh.shape[0]):
                acc = acc + kf32[pl.ds(8 + j * _T - s, _T), :] * sh[s:s + 1, :]
            kv = (acc * av_v[pl.ds(j * _T, _T), cols].astype(_F32)).astype(_BF)
            kvs[j] = kv
            spec_store(0, j, _dot(dft_v[0:2 * _T, :], kv))

        def dft_k(j):
            s = _dot_nt(dft_v[2 * _T:4 * _T, :], sk_v[cols, pl.ds(j * _T, _T)])
            if j == 0:
                spec_store(1, j, s)
            else:
                p = state["prev"]
                spec_store(1, j, jnp.concatenate(
                    [s[0:HF] - p[_T:_T + HF], s[HF:_T] + p[_T + HF:],
                     s[_T:_T + HF] + p[0:HF], s[_T + HF:] - p[HF:_T]], axis=0))
            state["prev"] = s

        def mac(arg):
            fg, a = arg
            new_step()
            kc, y = {}, {}
            for j in range(4 * a + 4):
                ur, ui = spec_load(0, j, fg)
                for i in range(max(4 * a, j), 4 * a + 4):
                    if i - j not in kc:
                        kc[i - j] = spec_load(1, i - j, fg)
                    kr, ki = kc[i - j]
                    tr, ti = kr * ur - ki * ui, kr * ui + ki * ur
                    y[i] = (tr, ti) if i not in y else (y[i][0] + tr, y[i][1] + ti)
            for i, parts in y.items():
                for part in range(2):
                    spec_v[spec_rows(2, i, part, fg * 8, 8), :] = parts[part]

        def idft(c):
            new_step()
            even, odd = [_dot(dft_v[4 * _T + part * HF:4 * _T + (part + 1) * HF, :],
                              spec_v[spec_rows(2, c, part), :].astype(_BF))
                         for part in range(2)]
            mirrored = even + odd
            yt[c] = jnp.concatenate(
                [jnp.take_along_axis(mirrored[lo:lo + 8], flip, axis=0)
                 for lo in range(HF - 8, -8, -8)] + [even - odd], axis=0)

        def combine(c):
            rows = pl.ds(c * _T, _T)
            off = (c % TPB) * _T
            y = yt[c] + kvs[c].astype(_F32) * dvec
            a = x_v[rows, cols].astype(_F32) * y
            g = g_v[rows, :]
            o_v[cb, rows, :] = (g * a + (1.0 - g) * bacc[c // TPB][off:off + _T]).astype(_BF)

        main = [(i, g) for i in range(NQ) for g in range(H // 4)]
        f0, f1, f2, f3 = 0.02, 0.2, 0.85, 0.92
        stage1 = [(dft_k, j) for j in range(NC)] + [(dft_u, j) for j in range(NC)]
        stage2 = [(fg, a) for fg in range(_T // 8) for a in range(NC // 4)]
        side = [(f0 + (f1 - f0) * n / len(stage1), f, a) for n, (f, a) in enumerate(stage1)]
        side += [(f1 + (f2 - f1) * n / len(stage2), mac, a) for n, a in enumerate(stage2)]
        side += [(f2 + (f3 - f2) * c / NC, idft, c) for c in range(NC)]
        side += [(max(f2 + (f3 - f2) * (c + 0.5) / NC, (c // TPB + 1) / NQ), combine, c)
                 for c in range(NC)]
        side.sort(key=lambda t: t[0])
        new_step()
        k = 0
        for n, (i, g) in enumerate(main):
            while k < len(side) and side[k][0] <= n / len(main) + 1e-9:
                side[k][1](side[k][2])
                k += 1
            out_proj(i, g)
        for _, f, a in side[k:]:
            f(a)
        out_copy(cb).start()
        return carry

    lax.fori_loop(0, NB, col_body, 0)
    for cb in range(NB):
        out_copy(cb).wait()


@jax.jit
def pallas_gated_mix__ssm_conv_h3__compressed_kv_cla__prompt_kernel(
    A_q: jax.Array,
    A_k: jax.Array,
    A_v: jax.Array,
    A_shift_k: jax.Array,
    A_ssm_k: jax.Array,
    A_ssm_D: jax.Array,
    B_x: jax.Array,
    B_c_kv: jax.Array,
    B_w_q: jax.Array,
    B_w_uk: jax.Array,
    B_w_uv: jax.Array,
    B_w_o: jax.Array,
    gate_w: jax.Array,
):
    del B_x
    B, S, M = A_q.shape
    _, H, D = B_w_q.shape
    DC = B_c_kv.shape[-1]
    assert B == 1 and D == _T and H % 2 == 0 and H >= 6 and S >= 4 * _BQ and S % (2 * _BQ) == 0 and B_c_kv.shape[1] == S
    NP, NC = H // 2, S // _T

    def body(*refs):
        _kernel(*refs, S=S, M=M, H=H, D=D)

    hbm = pl.BlockSpec(memory_space=pl.ANY)
    scratch = [
        pltpu.VMEM((S, M), _BF),
        pltpu.VMEM((S, DC), _BF),
        pltpu.VMEM((NP, M, D), jnp.uint32),
        pltpu.VMEM((NP, DC, D), jnp.uint32),
        pltpu.VMEM((NP, DC, D), jnp.uint32),
        pltpu.VMEM((H, D, M + _T), _BF),
        pltpu.VMEM((S, M), _BF),
        pltpu.VMEM((S, M), _BF),
        pltpu.VMEM((M, S), _BF),
        pltpu.VMEM((H, S, D), _BF),
    ] + [
        pltpu.VMEM((M, D), _BF),
        pltpu.VMEM((DC, 2 * D), _BF),
    ] * 2 + [pltpu.VMEM((S, D), _BF)] * 6 + [
        pltpu.VMEM((S, _T), _F32),
        pltpu.VMEM((S + 8, _T), _F32),
        pltpu.VMEM((3 * 2 * NC * _SPEC_STRIDE, _T), _F32),
        pltpu.VMEM((M // _T, S, _T), _BF),
        pltpu.VMEM((A_shift_k.shape[1], M), _BF),
        pltpu.VMEM((M // _T, _T), _BF),
        pltpu.VMEM((M // _T, _T), _BF),
        pltpu.VMEM(_DFT_NP.shape, _BF),
        pltpu.VMEM((M // _T, _T), _F32),
        pltpu.SMEM((1 + (_T // 8) * (NC // 4) + NC,), jnp.int32),
        pltpu.SemaphoreType.DMA((6,)),
        pltpu.SemaphoreType.DMA((S // (2 * _BQ),)),
        pltpu.SemaphoreType.DMA((S // _BQ,)),
    ]
    out = pl.pallas_call(
        body,
        out_shape=jax.ShapeDtypeStruct((S, M), _BF),
        in_specs=[hbm] * 13,
        out_specs=hbm,
        scratch_shapes=scratch,
        compiler_params=pltpu.CompilerParams(vmem_limit_bytes=112 * 2 ** 20),
    )(
        A_q.reshape(S, M), A_k.reshape(S, M), A_v.reshape(S, M), A_shift_k.T, A_ssm_k,
        A_ssm_D.reshape(M // _T, _T), B_c_kv.reshape(S, DC), B_w_q, B_w_uk, B_w_uv, B_w_o,
        gate_w.reshape(M // _T, _T), jnp.asarray(_DFT_NP, _BF),
    )
    return out.reshape(B, S, M)
```

```python
import numpy as np
import jax
import jax.numpy as jnp
from jax import lax
import jax.experimental.pallas as pl
import jax.experimental.pallas.tpu as pltpu

_BF = jnp.bfloat16
_F32 = jnp.float32
_NT = (((1,), (1,)), ((), ()))
_T = 128
_BQ = 256
_SPEC_STRIDE = _T + 8
_NEG = -1e30
_LOG2E = 1.4426950408889634


def _dft_tables(c):
    f = np.concatenate([np.arange(0, c, 2), np.arange(1, c, 2)]).astype(np.float64)
    w = np.pi * (f + 0.5) / c
    b = np.arange(c, dtype=np.float64)
    n = np.arange(c // 2, dtype=np.float64) + 0.5

    def forward(origin):
        ang = w[:, None] * (b[None, :] - origin)
        return np.concatenate([np.cos(ang), -np.sin(ang)], axis=0)

    inverse = np.concatenate([np.cos(n[:, None] * w[None, :]),
                              np.sin(n[:, None] * w[None, :])], axis=0) / c
    return np.concatenate([forward(0.0), forward((c - 1) / 2), inverse]).astype(_BF)


_DFT_NP = _dft_tables(_T)


def _dot(a, b):
    return jnp.dot(a, b, preferred_element_type=_F32)


def _dot_nt(a, b):
    return lax.dot_general(a, b, _NT, preferred_element_type=_F32)


def _unpack_head(w32, odd):
    bits = (w32 & jnp.uint32(0xFFFF0000)) if odd else (w32 << 16)
    return pltpu.bitcast(bits, _F32).astype(_BF)


def _merge(a, b):
    out, ia, ib = [], 0, 0
    while ia < len(a) or ib < len(b):
        if ib >= len(b) or (ia < len(a) and ia * len(b) <= ib * len(a)):
            out.append(a[ia])
            ia += 1
        else:
            out.append(b[ib])
            ib += 1
    return out


def _kernel(x_hbm, k_hbm, v_hbm, shift_hbm, ssmk_hbm, ssmd_hbm, c_hbm, wq_hbm, wuk_hbm,
            wuv_hbm, wo_hbm, gate_hbm, dft_hbm, out_hbm,
            x_v, c_v, wq_v, wuk_v, wuv_v, wo_v, ak_v, av_v, sk_v, ctx_v,
            wq0, wkv0, wq1, wkv1, q0, k0, v0, q1, k1, v1, g_v, kf32, spec_v, o_v,
            shift_v, ssmd_v, gate_v, dft_v, ssmd_f, zero_s,
            sem, sem_c, sem_x, *, S, M, H, D):
    NP = H // 2
    NQ = S // _BQ
    TPB = _BQ // _T
    qscale = float(D ** -0.5 * _LOG2E)

    def w_copies(p, sems):
        return [pltpu.make_async_copy(src.bitcast(jnp.uint32).at[:, p, :], dst.at[p], sem.at[n])
                for n, (src, dst) in zip(sems, ((wuk_hbm, wuk_v), (wuv_hbm, wuv_v),
                                                (wq_hbm, wq_v)))]

    cp_gate = pltpu.make_async_copy(gate_hbm, gate_v, sem.at[1])
    cp_w1 = w_copies(1, (2, 2, 2))
    cp_w = [cp for n in range(2, NP) for cp in w_copies(n, (3, 3, 3))]
    cp_late = [pltpu.make_async_copy(src, dst, sem.at[4]) for src, dst in (
        (wo_hbm, wo_v.at[:, :, pl.ds(0, M)]), (k_hbm, ak_v), (v_hbm, av_v), (ssmk_hbm, sk_v),
        (shift_hbm, shift_v), (ssmd_hbm, ssmd_v), (dft_hbm, dft_v))]

    def aligned(n, size):
        return pl.ds(n * size if isinstance(n, int) else pl.multiple_of(n * size, size), size)

    def c_copy(n):
        rows = aligned(n, 2 * _BQ)
        return pltpu.make_async_copy(c_hbm.at[rows], c_v.at[rows], sem_c.at[n])

    def x_copy(n):
        rows = aligned(n, _BQ)
        return pltpu.make_async_copy(x_hbm.at[rows], x_v.at[rows], sem_x.at[n])

    def out_copy(cb, part):
        rows = pl.ds(0, S - _BQ) if part == 0 else pl.ds(S - _BQ, _BQ)
        return pltpu.make_async_copy(o_v.at[cb, rows], out_hbm.at[rows, aligned(cb, _T)],
                                     sem.at[5])

    tri = (lax.broadcasted_iota(jnp.int32, (_T, _T), 1)
           <= lax.broadcasted_iota(jnp.int32, (_T, _T), 0))
    bufs = ((q0, k0, v0, wq0, wkv0), (q1, k1, v1, wq1, wkv1))

    def prep_kv(p, odd):
        wkv_b = bufs[odd][4]
        wkv_b[:, 0:D] = _unpack_head(wuk_v[p], odd)
        wkv_b[:, D:2 * D] = _unpack_head(wuv_v[p], odd)

    def prep_q(p, odd):
        bufs[odd][3][...] = _unpack_head(wq_v[p], odd)

    def prep(p, odd):
        prep_kv(p, odd)
        prep_q(p, odd)

    def proj_q(r, odd):
        rows = aligned(r, _BQ)
        q = _dot(x_v[rows, :], bufs[odd][3][...]) * qscale
        bufs[odd][0][rows, :] = q.astype(_BF)

    def proj_k(r, odd):
        rows = aligned(r, _BQ)
        bufs[odd][1][rows, :] = _dot(c_v[rows, :], bufs[odd][4][:, 0:D]).astype(_BF)

    def proj_v(r, odd):
        rows = aligned(r, _BQ)
        bufs[odd][2][rows, :] = _dot(c_v[rows, :], bufs[odd][4][:, D:2 * D]).astype(_BF)

    def first_row(i, j):
        return max(0, j - TPB * i) * _T

    def accum(old, new, lo, op):
        if old is None:
            return new
        if lo == 0:
            return op(old, new)
        return jnp.concatenate([old[:lo], op(old[lo:], new)], axis=0)

    def head(h, odd, project_next):
        q_b, k_b, v_b, _, _ = bufs[odd]
        st = {}

        def qk(i, js):
            s = st.setdefault(i, dict(t={}, m=None, l=None, acc=None))
            q = q_b[pl.ds(i * _BQ, _BQ), :]
            for j in js:
                lo = first_row(i, j)
                t = _dot_nt(q[lo:], k_b[pl.ds(j * _T, _T), :])
                if j >= TPB * i:
                    top = jnp.where(tri, t[0:_T], _NEG)
                    t = top if t.shape[0] == _T else jnp.concatenate([top, t[_T:]], axis=0)
                s["t"][j] = t
                s["m"] = accum(s["m"], t, lo, jnp.maximum)
            if js[-1] == TPB * (i + 1) - 1:
                s["m"] = jnp.broadcast_to(jnp.max(s["m"], axis=1, keepdims=True), (_BQ, _T))

        def pv(i, js):
            s = st[i]
            for j in js:
                lo = first_row(i, j)
                p = jnp.exp2(s["t"][j] - s["m"][lo:]).astype(_BF)
                p32 = p.astype(_F32)
                o = _dot(p, v_b[pl.ds(j * _T, _T), :])
                s["l"] = accum(s["l"], p32, lo, jnp.add)
                s["acc"] = accum(s["acc"], o, lo, jnp.add)
            if js[-1] == TPB * (i + 1) - 1:
                l = jnp.broadcast_to(jnp.sum(s["l"], axis=1, keepdims=True), (_BQ, _T))
                r = pltpu.reciprocal(l, approx=True)
                r = r * (2.0 - l * r)
                ctx_v[h, pl.ds(i * _BQ, _BQ), :] = (s["acc"] * r).astype(_BF)

        def groups(fn, i, size):
            n = TPB * (i + 1)
            return [(fn, i, list(range(a, min(a + size, n)))) for a in range(0, n, size)]

        order = list(range(NQ - 1, -1, -1))
        if NQ >= 4:
            order[2], order[3] = order[3], order[2]
        att = groups(qk, order[0], 5)
        for n, i in enumerate(order):
            att += _merge(groups(qk, order[n + 1], 5) if n + 1 < NQ else [], groups(pv, i, 6))
        cost = [sum(_BQ - first_row(i, j) for j in js) * (1.5 if fn is qk else 1.0)
                for fn, i, js in att]

        side = [(f, r, c) for f, c in ((proj_q, 8), (proj_k, 4), (proj_v, 4))
                for r in range(NQ)] if project_next else []
        lead, tail = side[:1], side[len(side) - 3:]
        side = side[1:len(side) - 3]
        budget = sum(c for _, _, c in side)
        for f, r, _ in lead:
            f(r, 1 - odd)
        done = spent = 0
        for (fn, i, js), c in zip(att, cost):
            fn(i, js)
            done += c
            while side and spent + 0.8 * side[0][2] <= budget * (done / sum(cost)):
                f, r, c2 = side.pop(0)
                f(r, 1 - odd)
                spent += c2
        for f, r, _ in side + tail:
            f(r, 1 - odd)

    def prologue():
        cp_uk, cp_uv, cp_q = w_copies(0, (0, 0, 1))

        def clear(i, carry):
            zero_s[i] = 0
            return carry

        def kv_body(n, carry):
            c_copy(n).wait()
            x_copy(2 * n).start()
            x_copy(2 * n + 1).start()
            for r in (2 * n, 2 * n + 1):
                proj_k(r, 0)
                proj_v(r, 0)
            return carry

        for cp in (cp_uk, cp_uv, c_copy(0), c_copy(1)):
            cp.start()
        lax.fori_loop(0, zero_s.shape[0], clear, 0)
        cp_uk.wait()
        cp_uv.wait()
        for cp in [c_copy(n) for n in range(2, NQ // 2)] + [cp_q, cp_gate]:
            cp.start()
        prep_kv(0, 0)
        lax.fori_loop(0, NQ // 2, kv_body, 0)
        cp_q.wait()
        cp_gate.wait()
        prep_q(0, 0)
        prep(0, 1)
        gw = gate_v[...].astype(_F32)
        waits = [0] + list(range(3, NQ, 2)) + [NQ]
        for lo, hi in zip(waits[:-1], waits[1:]):
            for r in range(lo, hi):
                x_copy(r).wait()
            if lo == waits[1]:
                for cp in cp_w1:
                    cp.start()
            for r in range(lo, hi):
                proj_q(r, 0)
                rows = pl.ds(r * _BQ, _BQ)
                z = None
                for n in range(M // _T):
                    t = x_v[rows, pl.ds(n * _T, _T)].astype(_F32) * gw[n:n + 1, :]
                    z = t if z is None else z + t
                g = lax.logistic(jnp.sum(z, axis=1, keepdims=True))
                g_v[rows, :] = jnp.broadcast_to(g, (_BQ, _T))
        for cp in cp_w1:
            cp.wait()

    def pair_body(p, carry):
        @pl.when(p == 0)
        def _():
            for cp in cp_w:
                cp.start()

        @pl.when(p == 1)
        def _():
            for cp in cp_w:
                cp.wait()
            for cp in cp_late:
                cp.start()

        prep(p + 1, 0)
        head(2 * p, 0, True)
        prep(p + 1, 1)
        head(2 * p + 1, 1, True)
        return carry

    prologue()
    lax.fori_loop(0, NP - 1, pair_body, 0)
    head(H - 2, 0, True)
    head(H - 1, 1, False)

    for cp in cp_late:
        cp.wait()
    ssmd_f[...] = ssmd_v[...].astype(_F32)
    NC = S // _T
    NB = M // _T
    HF = _T // 2

    kf32[0:8, :] = jnp.zeros((8, _T), _F32)

    def col_body(cb, carry):
        cols = aligned(cb, _T)
        sh = shift_v[:, cols].astype(_F32)
        dvec = ssmd_f[pl.ds(cb, 1), :]
        flip = 7 - lax.broadcasted_iota(jnp.int32, (8, _T), 0)
        bacc, kvs, yt, state = {}, {}, {}, {"n": 0}

        def new_step():
            state["z"] = pl.multiple_of(zero_s[state["n"]] * 8, 8)
            state["n"] += 1

        def spec_rows(kind, c, part, lo=0, n=_T):
            return pl.ds(state["z"] + ((kind * NC + c) * 2 + part) * _SPEC_STRIDE + lo, n)

        def spec_load(kind, c, fg):
            return tuple(spec_v[spec_rows(kind, c, part, fg * 8, 8), :] for part in range(2))

        def spec_store(kind, c, val):
            for part in range(2):
                spec_v[spec_rows(kind, c, part), :] = val[part * _T:(part + 1) * _T]

        def out_proj(i, g):
            rows = pl.ds(i * _BQ, _BQ)
            for h in range(4 * g, 4 * g + 4):
                t = _dot(ctx_v[h, rows, :], wo_v[h, :, cols])
                bacc[i] = t if h == 0 else bacc[i] + t

        def dft_u(j):
            kf32[pl.ds(8 + j * _T, _T), :] = ak_v[pl.ds(j * _T, _T), cols].astype(_F32)
            acc = kf32[pl.ds(8 + j * _T, _T), :] * sh[0:1, :]
            for s in range(1, sh.shape[0]):
                acc = acc + kf32[pl.ds(8 + j * _T - s, _T), :] * sh[s:s + 1, :]
            kv = (acc * av_v[pl.ds(j * _T, _T), cols].astype(_F32)).astype(_BF)
            kvs[j] = kv
            spec_store(0, j, _dot(dft_v[0:2 * _T, :], kv))

        def dft_k(j):
            s = _dot_nt(dft_v[2 * _T:4 * _T, :], sk_v[cols, pl.ds(j * _T, _T)])
            if j == 0:
                spec_store(1, j, s)
            else:
                p = state["prev"]
                spec_store(1, j, jnp.concatenate(
                    [s[0:HF] - p[_T:_T + HF], s[HF:_T] + p[_T + HF:],
                     s[_T:_T + HF] + p[0:HF], s[_T + HF:] - p[HF:_T]], axis=0))
            state["prev"] = s

        def mac(arg):
            fg, a = arg
            new_step()
            kc, y = {}, {}
            for j in range(4 * a + 4):
                ur, ui = spec_load(0, j, fg)
                for i in range(max(4 * a, j), 4 * a + 4):
                    if i - j not in kc:
                        kc[i - j] = spec_load(1, i - j, fg)
                    kr, ki = kc[i - j]
                    tr, ti = kr * ur - ki * ui, kr * ui + ki * ur
                    y[i] = (tr, ti) if i not in y else (y[i][0] + tr, y[i][1] + ti)
            for i, parts in y.items():
                for part in range(2):
                    spec_v[spec_rows(2, i, part, fg * 8, 8), :] = parts[part]

        def idft(c):
            new_step()
            even, odd = [_dot(dft_v[4 * _T + part * HF:4 * _T + (part + 1) * HF, :],
                              spec_v[spec_rows(2, c, part), :].astype(_BF))
                         for part in range(2)]
            mirrored = even + odd
            yt[c] = jnp.concatenate(
                [jnp.take_along_axis(mirrored[lo:lo + 8], flip, axis=0)
                 for lo in range(HF - 8, -8, -8)] + [even - odd], axis=0)

        def combine(c):
            rows = pl.ds(c * _T, _T)
            off = (c % TPB) * _T
            y = yt[c] + kvs[c].astype(_F32) * dvec
            a = x_v[rows, cols].astype(_F32) * y
            g = g_v[rows, :]
            o_v[cb, rows, :] = (g * a + (1.0 - g) * bacc[c // TPB][off:off + _T]).astype(_BF)
            if c + 1 in (NC - TPB, NC):
                out_copy(cb, int(c + 1 == NC)).start()

        main = [(i, g) for i in range(NQ) for g in range(H // 4)]
        f0, f1, f2, f3 = 0.02, 0.2, 0.85, 0.92
        stage1 = [(dft_k, j) for j in range(NC)] + [(dft_u, j) for j in range(NC)]
        stage2 = [(fg, a) for fg in range(_T // 8) for a in range(NC // 4)]
        side = [(f0 + (f1 - f0) * n / len(stage1), f, a) for n, (f, a) in enumerate(stage1)]
        side += [(f1 + (f2 - f1) * n / len(stage2), mac, a) for n, a in enumerate(stage2)]
        side += [(f2 + (f3 - f2) * c / NC, idft, c) for c in range(NC)]
        side += [(max(f2 + (f3 - f2) * (c + 0.5) / NC, (c // TPB + 1) / NQ), combine, c)
                 for c in range(NC)]
        side.sort(key=lambda t: t[0])
        new_step()
        k = 0
        for n, (i, g) in enumerate(main):
            while k < len(side) and side[k][0] <= n / len(main) + 1e-9:
                side[k][1](side[k][2])
                k += 1
            out_proj(i, g)
        for _, f, a in side[k:]:
            f(a)
        return carry

    lax.fori_loop(0, NB, col_body, 0)
    for cb in range(NB):
        out_copy(cb, 0).wait()
        out_copy(cb, 1).wait()


@jax.jit
def pallas_gated_mix__ssm_conv_h3__compressed_kv_cla__prompt_kernel(
    A_q: jax.Array,
    A_k: jax.Array,
    A_v: jax.Array,
    A_shift_k: jax.Array,
    A_ssm_k: jax.Array,
    A_ssm_D: jax.Array,
    B_x: jax.Array,
    B_c_kv: jax.Array,
    B_w_q: jax.Array,
    B_w_uk: jax.Array,
    B_w_uv: jax.Array,
    B_w_o: jax.Array,
    gate_w: jax.Array,
):
    del B_x
    B, S, M = A_q.shape
    _, H, D = B_w_q.shape
    DC = B_c_kv.shape[-1]
    assert B == 1 and D == _T and H % 2 == 0 and H >= 6 and S >= 4 * _BQ and S % (2 * _BQ) == 0 and B_c_kv.shape[1] == S
    NP, NC = H // 2, S // _T

    def body(*refs):
        _kernel(*refs, S=S, M=M, H=H, D=D)

    hbm = pl.BlockSpec(memory_space=pl.ANY)
    scratch = [
        pltpu.VMEM((S, M), _BF),
        pltpu.VMEM((S, DC), _BF),
        pltpu.VMEM((NP, M, D), jnp.uint32),
        pltpu.VMEM((NP, DC, D), jnp.uint32),
        pltpu.VMEM((NP, DC, D), jnp.uint32),
        pltpu.VMEM((H, D, M + _T), _BF),
        pltpu.VMEM((S, M), _BF),
        pltpu.VMEM((S, M), _BF),
        pltpu.VMEM((M, S), _BF),
        pltpu.VMEM((H, S, D), _BF),
    ] + [
        pltpu.VMEM((M, D), _BF),
        pltpu.VMEM((DC, 2 * D), _BF),
    ] * 2 + [pltpu.VMEM((S, D), _BF)] * 6 + [
        pltpu.VMEM((S, _T), _F32),
        pltpu.VMEM((S + 8, _T), _F32),
        pltpu.VMEM((3 * 2 * NC * _SPEC_STRIDE, _T), _F32),
        pltpu.VMEM((M // _T, S, _T), _BF),
        pltpu.VMEM((A_shift_k.shape[1], M), _BF),
        pltpu.VMEM((M // _T, _T), _BF),
        pltpu.VMEM((M // _T, _T), _BF),
        pltpu.VMEM(_DFT_NP.shape, _BF),
        pltpu.VMEM((M // _T, _T), _F32),
        pltpu.SMEM((1 + (_T // 8) * (NC // 4) + NC,), jnp.int32),
        pltpu.SemaphoreType.DMA((6,)),
        pltpu.SemaphoreType.DMA((S // (2 * _BQ),)),
        pltpu.SemaphoreType.DMA((S // _BQ,)),
    ]
    out = pl.pallas_call(
        body,
        out_shape=jax.ShapeDtypeStruct((S, M), _BF),
        in_specs=[hbm] * 13,
        out_specs=hbm,
        scratch_shapes=scratch,
        compiler_params=pltpu.CompilerParams(vmem_limit_bytes=112 * 2 ** 20),
    )(
        A_q.reshape(S, M), A_k.reshape(S, M), A_v.reshape(S, M), A_shift_k.T, A_ssm_k,
        A_ssm_D.reshape(M // _T, _T), B_c_kv.reshape(S, DC), B_w_q, B_w_uk, B_w_uv, B_w_o,
        gate_w.reshape(M // _T, _T), _DFT_NP,
    )
    return out.reshape(B, S, M)
```

```python
import numpy as np
import jax
import jax.numpy as jnp
from jax import lax
import jax.experimental.pallas as pl
import jax.experimental.pallas.tpu as pltpu

_BF = jnp.bfloat16
_F32 = jnp.float32
_NT = (((1,), (1,)), ((), ()))
_T = 128
_BQ = 256
_SPEC_STRIDE = _T + 8
_NEG = -1e30
_LOG2E = 1.4426950408889634


def _dft_tables(c):
    f = np.concatenate([np.arange(0, c, 2), np.arange(1, c, 2)]).astype(np.float64)
    w = np.pi * (f + 0.5) / c
    b = np.arange(c, dtype=np.float64)
    n = np.arange(c // 2, dtype=np.float64) + 0.5

    def forward(origin):
        ang = w[:, None] * (b[None, :] - origin)
        return np.concatenate([np.cos(ang), -np.sin(ang)], axis=0)

    inverse = np.concatenate([np.cos(n[:, None] * w[None, :]),
                              np.sin(n[:, None] * w[None, :])], axis=0) / c
    return np.concatenate([forward(0.0), forward((c - 1) / 2), inverse]).astype(_BF)


_DFT_NP = _dft_tables(_T)


def _dot(a, b):
    return jnp.dot(a, b, preferred_element_type=_F32)


def _dot_nt(a, b):
    return lax.dot_general(a, b, _NT, preferred_element_type=_F32)


def _unpack_head(w32, odd):
    bits = (w32 & jnp.uint32(0xFFFF0000)) if odd else (w32 << 16)
    return pltpu.bitcast(bits, _F32).astype(_BF)


def _merge(a, b):
    out, ia, ib = [], 0, 0
    while ia < len(a) or ib < len(b):
        if ib >= len(b) or (ia < len(a) and ia * len(b) <= ib * len(a)):
            out.append(a[ia])
            ia += 1
        else:
            out.append(b[ib])
            ib += 1
    return out


def _kernel(x_hbm, k_hbm, v_hbm, shift_hbm, ssmk_hbm, ssmd_hbm, c_hbm, wq_hbm, wuk_hbm,
            wuv_hbm, wo_hbm, gate_hbm, dft_hbm, out_hbm,
            x_v, c_v, wq_v, wuk_v, wuv_v, wo_v, ak_v, av_v, sk_v, ctx_v,
            wq0, wkv0, wq1, wkv1, q0, k0, v0, q1, k1, v1, g_v, kf32, spec_v, o_v,
            shift_v, ssmd_v, gate_v, dft_v, ssmd_f, zero_s,
            sem, sem_c, sem_x, *, S, M, H, D):
    NP = H // 2
    NQ = S // _BQ
    TPB = _BQ // _T
    qscale = float(D ** -0.5 * _LOG2E)

    def w_copies(p, sems):
        return [pltpu.make_async_copy(src.bitcast(jnp.uint32).at[:, p, :], dst.at[p], sem.at[n])
                for n, (src, dst) in zip(sems, ((wuk_hbm, wuk_v), (wuv_hbm, wuv_v),
                                                (wq_hbm, wq_v)))]

    cp_gate = pltpu.make_async_copy(gate_hbm, gate_v, sem.at[1])
    cp_w1 = w_copies(1, (2, 2, 2))
    cp_w = [cp for n in range(2, NP) for cp in w_copies(n, (3, 3, 3))]
    cp_late = [pltpu.make_async_copy(src, dst, sem.at[4]) for src, dst in (
        (wo_hbm, wo_v.at[:, :, pl.ds(0, M)]), (k_hbm, ak_v), (v_hbm, av_v), (ssmk_hbm, sk_v),
        (shift_hbm, shift_v), (ssmd_hbm, ssmd_v), (dft_hbm, dft_v))]

    def aligned(n, size):
        return pl.ds(n * size if isinstance(n, int) else pl.multiple_of(n * size, size), size)

    def c_copy(n):
        rows = aligned(n, 2 * _BQ)
        return pltpu.make_async_copy(c_hbm.at[rows], c_v.at[rows], sem_c.at[n])

    def x_copy(n):
        rows = aligned(n, _BQ)
        return pltpu.make_async_copy(x_hbm.at[rows], x_v.at[rows], sem_x.at[n])

    def out_copy(cb, part):
        rows = pl.ds(0, S - _BQ) if part == 0 else pl.ds(S - _BQ, _BQ)
        return pltpu.make_async_copy(o_v.at[cb, rows], out_hbm.at[rows, aligned(cb, _T)],
                                     sem.at[5])

    tri = (lax.broadcasted_iota(jnp.int32, (_T, _T), 1)
           <= lax.broadcasted_iota(jnp.int32, (_T, _T), 0))
    bufs = ((q0, k0, v0, wq0, wkv0), (q1, k1, v1, wq1, wkv1))

    def prep_kv(p, odd):
        wkv_b = bufs[odd][4]
        wkv_b[:, 0:D] = _unpack_head(wuk_v[p], odd)
        wkv_b[:, D:2 * D] = _unpack_head(wuv_v[p], odd)

    def prep_q(p, odd):
        bufs[odd][3][...] = _unpack_head(wq_v[p], odd)

    def prep(p, odd):
        prep_kv(p, odd)
        prep_q(p, odd)

    def proj_q(r, odd):
        rows = aligned(r, _BQ)
        q = _dot(x_v[rows, :], bufs[odd][3][...]) * qscale
        bufs[odd][0][rows, :] = q.astype(_BF)

    def proj_k(r, odd):
        rows = aligned(r, _BQ)
        bufs[odd][1][rows, :] = _dot(c_v[rows, :], bufs[odd][4][:, 0:D]).astype(_BF)

    def proj_v(r, odd):
        rows = aligned(r, _BQ)
        bufs[odd][2][rows, :] = _dot(c_v[rows, :], bufs[odd][4][:, D:2 * D]).astype(_BF)

    def first_row(i, j):
        return max(0, j - TPB * i) * _T

    def accum(old, new, lo, op):
        if old is None:
            return new
        if lo == 0:
            return op(old, new)
        return jnp.concatenate([old[:lo], op(old[lo:], new)], axis=0)

    def head(h, odd, project_next):
        q_b, k_b, v_b, _, _ = bufs[odd]
        st = {}

        def qk(i, js):
            s = st.setdefault(i, dict(t={}, m=None, l=None, acc=None))
            q = q_b[pl.ds(i * _BQ, _BQ), :]
            for j in js:
                lo = first_row(i, j)
                t = _dot_nt(q[lo:], k_b[pl.ds(j * _T, _T), :])
                if j >= TPB * i:
                    top = jnp.where(tri, t[0:_T], _NEG)
                    t = top if t.shape[0] == _T else jnp.concatenate([top, t[_T:]], axis=0)
                s["t"][j] = t
                s["m"] = accum(s["m"], t, lo, jnp.maximum)
            if js[-1] == TPB * (i + 1) - 1:
                s["m"] = jnp.broadcast_to(jnp.max(s["m"], axis=1, keepdims=True), (_BQ, _T))

        def pv(i, js):
            s = st[i]
            for j in js:
                lo = first_row(i, j)
                p = jnp.exp2(s["t"][j] - s["m"][lo:]).astype(_BF)
                p32 = p.astype(_F32)
                o = _dot(p, v_b[pl.ds(j * _T, _T), :])
                s["l"] = accum(s["l"], p32, lo, jnp.add)
                s["acc"] = accum(s["acc"], o, lo, jnp.add)
            if js[-1] == TPB * (i + 1) - 1:
                l = jnp.broadcast_to(jnp.sum(s["l"], axis=1, keepdims=True), (_BQ, _T))
                r = pltpu.reciprocal(l, approx=True)
                r = r * (2.0 - l * r)
                ctx_v[h, pl.ds(i * _BQ, _BQ), :] = (s["acc"] * r).astype(_BF)

        def groups(fn, i, size):
            n = TPB * (i + 1)
            return [(fn, i, list(range(a, min(a + size, n)))) for a in range(0, n, size)]

        order = list(range(NQ - 1, -1, -1))
        if NQ >= 4:
            order[2], order[3] = order[3], order[2]
        att = groups(qk, order[0], 5)
        for n, i in enumerate(order):
            att += _merge(groups(qk, order[n + 1], 5) if n + 1 < NQ else [], groups(pv, i, 6))
        cost = [sum(_BQ - first_row(i, j) for j in js) * (1.5 if fn is qk else 1.0)
                for fn, i, js in att]

        side = [(f, r, c) for f, c in ((proj_q, 8), (proj_k, 4), (proj_v, 4))
                for r in range(NQ)] if project_next else []
        lead, tail = side[:1], side[len(side) - 3:]
        side = side[1:len(side) - 3]
        budget = sum(c for _, _, c in side)
        for f, r, _ in lead:
            f(r, 1 - odd)
        done = spent = 0
        for (fn, i, js), c in zip(att, cost):
            fn(i, js)
            done += c
            while side and spent + 0.8 * side[0][2] <= budget * (done / sum(cost)):
                f, r, c2 = side.pop(0)
                f(r, 1 - odd)
                spent += c2
        for f, r, _ in side + tail:
            f(r, 1 - odd)

    def prologue():
        cp_uk, cp_uv, cp_q = w_copies(0, (0, 0, 1))

        def clear(i, carry):
            zero_s[i] = 0
            return carry

        def kv_body(n, carry):
            c_copy(n).wait()
            x_copy(2 * n).start()
            x_copy(2 * n + 1).start()
            for r in (2 * n, 2 * n + 1):
                proj_k(r, 0)
                proj_v(r, 0)
            return carry

        for cp in (cp_uk, cp_uv, c_copy(0), c_copy(1)):
            cp.start()
        lax.fori_loop(0, zero_s.shape[0], clear, 0)
        cp_uk.wait()
        cp_uv.wait()
        for cp in [c_copy(n) for n in range(2, NQ // 2)] + [cp_q, cp_gate]:
            cp.start()
        prep_kv(0, 0)
        lax.fori_loop(0, NQ // 2, kv_body, 0)
        cp_q.wait()
        cp_gate.wait()
        prep_q(0, 0)
        prep(0, 1)
        gw = gate_v[...].astype(_F32)
        waits = [0] + list(range(3, NQ, 2)) + [NQ]
        for lo, hi in zip(waits[:-1], waits[1:]):
            for r in range(lo, hi):
                x_copy(r).wait()
            if lo == waits[1]:
                for cp in cp_w1:
                    cp.start()
            for r in range(lo, hi):
                proj_q(r, 0)
                rows = pl.ds(r * _BQ, _BQ)
                z = None
                for n in range(M // _T):
                    t = x_v[rows, pl.ds(n * _T, _T)].astype(_F32) * gw[n:n + 1, :]
                    z = t if z is None else z + t
                g = lax.logistic(jnp.sum(z, axis=1, keepdims=True))
                g_v[rows, :] = jnp.broadcast_to(g, (_BQ, _T))
        for cp in cp_w1:
            cp.wait()
        for cp in cp_w:
            cp.start()

    def pair_body(p, carry):
        @pl.when(p == 1)
        def _():
            for w in (wuk_v, wuv_v, wq_v):
                rest = w.at[pl.ds(2, NP - 2)]
                pltpu.make_async_copy(rest, rest, sem.at[3]).wait()
            for cp in cp_late:
                cp.start()

        prep(p + 1, 0)
        head(2 * p, 0, True)
        prep(p + 1, 1)
        head(2 * p + 1, 1, True)
        return carry

    prologue()
    lax.fori_loop(0, NP - 1, pair_body, 0)
    head(H - 2, 0, True)
    head(H - 1, 1, False)

    for cp in cp_late:
        cp.wait()
    ssmd_f[...] = ssmd_v[...].astype(_F32)
    NC = S // _T
    NB = M // _T
    HF = _T // 2

    kf32[0:8, :] = jnp.zeros((8, _T), _F32)

    def col_body(cb, carry):
        cols = aligned(cb, _T)
        sh = shift_v[:, cols].astype(_F32)
        dvec = ssmd_f[pl.ds(cb, 1), :]
        flip = 7 - lax.broadcasted_iota(jnp.int32, (8, _T), 0)
        bacc, kvs, yt, state = {}, {}, {}, {"n": 0}

        def new_step():
            state["z"] = pl.multiple_of(zero_s[state["n"]] * 8, 8)
            state["n"] += 1

        def spec_rows(kind, c, part, lo=0, n=_T):
            return pl.ds(state["z"] + ((kind * NC + c) * 2 + part) * _SPEC_STRIDE + lo, n)

        def spec_load(kind, c, fg):
            return tuple(spec_v[spec_rows(kind, c, part, fg * 8, 8), :] for part in range(2))

        def spec_store(kind, c, val):
            for part in range(2):
                spec_v[spec_rows(kind, c, part), :] = val[part * _T:(part + 1) * _T]

        def out_proj(i, g):
            rows = pl.ds(i * _BQ, _BQ)
            for h in range(4 * g, 4 * g + 4):
                t = _dot(ctx_v[h, rows, :], wo_v[h, :, cols])
                bacc[i] = t if h == 0 else bacc[i] + t

        def dft_u(j):
            kf32[pl.ds(8 + j * _T, _T), :] = ak_v[pl.ds(j * _T, _T), cols].astype(_F32)
            acc = kf32[pl.ds(8 + j * _T, _T), :] * sh[0:1, :]
            for s in range(1, sh.shape[0]):
                acc = acc + kf32[pl.ds(8 + j * _T - s, _T), :] * sh[s:s + 1, :]
            kv = (acc * av_v[pl.ds(j * _T, _T), cols].astype(_F32)).astype(_BF)
            kvs[j] = kv
            spec_store(0, j, _dot(dft_v[0:2 * _T, :], kv))

        def dft_k(j):
            s = _dot_nt(dft_v[2 * _T:4 * _T, :], sk_v[cols, pl.ds(j * _T, _T)])
            if j == 0:
                spec_store(1, j, s)
            else:
                p = state["prev"]
                spec_store(1, j, jnp.concatenate(
                    [s[0:HF] - p[_T:_T + HF], s[HF:_T] + p[_T + HF:],
                     s[_T:_T + HF] + p[0:HF], s[_T + HF:] - p[HF:_T]], axis=0))
            state["prev"] = s

        def mac(arg):
            fg, a = arg
            new_step()
            kc, y = {}, {}
            for j in range(4 * a + 4):
                ur, ui = spec_load(0, j, fg)
                for i in range(max(4 * a, j), 4 * a + 4):
                    if i - j not in kc:
                        kc[i - j] = spec_load(1, i - j, fg)
                    kr, ki = kc[i - j]
                    tr, ti = kr * ur - ki * ui, kr * ui + ki * ur
                    y[i] = (tr, ti) if i not in y else (y[i][0] + tr, y[i][1] + ti)
            for i, parts in y.items():
                for part in range(2):
                    spec_v[spec_rows(2, i, part, fg * 8, 8), :] = parts[part]

        def idft(c):
            new_step()
            even, odd = [_dot(dft_v[4 * _T + part * HF:4 * _T + (part + 1) * HF, :],
                              spec_v[spec_rows(2, c, part), :].astype(_BF))
                         for part in range(2)]
            mirrored = even + odd
            yt[c] = jnp.concatenate(
                [jnp.take_along_axis(mirrored[lo:lo + 8], flip, axis=0)
                 for lo in range(HF - 8, -8, -8)] + [even - odd], axis=0)

        def combine(c):
            rows = pl.ds(c * _T, _T)
            off = (c % TPB) * _T
            y = yt[c] + kvs[c].astype(_F32) * dvec
            a = x_v[rows, cols].astype(_F32) * y
            g = g_v[rows, :]
            o_v[cb, rows, :] = (g * a + (1.0 - g) * bacc[c // TPB][off:off + _T]).astype(_BF)
            if c + 1 in (NC - TPB, NC):
                out_copy(cb, int(c + 1 == NC)).start()

        main = [(i, g) for i in range(NQ) for g in range(H // 4)]
        f0, f1, f2, f3 = 0.02, 0.2, 0.85, 0.92
        stage1 = [(dft_k, j) for j in range(NC)] + [(dft_u, j) for j in range(NC)]
        stage2 = [(fg, a) for fg in range(_T // 8) for a in range(NC // 4)]
        side = [(f0 + (f1 - f0) * n / len(stage1), f, a) for n, (f, a) in enumerate(stage1)]
        side += [(f1 + (f2 - f1) * n / len(stage2), mac, a) for n, a in enumerate(stage2)]
        side += [(f2 + (f3 - f2) * c / NC, idft, c) for c in range(NC)]
        side += [(max(f2 + (f3 - f2) * (c + 0.5) / NC, (c // TPB + 1) / NQ), combine, c)
                 for c in range(NC)]
        side.sort(key=lambda t: t[0])
        new_step()
        k = 0
        for n, (i, g) in enumerate(main):
            while k < len(side) and side[k][0] <= n / len(main) + 1e-9:
                side[k][1](side[k][2])
                k += 1
            out_proj(i, g)
        for _, f, a in side[k:]:
            f(a)
        return carry

    lax.fori_loop(0, NB, col_body, 0)
    for cb in range(NB):
        out_copy(cb, 0).wait()
        out_copy(cb, 1).wait()


@jax.jit
def pallas_gated_mix__ssm_conv_h3__compressed_kv_cla__prompt_kernel(
    A_q: jax.Array,
    A_k: jax.Array,
    A_v: jax.Array,
    A_shift_k: jax.Array,
    A_ssm_k: jax.Array,
    A_ssm_D: jax.Array,
    B_x: jax.Array,
    B_c_kv: jax.Array,
    B_w_q: jax.Array,
    B_w_uk: jax.Array,
    B_w_uv: jax.Array,
    B_w_o: jax.Array,
    gate_w: jax.Array,
):
    del B_x
    B, S, M = A_q.shape
    _, H, D = B_w_q.shape
    DC = B_c_kv.shape[-1]
    assert B == 1 and D == _T and H % 2 == 0 and H >= 6 and S >= 4 * _BQ and S % (2 * _BQ) == 0 and B_c_kv.shape[1] == S
    NP, NC = H // 2, S // _T

    def body(*refs):
        _kernel(*refs, S=S, M=M, H=H, D=D)

    hbm = pl.BlockSpec(memory_space=pl.ANY)
    scratch = [
        pltpu.VMEM((S, M), _BF),
        pltpu.VMEM((S, DC), _BF),
        pltpu.VMEM((NP, M, D), jnp.uint32),
        pltpu.VMEM((NP, DC, D), jnp.uint32),
        pltpu.VMEM((NP, DC, D), jnp.uint32),
        pltpu.VMEM((H, D, M + _T), _BF),
        pltpu.VMEM((S, M), _BF),
        pltpu.VMEM((S, M), _BF),
        pltpu.VMEM((M, S), _BF),
        pltpu.VMEM((H, S, D), _BF),
    ] + [
        pltpu.VMEM((M, D), _BF),
        pltpu.VMEM((DC, 2 * D), _BF),
    ] * 2 + [pltpu.VMEM((S, D), _BF)] * 6 + [
        pltpu.VMEM((S, _T), _F32),
        pltpu.VMEM((S + 8, _T), _F32),
        pltpu.VMEM((3 * 2 * NC * _SPEC_STRIDE, _T), _F32),
        pltpu.VMEM((M // _T, S, _T), _BF),
        pltpu.VMEM((A_shift_k.shape[1], M), _BF),
        pltpu.VMEM((M // _T, _T), _BF),
        pltpu.VMEM((M // _T, _T), _BF),
        pltpu.VMEM(_DFT_NP.shape, _BF),
        pltpu.VMEM((M // _T, _T), _F32),
        pltpu.SMEM((1 + (_T // 8) * (NC // 4) + NC,), jnp.int32),
        pltpu.SemaphoreType.DMA((6,)),
        pltpu.SemaphoreType.DMA((S // (2 * _BQ),)),
        pltpu.SemaphoreType.DMA((S // _BQ,)),
    ]
    out = pl.pallas_call(
        body,
        out_shape=jax.ShapeDtypeStruct((S, M), _BF),
        in_specs=[hbm] * 13,
        out_specs=hbm,
        scratch_shapes=scratch,
        compiler_params=pltpu.CompilerParams(vmem_limit_bytes=112 * 2 ** 20),
    )(
        A_q.reshape(S, M), A_k.reshape(S, M), A_v.reshape(S, M), A_shift_k.T, A_ssm_k,
        A_ssm_D.reshape(M // _T, _T), B_c_kv.reshape(S, DC), B_w_q, B_w_uk, B_w_uv, B_w_o,
        gate_w.reshape(M // _T, _T), _DFT_NP,
    )
    return out.reshape(B, S, M)
```

```python
import numpy as np
import jax
import jax.numpy as jnp
from jax import lax
import jax.experimental.pallas as pl
import jax.experimental.pallas.tpu as pltpu

_BF = jnp.bfloat16
_F32 = jnp.float32
_NT = (((1,), (1,)), ((), ()))
_T = 128
_BQ = 256
_SPEC_STRIDE = _T + 8
_TAIL = 4
_NEG = -1e30
_LOG2E = 1.4426950408889634


def _dft_tables(c):
    f = np.concatenate([np.arange(0, c, 2), np.arange(1, c, 2)]).astype(np.float64)
    w = np.pi * (f + 0.5) / c
    b = np.arange(c, dtype=np.float64)
    n = np.arange(c // 2, dtype=np.float64) + 0.5

    def forward(origin):
        ang = w[:, None] * (b[None, :] - origin)
        return np.concatenate([np.cos(ang), -np.sin(ang)], axis=0)

    inverse = np.concatenate([np.cos(n[:, None] * w[None, :]),
                              np.sin(n[:, None] * w[None, :])], axis=0) / c
    return np.concatenate([forward(0.0), forward((c - 1) / 2), inverse]).astype(_BF)


_DFT_NP = _dft_tables(_T)


def _dot(a, b):
    return jnp.dot(a, b, preferred_element_type=_F32)


def _dot_nt(a, b):
    return lax.dot_general(a, b, _NT, preferred_element_type=_F32)


def _unpack_head(w32, odd):
    bits = (w32 & jnp.uint32(0xFFFF0000)) if odd else (w32 << 16)
    return pltpu.bitcast(bits, _F32).astype(_BF)


def _stage(ref, first, w):
    for n in range(w.shape[0] // _T):
        ref[first + n] = pltpu.bitcast(w[n * _T:(n + 1) * _T], jnp.uint32)


def _staged(ref, first, count):
    tiles = [pltpu.bitcast(ref[first + n], _BF) for n in range(count)]
    return tiles[0] if count == 1 else jnp.concatenate(tiles, axis=0)


def _merge(a, b):
    out, ia, ib = [], 0, 0
    while ia < len(a) or ib < len(b):
        if ib >= len(b) or (ia < len(a) and ia * len(b) <= ib * len(a)):
            out.append(a[ia])
            ia += 1
        else:
            out.append(b[ib])
            ib += 1
    return out


def _kernel(x_hbm, k_hbm, v_hbm, shift_hbm, ssmk_hbm, ssmd_hbm, c_hbm, wq_hbm, wuk_hbm,
            wuv_hbm, wo_hbm, gate_hbm, dft_hbm, out_hbm,
            x_v, c_v, wq_v, wuk_v, wuv_v, wo_v, ak_v, av_v, sk_v, ctx_v,
            w0, w1, wo_b, q0, k0, v0, q1, k1, v1, g_v, kf32, spec_v, o_v,
            shift_v, ssmd_v, gate_v, dft_v, ssmd_f, zero_s,
            sem, sem_c, sem_x, *, S, M, H, D):
    NP = H // 2
    NQ = S // _BQ
    TPB = _BQ // _T
    qscale = float(D ** -0.5 * _LOG2E)

    def w_copies(p, sems):
        return [pltpu.make_async_copy(src.bitcast(jnp.uint32).at[:, p, :], dst.at[p], sem.at[n])
                for n, (src, dst) in zip(sems, ((wuk_hbm, wuk_v), (wuv_hbm, wuv_v),
                                                (wq_hbm, wq_v)))]

    cp_gate = pltpu.make_async_copy(gate_hbm, gate_v, sem.at[1])
    cp_w1 = w_copies(1, (2, 2, 2))
    cp_w = [cp for n in range(2, NP) for cp in w_copies(n, (3, 3, 3))]
    cp_late = [pltpu.make_async_copy(src, dst, sem.at[4]) for src, dst in (
        (wo_hbm, wo_v.at[:, :, pl.ds(0, M)]), (k_hbm, ak_v), (v_hbm, av_v), (ssmk_hbm, sk_v),
        (shift_hbm, shift_v), (ssmd_hbm, ssmd_v), (dft_hbm, dft_v))]

    def aligned(n, size):
        return pl.ds(n * size if isinstance(n, int) else pl.multiple_of(n * size, size), size)

    def c_copy(n):
        rows = aligned(n, 2 * _BQ)
        return pltpu.make_async_copy(c_hbm.at[rows], c_v.at[rows], sem_c.at[n])

    def x_copy(n):
        rows = aligned(n, _BQ)
        return pltpu.make_async_copy(x_hbm.at[rows], x_v.at[rows], sem_x.at[n])

    def out_copy(cb, part):
        rows = pl.ds(0, S - _BQ) if part == 0 else pl.ds(S - _BQ, _BQ)
        return pltpu.make_async_copy(o_v.at[cb, rows], out_hbm.at[rows, aligned(cb, _T)],
                                     sem.at[5])

    tri = (lax.broadcasted_iota(jnp.int32, (_T, _T), 1)
           <= lax.broadcasted_iota(jnp.int32, (_T, _T), 0))
    bufs = ((q0, k0, v0, w0), (q1, k1, v1, w1))
    NM, NK = M // _T, c_v.shape[1] // _T

    def prep_kv(p, odd):
        _stage(bufs[odd][3], NM, _unpack_head(wuk_v[p], odd))
        _stage(bufs[odd][3], NM + NK, _unpack_head(wuv_v[p], odd))

    def prep_q(p, odd):
        _stage(bufs[odd][3], 0, _unpack_head(wq_v[p], odd))

    def proj_q(r, odd):
        rows = aligned(r, _BQ)
        q = _dot(x_v[rows, :], _staged(bufs[odd][3], 0, NM)) * qscale
        bufs[odd][0][rows, :] = q.astype(_BF)

    def proj_k(r, odd):
        rows = aligned(r, _BQ)
        bufs[odd][1][rows, :] = _dot(c_v[rows, :], _staged(bufs[odd][3], NM, NK)).astype(_BF)

    def proj_v(r, odd):
        rows = aligned(r, _BQ)
        bufs[odd][2][rows, :] = _dot(c_v[rows, :],
                                     _staged(bufs[odd][3], NM + NK, NK)).astype(_BF)

    def first_row(i, j):
        return max(0, j - TPB * i) * _T

    def accum(old, new, lo, op):
        if old is None:
            return new
        if lo == 0:
            return op(old, new)
        return jnp.concatenate([old[:lo], op(old[lo:], new)], axis=0)

    def head(h, odd, project_next):
        q_b, k_b, v_b, _ = bufs[odd]
        st = {}

        def qk(i, js):
            s = st.setdefault(i, dict(t={}, m=None, l=None, acc=None))
            q = q_b[pl.ds(i * _BQ, _BQ), :]
            for j in js:
                lo = first_row(i, j)
                t = _dot_nt(q[lo:], k_b[pl.ds(j * _T, _T), :])
                if j >= TPB * i:
                    top = jnp.where(tri, t[0:_T], _NEG)
                    t = top if t.shape[0] == _T else jnp.concatenate([top, t[_T:]], axis=0)
                s["t"][j] = t
                s["m"] = accum(s["m"], t, lo, jnp.maximum)
            if js[-1] == TPB * (i + 1) - 1:
                s["m"] = jnp.broadcast_to(jnp.max(s["m"], axis=1, keepdims=True), (_BQ, _T))

        def pv(i, js):
            s = st[i]
            for j in js:
                lo = first_row(i, j)
                p = jnp.exp2(s["t"][j] - s["m"][lo:]).astype(_BF)
                p32 = p.astype(_F32)
                o = _dot(p, v_b[pl.ds(j * _T, _T), :])
                s["l"] = accum(s["l"], p32, lo, jnp.add)
                s["acc"] = accum(s["acc"], o, lo, jnp.add)
            if js[-1] == TPB * (i + 1) - 1:
                l = jnp.broadcast_to(jnp.sum(s["l"], axis=1, keepdims=True), (_BQ, _T))
                r = pltpu.reciprocal(l, approx=True)
                r = r * (2.0 - l * r)
                ctx_v[h, pl.ds(i * _BQ, _BQ), :] = (s["acc"] * r).astype(_BF)

        def groups(fn, i, size):
            n = TPB * (i + 1)
            return [(fn, i, list(range(a, min(a + size, n)))) for a in range(0, n, size)]

        order = list(range(NQ - 1, 1, -1)) + [0, 1]
        att = groups(qk, order[0], 2)
        for n, i in enumerate(order):
            att += _merge(groups(qk, order[n + 1], 2) if n + 1 < NQ else [], groups(pv, i, 2))
        cost = [sum(_BQ - first_row(i, j) for j in js) * (2.0 if fn is qk else 1.0)
                for fn, i, js in att]

        def last_use(fn, blocks):
            return max(n for n, (f, i, _) in enumerate(att) if f is fn and i in blocks)

        side = []
        for r in order if project_next else []:
            side += [(last_use(qk, [r]), proj_q, r, 8), (last_use(qk, range(r, NQ)), proj_k, r, 4),
                     (last_use(pv, range(r, NQ)), proj_v, r, 4)]
        side.sort(key=lambda t: t[0])
        budget = sum(t[3] for t in side[:len(side) - _TAIL])
        done = spent = 0
        for n, ((fn, i, js), c) in enumerate(zip(att, cost)):
            fn(i, js)
            done += c
            while (len(side) > _TAIL and side[0][0] <= n
                   and spent + 0.5 * side[0][3] <= budget * (done / sum(cost)) ** 0.8):
                _, f, r, c2 = side.pop(0)
                f(r, odd)
                spent += c2
        for _, f, r, _ in side:
            f(r, odd)

    def prologue():
        cp_uk, cp_uv, cp_q = w_copies(0, (0, 0, 1))

        def clear(i, carry):
            zero_s[i] = 0
            return carry

        def kv_body(n, carry):
            c_copy(n).wait()
            x_copy(2 * n).start()
            x_copy(2 * n + 1).start()
            for r in (2 * n, 2 * n + 1):
                for odd in range(2):
                    proj_k(r, odd)
                    proj_v(r, odd)
            return carry

        for cp in (cp_uk, cp_uv, c_copy(0), c_copy(1)):
            cp.start()
        lax.fori_loop(0, zero_s.shape[0], clear, 0)
        cp_uk.wait()
        cp_uv.wait()
        for cp in [c_copy(n) for n in range(2, NQ // 2)] + [cp_q, cp_gate]:
            cp.start()
        prep_kv(0, 0)
        prep_kv(0, 1)
        lax.fori_loop(0, NQ // 2, kv_body, 0)
        cp_q.wait()
        cp_gate.wait()
        prep_q(0, 0)
        prep_q(0, 1)
        gw = gate_v[...].astype(_F32)
        waits = [0] + list(range(3, NQ, 2)) + [NQ]
        for lo, hi in zip(waits[:-1], waits[1:]):
            for r in range(lo, hi):
                x_copy(r).wait()
            if lo == waits[1]:
                for cp in cp_w1:
                    cp.start()
            for r in range(lo, hi):
                proj_q(r, 0)
                proj_q(r, 1)
                rows = pl.ds(r * _BQ, _BQ)
                z = None
                for n in range(M // _T):
                    t = x_v[rows, pl.ds(n * _T, _T)].astype(_F32) * gw[n:n + 1, :]
                    z = t if z is None else z + t
                g = lax.logistic(jnp.sum(z, axis=1, keepdims=True))
                g_v[rows, :] = jnp.broadcast_to(g, (_BQ, _T))
        for cp in cp_w1:
            cp.wait()
        for cp in cp_w:
            cp.start()

    def pair_body(p, carry):
        @pl.when(p == 1)
        def _():
            for w in (wuk_v, wuv_v, wq_v):
                rest = w.at[pl.ds(2, NP - 2)]
                pltpu.make_async_copy(rest, rest, sem.at[3]).wait()
            for cp in cp_late:
                cp.start()

        for odd in range(2):
            prep_kv(p + 1, odd)
            prep_q(p + 1, odd)
        head(2 * p, 0, True)
        head(2 * p + 1, 1, True)
        return carry

    prologue()
    lax.fori_loop(0, NP - 1, pair_body, 0)
    head(H - 2, 0, False)
    head(H - 1, 1, False)

    for cp in cp_late:
        cp.wait()
    ssmd_f[...] = ssmd_v[...].astype(_F32)
    NC = S // _T
    NB = M // _T
    HF = _T // 2

    kf32[0:8, :] = jnp.zeros((8, _T), _F32)

    def col_body(cb, carry):
        cols = aligned(cb, _T)
        sh = shift_v[:, cols].astype(_F32)
        dvec = ssmd_f[pl.ds(cb, 1), :]
        flip = 7 - lax.broadcasted_iota(jnp.int32, (8, _T), 0)
        bacc, kvs, yt, state = {}, {}, {}, {"n": 0}

        def new_step():
            state["z"] = pl.multiple_of(zero_s[state["n"]] * 8, 8)
            state["n"] += 1

        def spec_rows(kind, c, part, lo=0, n=_T):
            return pl.ds(state["z"] + ((kind * NC + c) * 2 + part) * _SPEC_STRIDE + lo, n)

        def spec_load(kind, c, fg):
            return tuple(spec_v[spec_rows(kind, c, part, fg * 8, 8), :] for part in range(2))

        def spec_store(kind, c, val):
            for part in range(2):
                spec_v[spec_rows(kind, c, part), :] = val[part * _T:(part + 1) * _T]

        def out_proj(i, g):
            rows = pl.ds(i * _BQ, _BQ)
            for h in range(4 * g, 4 * g + 4):
                t = _dot(ctx_v[h, rows, :], _staged(wo_b, h, 1))
                bacc[i] = t if h == 0 else bacc[i] + t

        def dft_u(j):
            kf32[pl.ds(8 + j * _T, _T), :] = ak_v[pl.ds(j * _T, _T), cols].astype(_F32)
            acc = kf32[pl.ds(8 + j * _T, _T), :] * sh[0:1, :]
            for s in range(1, sh.shape[0]):
                acc = acc + kf32[pl.ds(8 + j * _T - s, _T), :] * sh[s:s + 1, :]
            kv = (acc * av_v[pl.ds(j * _T, _T), cols].astype(_F32)).astype(_BF)
            kvs[j] = kv
            spec_store(0, j, _dot(dft_v[0:2 * _T, :], kv))

        def dft_k(j):
            s = _dot_nt(dft_v[2 * _T:4 * _T, :], sk_v[cols, pl.ds(j * _T, _T)])
            if j == 0:
                spec_store(1, j, s)
            else:
                p = state["prev"]
                spec_store(1, j, jnp.concatenate(
                    [s[0:HF] - p[_T:_T + HF], s[HF:_T] + p[_T + HF:],
                     s[_T:_T + HF] + p[0:HF], s[_T + HF:] - p[HF:_T]], axis=0))
            state["prev"] = s

        def mac(arg):
            fg, a = arg
            new_step()
            kc, y = {}, {}
            for j in range(4 * a + 4):
                ur, ui = spec_load(0, j, fg)
                for i in range(max(4 * a, j), 4 * a + 4):
                    if i - j not in kc:
                        kc[i - j] = spec_load(1, i - j, fg)
                    kr, ki = kc[i - j]
                    tr, ti = kr * ur - ki * ui, kr * ui + ki * ur
                    y[i] = (tr, ti) if i not in y else (y[i][0] + tr, y[i][1] + ti)
            for i, parts in y.items():
                for part in range(2):
                    spec_v[spec_rows(2, i, part, fg * 8, 8), :] = parts[part]

        def idft(c):
            new_step()
            even, odd = [_dot(dft_v[4 * _T + part * HF:4 * _T + (part + 1) * HF, :],
                              spec_v[spec_rows(2, c, part), :].astype(_BF))
                         for part in range(2)]
            mirrored = even + odd
            yt[c] = jnp.concatenate(
                [jnp.take_along_axis(mirrored[lo:lo + 8], flip, axis=0)
                 for lo in range(HF - 8, -8, -8)] + [even - odd], axis=0)

        def combine(c):
            rows = pl.ds(c * _T, _T)
            off = (c % TPB) * _T
            y = yt[c] + kvs[c].astype(_F32) * dvec
            a = x_v[rows, cols].astype(_F32) * y
            g = g_v[rows, :]
            o_v[cb, rows, :] = (g * a + (1.0 - g) * bacc[c // TPB][off:off + _T]).astype(_BF)
            if c + 1 in (NC - TPB, NC):
                out_copy(cb, int(c + 1 == NC)).start()

        for h in range(H):
            _stage(wo_b, h, wo_v[h, :, cols])
        main = [(i, g) for i in range(NQ) for g in range(H // 4)]
        f0, f1, f2, f3 = 0.02, 0.2, 0.85, 0.92
        stage1 = [(dft_k, j) for j in range(NC)] + [(dft_u, j) for j in range(NC)]
        stage2 = [(fg, a) for fg in range(_T // 8) for a in range(NC // 4)]
        side = [(f0 + (f1 - f0) * n / len(stage1), f, a) for n, (f, a) in enumerate(stage1)]
        side += [(f1 + (f2 - f1) * n / len(stage2), mac, a) for n, a in enumerate(stage2)]
        side += [(f2 + (f3 - f2) * c / NC, idft, c) for c in range(NC)]
        side += [(max(f2 + (f3 - f2) * (c + 0.5) / NC, (c // TPB + 1) / NQ), combine, c)
                 for c in range(NC)]
        side.sort(key=lambda t: t[0])
        new_step()
        k = 0
        for n, (i, g) in enumerate(main):
            while k < len(side) and side[k][0] <= n / len(main) + 1e-9:
                side[k][1](side[k][2])
                k += 1
            out_proj(i, g)
        for _, f, a in side[k:]:
            f(a)
        return carry

    lax.fori_loop(0, NB, col_body, 0)
    for cb in range(NB):
        out_copy(cb, 0).wait()
        out_copy(cb, 1).wait()


@jax.jit
def pallas_gated_mix__ssm_conv_h3__compressed_kv_cla__prompt_kernel(
    A_q: jax.Array,
    A_k: jax.Array,
    A_v: jax.Array,
    A_shift_k: jax.Array,
    A_ssm_k: jax.Array,
    A_ssm_D: jax.Array,
    B_x: jax.Array,
    B_c_kv: jax.Array,
    B_w_q: jax.Array,
    B_w_uk: jax.Array,
    B_w_uv: jax.Array,
    B_w_o: jax.Array,
    gate_w: jax.Array,
):
    del B_x
    B, S, M = A_q.shape
    _, H, D = B_w_q.shape
    DC = B_c_kv.shape[-1]
    assert B == 1 and D == _T and H % 2 == 0 and H >= 6 and S >= 4 * _BQ and S % (2 * _BQ) == 0 and B_c_kv.shape[1] == S
    NP, NC = H // 2, S // _T

    def body(*refs):
        _kernel(*refs, S=S, M=M, H=H, D=D)

    hbm = pl.BlockSpec(memory_space=pl.ANY)
    scratch = [
        pltpu.VMEM((S, M), _BF),
        pltpu.VMEM((S, DC), _BF),
        pltpu.VMEM((NP, M, D), jnp.uint32),
        pltpu.VMEM((NP, DC, D), jnp.uint32),
        pltpu.VMEM((NP, DC, D), jnp.uint32),
        pltpu.VMEM((H, D, M + _T), _BF),
        pltpu.VMEM((S, M), _BF),
        pltpu.VMEM((S, M), _BF),
        pltpu.VMEM((M, S), _BF),
        pltpu.VMEM((H, S, D), _BF),
        pltpu.VMEM(((M + 2 * DC) // _T, _T // 2, D), jnp.uint32),
        pltpu.VMEM(((M + 2 * DC) // _T, _T // 2, D), jnp.uint32),
        pltpu.VMEM((H, D // 2, _T), jnp.uint32),
    ] + [pltpu.VMEM((S, D), _BF)] * 6 + [
        pltpu.VMEM((S, _T), _F32),
        pltpu.VMEM((S + 8, _T), _F32),
        pltpu.VMEM((3 * 2 * NC * _SPEC_STRIDE, _T), _F32),
        pltpu.VMEM((M // _T, S, _T), _BF),
        pltpu.VMEM((A_shift_k.shape[1], M), _BF),
        pltpu.VMEM((M // _T, _T), _BF),
        pltpu.VMEM((M // _T, _T), _BF),
        pltpu.VMEM(_DFT_NP.shape, _BF),
        pltpu.VMEM((M // _T, _T), _F32),
        pltpu.SMEM((1 + (_T // 8) * (NC // 4) + NC,), jnp.int32),
        pltpu.SemaphoreType.DMA((6,)),
        pltpu.SemaphoreType.DMA((S // (2 * _BQ),)),
        pltpu.SemaphoreType.DMA((S // _BQ,)),
    ]
    out = pl.pallas_call(
        body,
        out_shape=jax.ShapeDtypeStruct((S, M), _BF),
        in_specs=[hbm] * 13,
        out_specs=hbm,
        scratch_shapes=scratch,
        compiler_params=pltpu.CompilerParams(vmem_limit_bytes=112 * 2 ** 20),
    )(
        A_q.reshape(S, M), A_k.reshape(S, M), A_v.reshape(S, M), A_shift_k.T, A_ssm_k,
        A_ssm_D.reshape(M // _T, _T), B_c_kv.reshape(S, DC), B_w_q, B_w_uk, B_w_uv, B_w_o,
        gate_w.reshape(M // _T, _T), _DFT_NP,
    )
    return out.reshape(B, S, M)
```

```python
import numpy as np
import jax
import jax.numpy as jnp
from jax import lax
import jax.experimental.pallas as pl
import jax.experimental.pallas.tpu as pltpu

_BF = jnp.bfloat16
_F32 = jnp.float32
_NT = (((1,), (1,)), ((), ()))
_T = 128
_BQ = 256
_SPEC_STRIDE = _T + 8
_TAIL = 4
_NEG = -1e30
_LOG2E = 1.4426950408889634


def _dft_tables(c):
    f = np.concatenate([np.arange(0, c, 2), np.arange(1, c, 2)]).astype(np.float64)
    w = np.pi * (f + 0.5) / c
    b = np.arange(c, dtype=np.float64)
    n = np.arange(c // 2, dtype=np.float64) + 0.5

    def forward(origin):
        ang = w[:, None] * (b[None, :] - origin)
        return np.concatenate([np.cos(ang), -np.sin(ang)], axis=0)

    inverse = np.concatenate([np.cos(n[:, None] * w[None, :]),
                              np.sin(n[:, None] * w[None, :])], axis=0) / c
    return np.concatenate([forward(0.0), forward((c - 1) / 2), inverse]).astype(_BF)


_DFT_NP = _dft_tables(_T)


def _dot(a, b):
    return jnp.dot(a, b, preferred_element_type=_F32)


def _dot_nt(a, b):
    return lax.dot_general(a, b, _NT, preferred_element_type=_F32)


def _unpack_head(w32, odd):
    bits = (w32 & jnp.uint32(0xFFFF0000)) if odd else (w32 << 16)
    return pltpu.bitcast(bits, _F32).astype(_BF)


def _stage(ref, first, w):
    for n in range(w.shape[0] // _T):
        ref[first + n] = pltpu.bitcast(w[n * _T:(n + 1) * _T], jnp.uint32)


def _staged(ref, first, count):
    tiles = [pltpu.bitcast(ref[first + n], _BF) for n in range(count)]
    return tiles[0] if count == 1 else jnp.concatenate(tiles, axis=0)


def _merge(a, b):
    out, ia, ib = [], 0, 0
    while ia < len(a) or ib < len(b):
        if ib >= len(b) or (ia < len(a) and ia * len(b) <= ib * len(a)):
            out.append(a[ia])
            ia += 1
        else:
            out.append(b[ib])
            ib += 1
    return out


def _kernel(x_hbm, k_hbm, v_hbm, shift_hbm, ssmk_hbm, ssmd_hbm, c_hbm, wq_hbm, wuk_hbm,
            wuv_hbm, wo_hbm, gate_hbm, dft_hbm, out_hbm,
            x_v, c_v, wq_v, wuk_v, wuv_v, wo_v, ak_v, av_v, sk_v, ctx_v,
            w0, w1, wo_b, q0, k0, v0, q1, k1, v1, g_v, spec_v, o_v,
            shift_v, ssmd_v, gate_v, dft_v, ssmd_f, zero_s,
            sem, sem_c, sem_x, *, S, M, H, D):
    NP = H // 2
    NQ = S // _BQ
    TPB = _BQ // _T
    qscale = float(D ** -0.5 * _LOG2E)

    def w_copies(p, sems):
        return [pltpu.make_async_copy(src.bitcast(jnp.uint32).at[:, p, :], dst.at[p], sem.at[n])
                for n, (src, dst) in zip(sems, ((wuk_hbm, wuk_v), (wuv_hbm, wuv_v),
                                                (wq_hbm, wq_v)))]

    cp_gate = pltpu.make_async_copy(gate_hbm, gate_v, sem.at[1])
    cp_w1 = w_copies(1, (2, 2, 2))
    cp_w = [cp for n in range(2, NP) for cp in w_copies(n, (3, 3, 3))]
    cp_late = [pltpu.make_async_copy(src, dst, sem.at[4]) for src, dst in (
        (wo_hbm, wo_v.at[:, :, pl.ds(0, M)]), (k_hbm, ak_v), (v_hbm, av_v), (ssmk_hbm, sk_v),
        (shift_hbm, shift_v), (ssmd_hbm, ssmd_v), (dft_hbm, dft_v))]

    def aligned(n, size):
        return pl.ds(n * size if isinstance(n, int) else pl.multiple_of(n * size, size), size)

    def c_copy(n):
        rows = aligned(n, 2 * _BQ)
        return pltpu.make_async_copy(c_hbm.at[rows], c_v.at[rows], sem_c.at[n])

    def x_copy(n):
        rows = aligned(n, _BQ)
        return pltpu.make_async_copy(x_hbm.at[rows], x_v.at[rows], sem_x.at[n])

    def out_copy(cb, part):
        rows = pl.ds(0, S - _BQ) if part == 0 else pl.ds(S - _BQ, _BQ)
        return pltpu.make_async_copy(o_v.at[cb, rows], out_hbm.at[rows, aligned(cb, _T)],
                                     sem.at[5])

    tri = (lax.broadcasted_iota(jnp.int32, (_T, _T), 1)
           <= lax.broadcasted_iota(jnp.int32, (_T, _T), 0))
    bufs = ((q0, k0, v0, w0), (q1, k1, v1, w1))
    NM, NK = M // _T, c_v.shape[1] // _T

    def prep_kv(p, odd):
        _stage(bufs[odd][3], NM, _unpack_head(wuk_v[p], odd))
        _stage(bufs[odd][3], NM + NK, _unpack_head(wuv_v[p], odd))

    def prep_q(p, odd):
        _stage(bufs[odd][3], 0, _unpack_head(wq_v[p], odd))

    def proj_q(r, odd):
        rows = aligned(r, _BQ)
        q = _dot(x_v[rows, :], _staged(bufs[odd][3], 0, NM)) * qscale
        bufs[odd][0][rows, :] = q.astype(_BF)

    def proj_k(r, odd):
        rows = aligned(r, _BQ)
        bufs[odd][1][rows, :] = _dot(c_v[rows, :], _staged(bufs[odd][3], NM, NK)).astype(_BF)

    def proj_v(r, odd):
        rows = aligned(r, _BQ)
        bufs[odd][2][rows, :] = _dot(c_v[rows, :],
                                     _staged(bufs[odd][3], NM + NK, NK)).astype(_BF)

    def first_row(i, j):
        return max(0, j - TPB * i) * _T

    def accum(old, new, lo, op):
        if old is None:
            return new
        if lo == 0:
            return op(old, new)
        return jnp.concatenate([old[:lo], op(old[lo:], new)], axis=0)

    def head(h, odd, project_next):
        q_b, k_b, v_b, _ = bufs[odd]
        st = {}

        def qk(i, js):
            s = st.setdefault(i, dict(t={}, m=None, l=None, acc=None))
            q = q_b[pl.ds(i * _BQ, _BQ), :]
            for j in js:
                lo = first_row(i, j)
                t = _dot_nt(q[lo:], k_b[pl.ds(j * _T, _T), :])
                if j >= TPB * i:
                    top = jnp.where(tri, t[0:_T], _NEG)
                    t = top if t.shape[0] == _T else jnp.concatenate([top, t[_T:]], axis=0)
                s["t"][j] = t
                s["m"] = accum(s["m"], t, lo, jnp.maximum)
            if js[-1] == TPB * (i + 1) - 1:
                s["m"] = jnp.broadcast_to(jnp.max(s["m"], axis=1, keepdims=True), (_BQ, _T))

        def pv(i, js):
            s = st[i]
            for j in js:
                lo = first_row(i, j)
                p = jnp.exp2(s["t"][j] - s["m"][lo:]).astype(_BF)
                p32 = p.astype(_F32)
                o = _dot(p, v_b[pl.ds(j * _T, _T), :])
                s["l"] = accum(s["l"], p32, lo, jnp.add)
                s["acc"] = accum(s["acc"], o, lo, jnp.add)
            if js[-1] == TPB * (i + 1) - 1:
                l = jnp.broadcast_to(jnp.sum(s["l"], axis=1, keepdims=True), (_BQ, _T))
                r = pltpu.reciprocal(l, approx=True)
                r = r * (2.0 - l * r)
                ctx_v[h, pl.ds(i * _BQ, _BQ), :] = (s["acc"] * r).astype(_BF)

        def groups(fn, i, size):
            n = TPB * (i + 1)
            return [(fn, i, list(range(a, min(a + size, n)))) for a in range(0, n, size)]

        order = list(range(NQ - 1, 1, -1)) + [0, 1]
        att = groups(qk, order[0], 2)
        for n, i in enumerate(order):
            att += _merge(groups(qk, order[n + 1], 2) if n + 1 < NQ else [], groups(pv, i, 2))
        cost = [sum(_BQ - first_row(i, j) for j in js) * (2.0 if fn is qk else 1.0)
                for fn, i, js in att]

        def last_use(fn, blocks):
            return max(n for n, (f, i, _) in enumerate(att) if f is fn and i in blocks)

        side = []
        for r in order if project_next else []:
            side += [(last_use(qk, [r]), proj_q, r, 8), (last_use(qk, range(r, NQ)), proj_k, r, 4),
                     (last_use(pv, range(r, NQ)), proj_v, r, 4)]
        side.sort(key=lambda t: t[0])
        budget = sum(t[3] for t in side[:len(side) - _TAIL])
        done = spent = 0
        for n, ((fn, i, js), c) in enumerate(zip(att, cost)):
            fn(i, js)
            done += c
            while (len(side) > _TAIL and side[0][0] <= n
                   and spent + 0.5 * side[0][3] <= budget * (done / sum(cost)) ** 0.8):
                _, f, r, c2 = side.pop(0)
                f(r, odd)
                spent += c2
        for _, f, r, _ in side:
            f(r, odd)

    def prologue():
        cp_uk, cp_uv, cp_q = w_copies(0, (0, 0, 1))

        def clear(i, carry):
            zero_s[i] = 0
            return carry

        def kv_body(n, carry):
            c_copy(n).wait()
            x_copy(2 * n).start()
            x_copy(2 * n + 1).start()
            for r in (2 * n, 2 * n + 1):
                for odd in range(2):
                    proj_k(r, odd)
                    proj_v(r, odd)
            return carry

        for cp in (cp_uk, cp_uv, c_copy(0), c_copy(1)):
            cp.start()
        lax.fori_loop(0, zero_s.shape[0], clear, 0)
        cp_uk.wait()
        cp_uv.wait()
        for cp in [c_copy(n) for n in range(2, NQ // 2)] + [cp_q, cp_gate]:
            cp.start()
        prep_kv(0, 0)
        prep_kv(0, 1)
        lax.fori_loop(0, NQ // 2, kv_body, 0)
        cp_q.wait()
        cp_gate.wait()
        prep_q(0, 0)
        prep_q(0, 1)
        gw = gate_v[...].astype(_F32)
        waits = [0] + list(range(3, NQ, 2)) + [NQ]
        for lo, hi in zip(waits[:-1], waits[1:]):
            for r in range(lo, hi):
                x_copy(r).wait()
            if lo == waits[1]:
                for cp in cp_w1:
                    cp.start()
            for r in range(lo, hi):
                proj_q(r, 0)
                proj_q(r, 1)
                rows = pl.ds(r * _BQ, _BQ)
                z = None
                for n in range(M // _T):
                    t = x_v[rows, pl.ds(n * _T, _T)].astype(_F32) * gw[n:n + 1, :]
                    z = t if z is None else z + t
                g = lax.logistic(jnp.sum(z, axis=1, keepdims=True))
                g_v[rows, :] = jnp.broadcast_to(g, (_BQ, _T))
        for cp in cp_w1:
            cp.wait()
        for cp in cp_w:
            cp.start()

    def pair_body(p, carry):
        @pl.when(p == 1)
        def _():
            for w in (wuk_v, wuv_v, wq_v):
                rest = w.at[pl.ds(2, NP - 2)]
                pltpu.make_async_copy(rest, rest, sem.at[3]).wait()
            for cp in cp_late:
                cp.start()

        for odd in range(2):
            prep_kv(p + 1, odd)
            prep_q(p + 1, odd)
        head(2 * p, 0, True)
        head(2 * p + 1, 1, True)
        return carry

    prologue()
    lax.fori_loop(0, NP - 1, pair_body, 0)
    head(H - 2, 0, False)
    head(H - 1, 1, False)

    for cp in cp_late:
        cp.wait()
    ssmd_f[...] = ssmd_v[...].astype(_F32)
    NC = S // _T
    NB = M // _T
    HF = _T // 2

    def col_body(cb, carry):
        cols = aligned(cb, _T)
        sh = shift_v[:, cols].astype(_F32)
        dvec = ssmd_f[pl.ds(cb, 1), :]
        flip = 7 - lax.broadcasted_iota(jnp.int32, (8, _T), 0)
        bacc, kvs, yt, state = {}, {}, {}, {"n": 0, "tail": jnp.zeros((8, _T), _F32)}

        def new_step():
            state["z"] = pl.multiple_of(zero_s[state["n"]] * 8, 8)
            state["n"] += 1

        def spec_rows(kind, c, part, lo=0, n=_T):
            return pl.ds(state["z"] + ((kind * NC + c) * 2 + part) * _SPEC_STRIDE + lo, n)

        def spec_load(kind, c, fg):
            return tuple(spec_v[spec_rows(kind, c, part, fg * 8, 8), :] for part in range(2))

        def spec_store(kind, c, val):
            for part in range(2):
                spec_v[spec_rows(kind, c, part), :] = val[part * _T:(part + 1) * _T]

        def out_proj(i, g):
            rows = pl.ds(i * _BQ, _BQ)
            for h in range(4 * g, 4 * g + 4):
                t = _dot(ctx_v[h, rows, :], _staged(wo_b, h, 1))
                bacc[i] = t if h == 0 else bacc[i] + t

        def dft_u(j):
            cur = ak_v[pl.ds(j * _T, _T), cols].astype(_F32)
            ext = jnp.concatenate([state["tail"], cur], axis=0)
            state["tail"] = cur[_T - 8:]
            acc = cur * sh[0:1, :]
            for s in range(1, sh.shape[0]):
                acc = acc + ext[8 - s:8 - s + _T] * sh[s:s + 1, :]
            kv = (acc * av_v[pl.ds(j * _T, _T), cols].astype(_F32)).astype(_BF)
            kvs[j] = kv
            spec_store(0, j, _dot(dft_v[0:2 * _T, :], kv))

        def dft_k(j):
            s = _dot_nt(dft_v[2 * _T:4 * _T, :], sk_v[cols, pl.ds(j * _T, _T)])
            if j == 0:
                spec_store(1, j, s)
            else:
                p = state["prev"]
                spec_store(1, j, jnp.concatenate(
                    [s[0:HF] - p[_T:_T + HF], s[HF:_T] + p[_T + HF:],
                     s[_T:_T + HF] + p[0:HF], s[_T + HF:] - p[HF:_T]], axis=0))
            state["prev"] = s

        def mac(arg):
            fg, a = arg
            new_step()
            kc, y = {}, {}
            for j in range(4 * a + 4):
                ur, ui = spec_load(0, j, fg)
                for i in range(max(4 * a, j), 4 * a + 4):
                    if i - j not in kc:
                        kc[i - j] = spec_load(1, i - j, fg)
                    kr, ki = kc[i - j]
                    tr, ti = kr * ur - ki * ui, kr * ui + ki * ur
                    y[i] = (tr, ti) if i not in y else (y[i][0] + tr, y[i][1] + ti)
            for i, parts in y.items():
                for part in range(2):
                    spec_v[spec_rows(2, i, part, fg * 8, 8), :] = parts[part]

        def idft(c):
            new_step()
            even, odd = [_dot(dft_v[4 * _T + part * HF:4 * _T + (part + 1) * HF, :],
                              spec_v[spec_rows(2, c, part), :].astype(_BF))
                         for part in range(2)]
            mirrored = even + odd
            yt[c] = jnp.concatenate(
                [jnp.take_along_axis(mirrored[lo:lo + 8], flip, axis=0)
                 for lo in range(HF - 8, -8, -8)] + [even - odd], axis=0)

        def combine(c):
            rows = pl.ds(c * _T, _T)
            off = (c % TPB) * _T
            y = yt[c] + kvs[c].astype(_F32) * dvec
            a = x_v[rows, cols].astype(_F32) * y
            g = g_v[rows, :]
            o_v[cb, rows, :] = (g * a + (1.0 - g) * bacc[c // TPB][off:off + _T]).astype(_BF)
            if c + 1 in (NC - TPB, NC):
                out_copy(cb, int(c + 1 == NC)).start()

        for h in range(H):
            _stage(wo_b, h, wo_v[h, :, cols])
        main = [(i, g) for i in range(NQ) for g in range(H // 4)]
        f0, f1, f2, f3 = 0.02, 0.2, 0.75, 0.86
        stage1 = [(dft_k, j) for j in range(NC)] + [(dft_u, j) for j in range(NC)]
        stage2 = [(fg, a) for fg in range(_T // 8) for a in range(NC // 4)]
        side = [(f0 + (f1 - f0) * n / len(stage1), f, a) for n, (f, a) in enumerate(stage1)]
        side += [(f1 + (f2 - f1) * n / len(stage2), mac, a) for n, a in enumerate(stage2)]
        side += [(f2 + (f3 - f2) * c / NC, idft, c) for c in range(NC)]
        side += [(max(f2 + (f3 - f2) * (c + 0.5) / NC, (c // TPB + 1) / NQ), combine, c)
                 for c in range(NC)]
        side.sort(key=lambda t: t[0])
        new_step()
        k = 0
        for n, (i, g) in enumerate(main):
            while k < len(side) and side[k][0] <= n / len(main) + 1e-9:
                side[k][1](side[k][2])
                k += 1
            out_proj(i, g)
        for _, f, a in side[k:]:
            f(a)
        return carry

    lax.fori_loop(0, NB, col_body, 0)
    for cb in range(NB):
        out_copy(cb, 0).wait()
        out_copy(cb, 1).wait()


@jax.jit
def pallas_gated_mix__ssm_conv_h3__compressed_kv_cla__prompt_kernel(
    A_q: jax.Array,
    A_k: jax.Array,
    A_v: jax.Array,
    A_shift_k: jax.Array,
    A_ssm_k: jax.Array,
    A_ssm_D: jax.Array,
    B_x: jax.Array,
    B_c_kv: jax.Array,
    B_w_q: jax.Array,
    B_w_uk: jax.Array,
    B_w_uv: jax.Array,
    B_w_o: jax.Array,
    gate_w: jax.Array,
):
    del B_x
    B, S, M = A_q.shape
    _, H, D = B_w_q.shape
    DC = B_c_kv.shape[-1]
    assert B == 1 and D == _T and H % 2 == 0 and H >= 6 and S >= 4 * _BQ and S % (2 * _BQ) == 0 and B_c_kv.shape[1] == S
    NP, NC = H // 2, S // _T

    def body(*refs):
        _kernel(*refs, S=S, M=M, H=H, D=D)

    hbm = pl.BlockSpec(memory_space=pl.ANY)
    scratch = [
        pltpu.VMEM((S, M), _BF),
        pltpu.VMEM((S, DC), _BF),
        pltpu.VMEM((NP, M, D), jnp.uint32),
        pltpu.VMEM((NP, DC, D), jnp.uint32),
        pltpu.VMEM((NP, DC, D), jnp.uint32),
        pltpu.VMEM((H, D, M + _T), _BF),
        pltpu.VMEM((S, M), _BF),
        pltpu.VMEM((S, M), _BF),
        pltpu.VMEM((M, S), _BF),
        pltpu.VMEM((H, S, D), _BF),
        pltpu.VMEM(((M + 2 * DC) // _T, _T // 2, D), jnp.uint32),
        pltpu.VMEM(((M + 2 * DC) // _T, _T // 2, D), jnp.uint32),
        pltpu.VMEM((H, D // 2, _T), jnp.uint32),
    ] + [pltpu.VMEM((S, D), _BF)] * 6 + [
        pltpu.VMEM((S, _T), _F32),
        pltpu.VMEM((3 * 2 * NC * _SPEC_STRIDE, _T), _F32),
        pltpu.VMEM((M // _T, S, _T), _BF),
        pltpu.VMEM((A_shift_k.shape[1], M), _BF),
        pltpu.VMEM((M // _T, _T), _BF),
        pltpu.VMEM((M // _T, _T), _BF),
        pltpu.VMEM(_DFT_NP.shape, _BF),
        pltpu.VMEM((M // _T, _T), _F32),
        pltpu.SMEM((1 + (_T // 8) * (NC // 4) + NC,), jnp.int32),
        pltpu.SemaphoreType.DMA((6,)),
        pltpu.SemaphoreType.DMA((S // (2 * _BQ),)),
        pltpu.SemaphoreType.DMA((S // _BQ,)),
    ]
    out = pl.pallas_call(
        body,
        out_shape=jax.ShapeDtypeStruct((S, M), _BF),
        in_specs=[hbm] * 13,
        out_specs=hbm,
        scratch_shapes=scratch,
        compiler_params=pltpu.CompilerParams(vmem_limit_bytes=112 * 2 ** 20),
    )(
        A_q.reshape(S, M), A_k.reshape(S, M), A_v.reshape(S, M), A_shift_k.T, A_ssm_k,
        A_ssm_D.reshape(M // _T, _T), B_c_kv.reshape(S, DC), B_w_q, B_w_uk, B_w_uv, B_w_o,
        gate_w.reshape(M // _T, _T), _DFT_NP,
    )
    return out.reshape(B, S, M)
```

```python
import numpy as np
import jax
import jax.numpy as jnp
from jax import lax
import jax.experimental.pallas as pl
import jax.experimental.pallas.tpu as pltpu

_BF = jnp.bfloat16
_F32 = jnp.float32
_NT = (((1,), (1,)), ((), ()))
_T = 128
_BQ = 256
_SPEC_STRIDE = _T + 8
_TAIL = 4
_NEG = -1e30
_LOG2E = 1.4426950408889634


def _dft_tables(c):
    f = np.concatenate([np.arange(0, c, 2), np.arange(1, c, 2)]).astype(np.float64)
    w = np.pi * (f + 0.5) / c
    b = np.arange(c, dtype=np.float64)
    n = np.arange(c // 2, dtype=np.float64) + 0.5

    def forward(origin):
        ang = w[:, None] * (b[None, :] - origin)
        return np.concatenate([np.cos(ang), -np.sin(ang)], axis=0)

    inverse = np.concatenate([np.cos(n[:, None] * w[None, :]),
                              np.sin(n[:, None] * w[None, :])], axis=0) / c
    return np.concatenate([forward(0.0), forward((c - 1) / 2), inverse]).astype(_BF)


_DFT_NP = _dft_tables(_T)


def _dot(a, b):
    return jnp.dot(a, b, preferred_element_type=_F32)


def _dot_nt(a, b):
    return lax.dot_general(a, b, _NT, preferred_element_type=_F32)


def _unpack_head(w32, odd):
    bits = (w32 & jnp.uint32(0xFFFF0000)) if odd else (w32 << 16)
    return pltpu.bitcast(bits, _F32).astype(_BF)


def _stage(ref, first, w):
    for n in range(w.shape[0] // _T):
        ref[first + n] = pltpu.bitcast(w[n * _T:(n + 1) * _T], jnp.uint32)


def _staged(ref, first, count):
    tiles = [pltpu.bitcast(ref[first + n], _BF) for n in range(count)]
    return tiles[0] if count == 1 else jnp.concatenate(tiles, axis=0)


def _merge(a, b):
    out, ia, ib = [], 0, 0
    while ia < len(a) or ib < len(b):
        if ib >= len(b) or (ia < len(a) and ia * len(b) <= ib * len(a)):
            out.append(a[ia])
            ia += 1
        else:
            out.append(b[ib])
            ib += 1
    return out


def _kernel(x_hbm, k_hbm, v_hbm, shift_hbm, ssmk_hbm, ssmd_hbm, c_hbm, wq_hbm, wuk_hbm,
            wuv_hbm, wo_hbm, gate_hbm, dft_hbm, out_hbm,
            x_v, c_v, wq_v, wuk_v, wuv_v, wo_v, ak_v, av_v, sk_v, ctx_v,
            w0, w1, wo_b, q0, k0, v0, q1, k1, v1, g_v, spec_v, o_v,
            shift_v, ssmd_v, gate_v, dft_v, ssmd_f, zero_s,
            sem, sem_c, sem_x, *, S, M, H, D):
    NP = H // 2
    NQ = S // _BQ
    TPB = _BQ // _T
    qscale = float(D ** -0.5 * _LOG2E)

    def w_copies(p, sems):
        return [pltpu.make_async_copy(src.bitcast(jnp.uint32).at[:, p, :], dst.at[p], sem.at[n])
                for n, (src, dst) in zip(sems, ((wuk_hbm, wuk_v), (wuv_hbm, wuv_v),
                                                (wq_hbm, wq_v)))]

    cp_gate = pltpu.make_async_copy(gate_hbm, gate_v, sem.at[1])
    cp_w1 = w_copies(1, (2, 2, 2))
    cp_w = [cp for n in range(2, NP) for cp in w_copies(n, (3, 3, 3))]
    cp_late = [pltpu.make_async_copy(src, dst, sem.at[4]) for src, dst in (
        (wo_hbm, wo_v.at[:, :, pl.ds(0, M)]), (k_hbm, ak_v), (v_hbm, av_v), (ssmk_hbm, sk_v),
        (shift_hbm, shift_v), (ssmd_hbm, ssmd_v), (dft_hbm, dft_v))]

    def aligned(n, size):
        return pl.ds(n * size if isinstance(n, int) else pl.multiple_of(n * size, size), size)

    def c_copy(n):
        rows = aligned(n, 2 * _BQ)
        return pltpu.make_async_copy(c_hbm.at[rows], c_v.at[rows], sem_c.at[n])

    def x_copy(n):
        rows = aligned(n, _BQ)
        return pltpu.make_async_copy(x_hbm.at[rows], x_v.at[rows], sem_x.at[n])

    def out_copy(cb, part):
        rows = pl.ds(0, S - _BQ) if part == 0 else pl.ds(S - _BQ, _BQ)
        return pltpu.make_async_copy(o_v.at[cb, rows], out_hbm.at[rows, aligned(cb, _T)],
                                     sem.at[5])

    tri = (lax.broadcasted_iota(jnp.int32, (_T, _T), 1)
           <= lax.broadcasted_iota(jnp.int32, (_T, _T), 0))
    bufs = ((q0, k0, v0, w0), (q1, k1, v1, w1))
    NM, NK = M // _T, c_v.shape[1] // _T

    def prep_kv(p, odd):
        _stage(bufs[odd][3], NM, _unpack_head(wuk_v[p], odd))
        _stage(bufs[odd][3], NM + NK, _unpack_head(wuv_v[p], odd))

    def prep_q(p, odd):
        _stage(bufs[odd][3], 0, _unpack_head(wq_v[p], odd))

    def proj_q(r, odd):
        rows = aligned(r, _BQ)
        q = _dot(x_v[rows, :], _staged(bufs[odd][3], 0, NM)) * qscale
        bufs[odd][0][rows, :] = q.astype(_BF)

    def proj_k(r, odd):
        rows = aligned(r, _BQ)
        bufs[odd][1][rows, :] = _dot(c_v[rows, :], _staged(bufs[odd][3], NM, NK)).astype(_BF)

    def proj_v(r, odd):
        rows = aligned(r, _BQ)
        bufs[odd][2][rows, :] = _dot(c_v[rows, :],
                                     _staged(bufs[odd][3], NM + NK, NK)).astype(_BF)

    def first_row(i, j):
        return max(0, j - TPB * i) * _T

    def accum(old, new, lo, op):
        if old is None:
            return new
        if lo == 0:
            return op(old, new)
        return jnp.concatenate([old[:lo], op(old[lo:], new)], axis=0)

    def head(h, odd, project_next):
        q_b, k_b, v_b, _ = bufs[odd]
        st = {}

        def qk(i, js):
            s = st.setdefault(i, dict(t={}, m=None, l=None, acc=None))
            q = q_b[pl.ds(i * _BQ, _BQ), :]
            for j in js:
                lo = first_row(i, j)
                t = _dot_nt(q[lo:], k_b[pl.ds(j * _T, _T), :])
                if j >= TPB * i:
                    top = jnp.where(tri, t[0:_T], _NEG)
                    t = top if t.shape[0] == _T else jnp.concatenate([top, t[_T:]], axis=0)
                s["t"][j] = t
                s["m"] = accum(s["m"], t, lo, jnp.maximum)
            if js[-1] == TPB * (i + 1) - 1:
                s["m"] = jnp.broadcast_to(jnp.max(s["m"], axis=1, keepdims=True), (_BQ, _T))

        def pv(i, js):
            s = st[i]
            for j in js:
                lo = first_row(i, j)
                p = jnp.exp2(s["t"][j] - s["m"][lo:]).astype(_BF)
                p32 = p.astype(_F32)
                o = _dot(p, v_b[pl.ds(j * _T, _T), :])
                s["l"] = accum(s["l"], p32, lo, jnp.add)
                s["acc"] = accum(s["acc"], o, lo, jnp.add)
            if js[-1] == TPB * (i + 1) - 1:
                l = jnp.broadcast_to(jnp.sum(s["l"], axis=1, keepdims=True), (_BQ, _T))
                r = pltpu.reciprocal(l, approx=True)
                r = r * (2.0 - l * r)
                ctx_v[h, pl.ds(i * _BQ, _BQ), :] = (s["acc"] * r).astype(_BF)

        def groups(fn, i, size):
            n = TPB * (i + 1)
            return [(fn, i, list(range(a, min(a + size, n)))) for a in range(0, n, size)]

        order = list(range(NQ - 1, 1, -1)) + [0, 1]
        att = groups(qk, order[0], 2)
        for n, i in enumerate(order):
            att += _merge(groups(qk, order[n + 1], 2) if n + 1 < NQ else [], groups(pv, i, 2))
        cost = [sum(_BQ - first_row(i, j) for j in js) * (2.0 if fn is qk else 1.0)
                for fn, i, js in att]

        def last_use(fn, blocks):
            return max(n for n, (f, i, _) in enumerate(att) if f is fn and i in blocks)

        side = []
        for r in order if project_next else []:
            side += [(last_use(qk, [r]), proj_q, r, 8), (last_use(qk, range(r, NQ)), proj_k, r, 4),
                     (last_use(pv, range(r, NQ)), proj_v, r, 4)]
        side.sort(key=lambda t: t[0])
        budget = sum(t[3] for t in side[:len(side) - _TAIL])
        tasks = []
        done = spent = 0
        for n, (task, c) in enumerate(zip(att, cost)):
            tasks.append(task)
            done += c
            while (len(side) > _TAIL and side[0][0] <= n
                   and spent + 0.5 * side[0][3] <= budget * (done / sum(cost)) ** 0.8):
                _, f, r, c2 = side.pop(0)
                tasks.append((f, r, odd))
                spent += c2
        return tasks + [(f, r, odd) for _, f, r, _ in side]

    def run(tasks):
        for fn, a, b in tasks:
            fn(a, b)

    def prologue():
        cp_uk, cp_uv, cp_q = w_copies(0, (0, 0, 1))

        def clear(i, carry):
            zero_s[i] = 0
            return carry

        def kv_body(n, carry):
            c_copy(n).wait()
            x_copy(2 * n).start()
            x_copy(2 * n + 1).start()
            for r in (2 * n, 2 * n + 1):
                for odd in range(2):
                    proj_k(r, odd)
                    proj_v(r, odd)
            return carry

        for cp in (cp_uk, cp_uv, c_copy(0)):
            cp.start()
        lax.fori_loop(0, zero_s.shape[0], clear, 0)
        cp_uk.wait()
        cp_uv.wait()
        for cp in [c_copy(n) for n in range(1, NQ // 2)] + [cp_q, cp_gate]:
            cp.start()
        prep_kv(0, 0)
        prep_kv(0, 1)
        lax.fori_loop(0, NQ // 2, kv_body, 0)
        cp_q.wait()
        cp_gate.wait()
        prep_q(0, 0)
        prep_q(0, 1)
        gw = gate_v[...].astype(_F32)
        waits = list(range(0, NQ + 1, 2))
        for lo, hi in zip(waits[:-1], waits[1:]):
            for r in range(lo, hi):
                x_copy(r).wait()
            if lo == NQ // 4 * 2:
                for cp in cp_w1:
                    cp.start()
            for r in range(lo, hi):
                proj_q(r, 0)
                proj_q(r, 1)
                rows = pl.ds(r * _BQ, _BQ)
                z = None
                for n in range(M // _T):
                    t = x_v[rows, pl.ds(n * _T, _T)].astype(_F32) * gw[n:n + 1, :]
                    z = t if z is None else z + t
                g = lax.logistic(jnp.sum(z, axis=1, keepdims=True))
                g_v[rows, :] = jnp.broadcast_to(g, (_BQ, _T))
        for cp in cp_w1:
            cp.wait()
        for cp in cp_w:
            cp.start()

    def pair_body(p, carry):
        @pl.when(p == 1)
        def _():
            for w in (wuk_v, wuv_v, wq_v):
                rest = w.at[pl.ds(2, NP - 2)]
                pltpu.make_async_copy(rest, rest, sem.at[3]).wait()
            for cp in cp_late:
                cp.start()

        for odd in range(2):
            prep_kv(p + 1, odd)
            prep_q(p + 1, odd)
        run(head(2 * p, 0, True) + head(2 * p + 1, 1, True))
        return carry

    prologue()
    lax.fori_loop(0, NP - 1, pair_body, 0)
    t0, t1 = head(H - 2, 0, False), head(H - 1, 1, False)
    run(t0[:8] + _merge(t0[8:], t1[:-8]) + t1[-8:])

    for cp in cp_late:
        cp.wait()
    ssmd_f[...] = ssmd_v[...].astype(_F32)
    NC = S // _T
    NB = M // _T
    HF = _T // 2

    def col_body(cb, carry):
        cols = aligned(cb, _T)
        sh = shift_v[:, cols].astype(_F32)
        dvec = ssmd_f[pl.ds(cb, 1), :]
        flip = 7 - lax.broadcasted_iota(jnp.int32, (8, _T), 0)
        bacc, kvs, yt, state = {}, {}, {}, {"n": 0, "tail": jnp.zeros((8, _T), _F32)}

        def new_step():
            state["z"] = pl.multiple_of(zero_s[state["n"]] * 8, 8)
            state["n"] += 1

        def spec_rows(kind, c, part, lo=0, n=_T):
            return pl.ds(state["z"] + ((kind * NC + c) * 2 + part) * _SPEC_STRIDE + lo, n)

        def spec_load(kind, c, fg):
            return tuple(spec_v[spec_rows(kind, c, part, fg * 8, 8), :] for part in range(2))

        def spec_store(kind, c, val):
            for part in range(2):
                spec_v[spec_rows(kind, c, part), :] = val[part * _T:(part + 1) * _T]

        def out_proj(i, g):
            rows = pl.ds(i * _BQ, _BQ)
            for h in range(4 * g, 4 * g + 4):
                t = _dot(ctx_v[h, rows, :], _staged(wo_b, h, 1))
                bacc[i] = t if h == 0 else bacc[i] + t

        def dft_u(j):
            cur = ak_v[pl.ds(j * _T, _T), cols].astype(_F32)
            ext = jnp.concatenate([state["tail"], cur], axis=0)
            state["tail"] = cur[_T - 8:]
            acc = cur * sh[0:1, :]
            for s in range(1, sh.shape[0]):
                acc = acc + ext[8 - s:8 - s + _T] * sh[s:s + 1, :]
            kv = (acc * av_v[pl.ds(j * _T, _T), cols].astype(_F32)).astype(_BF)
            kvs[j] = kv
            spec_store(0, j, _dot(dft_v[0:2 * _T, :], kv))

        def dft_k(j):
            s = _dot_nt(dft_v[2 * _T:4 * _T, :], sk_v[cols, pl.ds(j * _T, _T)])
            if j == 0:
                spec_store(1, j, s)
            else:
                p = state["prev"]
                spec_store(1, j, jnp.concatenate(
                    [s[0:HF] - p[_T:_T + HF], s[HF:_T] + p[_T + HF:],
                     s[_T:_T + HF] + p[0:HF], s[_T + HF:] - p[HF:_T]], axis=0))
            state["prev"] = s

        def mac(arg):
            fg, a = arg
            new_step()
            kc, y = {}, {}
            for j in range(4 * a + 4):
                ur, ui = spec_load(0, j, fg)
                for i in range(max(4 * a, j), 4 * a + 4):
                    if i - j not in kc:
                        kc[i - j] = spec_load(1, i - j, fg)
                    kr, ki = kc[i - j]
                    tr, ti = kr * ur - ki * ui, kr * ui + ki * ur
                    y[i] = (tr, ti) if i not in y else (y[i][0] + tr, y[i][1] + ti)
            for i, parts in y.items():
                for part in range(2):
                    spec_v[spec_rows(2, i, part, fg * 8, 8), :] = parts[part]

        def idft(c):
            new_step()
            even, odd = [_dot(dft_v[4 * _T + part * HF:4 * _T + (part + 1) * HF, :],
                              spec_v[spec_rows(2, c, part), :].astype(_BF))
                         for part in range(2)]
            mirrored = even + odd
            yt[c] = jnp.concatenate(
                [jnp.take_along_axis(mirrored[lo:lo + 8], flip, axis=0)
                 for lo in range(HF - 8, -8, -8)] + [even - odd], axis=0)

        def combine(c):
            rows = pl.ds(c * _T, _T)
            off = (c % TPB) * _T
            y = yt[c] + kvs[c].astype(_F32) * dvec
            a = x_v[rows, cols].astype(_F32) * y
            g = g_v[rows, :]
            o_v[cb, rows, :] = (g * a + (1.0 - g) * bacc[c // TPB][off:off + _T]).astype(_BF)
            if c + 1 in (NC - TPB, NC):
                out_copy(cb, int(c + 1 == NC)).start()

        for h in range(H):
            _stage(wo_b, h, wo_v[h, :, cols])
        main = [(i, g) for i in range(NQ) for g in range(H // 4)]
        f0, f1, f2, f3 = 0.02, 0.2, 0.75, 0.86
        stage1 = [(dft_k, j) for j in range(NC)] + [(dft_u, j) for j in range(NC)]
        stage2 = [(fg, a) for fg in range(_T // 8) for a in range(NC // 4)]
        side = [(f0 + (f1 - f0) * n / len(stage1), f, a) for n, (f, a) in enumerate(stage1)]
        side += [(f1 + (f2 - f1) * n / len(stage2), mac, a) for n, a in enumerate(stage2)]
        side += [(f2 + (f3 - f2) * c / NC, idft, c) for c in range(NC)]
        side += [(max(f2 + (f3 - f2) * (c + 0.5) / NC, (c // TPB + 1) / NQ), combine, c)
                 for c in range(NC)]
        side.sort(key=lambda t: t[0])
        new_step()
        k = 0
        for n, (i, g) in enumerate(main):
            while k < len(side) and side[k][0] <= n / len(main) + 1e-9:
                side[k][1](side[k][2])
                k += 1
            out_proj(i, g)
        for _, f, a in side[k:]:
            f(a)
        return carry

    lax.fori_loop(0, NB, col_body, 0)
    for cb in range(NB):
        out_copy(cb, 0).wait()
        out_copy(cb, 1).wait()


@jax.jit
def pallas_gated_mix__ssm_conv_h3__compressed_kv_cla__prompt_kernel(
    A_q: jax.Array,
    A_k: jax.Array,
    A_v: jax.Array,
    A_shift_k: jax.Array,
    A_ssm_k: jax.Array,
    A_ssm_D: jax.Array,
    B_x: jax.Array,
    B_c_kv: jax.Array,
    B_w_q: jax.Array,
    B_w_uk: jax.Array,
    B_w_uv: jax.Array,
    B_w_o: jax.Array,
    gate_w: jax.Array,
):
    del B_x
    B, S, M = A_q.shape
    _, H, D = B_w_q.shape
    DC = B_c_kv.shape[-1]
    assert B == 1 and D == _T and H % 2 == 0 and H >= 6 and S >= 4 * _BQ and S % (2 * _BQ) == 0 and B_c_kv.shape[1] == S
    NP, NC = H // 2, S // _T

    def body(*refs):
        _kernel(*refs, S=S, M=M, H=H, D=D)

    hbm = pl.BlockSpec(memory_space=pl.ANY)
    scratch = [
        pltpu.VMEM((S, M), _BF),
        pltpu.VMEM((S, DC), _BF),
        pltpu.VMEM((NP, M, D), jnp.uint32),
        pltpu.VMEM((NP, DC, D), jnp.uint32),
        pltpu.VMEM((NP, DC, D), jnp.uint32),
        pltpu.VMEM((H, D, M + _T), _BF),
        pltpu.VMEM((S, M), _BF),
        pltpu.VMEM((S, M), _BF),
        pltpu.VMEM((M, S), _BF),
        pltpu.VMEM((H, S, D), _BF),
        pltpu.VMEM(((M + 2 * DC) // _T, _T // 2, D), jnp.uint32),
        pltpu.VMEM(((M + 2 * DC) // _T, _T // 2, D), jnp.uint32),
        pltpu.VMEM((H, D // 2, _T), jnp.uint32),
    ] + [pltpu.VMEM((S, D), _BF)] * 6 + [
        pltpu.VMEM((S, _T), _F32),
        pltpu.VMEM((3 * 2 * NC * _SPEC_STRIDE, _T), _F32),
        pltpu.VMEM((M // _T, S, _T), _BF),
        pltpu.VMEM((A_shift_k.shape[1], M), _BF),
        pltpu.VMEM((M // _T, _T), _BF),
        pltpu.VMEM((M // _T, _T), _BF),
        pltpu.VMEM(_DFT_NP.shape, _BF),
        pltpu.VMEM((M // _T, _T), _F32),
        pltpu.SMEM((1 + (_T // 8) * (NC // 4) + NC,), jnp.int32),
        pltpu.SemaphoreType.DMA((6,)),
        pltpu.SemaphoreType.DMA((S // (2 * _BQ),)),
        pltpu.SemaphoreType.DMA((S // _BQ,)),
    ]
    out = pl.pallas_call(
        body,
        out_shape=jax.ShapeDtypeStruct((S, M), _BF),
        in_specs=[hbm] * 13,
        out_specs=hbm,
        scratch_shapes=scratch,
        compiler_params=pltpu.CompilerParams(vmem_limit_bytes=112 * 2 ** 20),
    )(
        A_q.reshape(S, M), A_k.reshape(S, M), A_v.reshape(S, M), A_shift_k.T, A_ssm_k,
        A_ssm_D.reshape(M // _T, _T), B_c_kv.reshape(S, DC), B_w_q, B_w_uk, B_w_uv, B_w_o,
        gate_w.reshape(M // _T, _T), _DFT_NP,
    )
    return out.reshape(B, S, M)
```

```python
import numpy as np
import jax
import jax.numpy as jnp
from jax import lax
import jax.experimental.pallas as pl
import jax.experimental.pallas.tpu as pltpu

_BF = jnp.bfloat16
_F32 = jnp.float32
_NT = (((1,), (1,)), ((), ()))
_T = 128
_BQ = 256
_SPEC_STRIDE = _T + 8
_TAIL = 4
_NEG = -1e30
_LOG2E = 1.4426950408889634


def _dft_tables(c):
    f = np.concatenate([np.arange(0, c, 2), np.arange(1, c, 2)]).astype(np.float64)
    w = np.pi * (f + 0.5) / c
    b = np.arange(c, dtype=np.float64)
    n = np.arange(c // 2, dtype=np.float64) + 0.5

    def forward(origin):
        ang = w[:, None] * (b[None, :] - origin)
        return np.concatenate([np.cos(ang), -np.sin(ang)], axis=0)

    inverse = np.concatenate([np.cos(n[:, None] * w[None, :]),
                              np.sin(n[:, None] * w[None, :])], axis=0) / c
    return np.concatenate([forward(0.0), forward((c - 1) / 2), inverse]).astype(_BF)


_DFT_NP = _dft_tables(_T)


def _dot(a, b):
    return jnp.dot(a, b, preferred_element_type=_F32)


def _dot_nt(a, b):
    return lax.dot_general(a, b, _NT, preferred_element_type=_F32)


def _unpack_head(w32, odd):
    bits = (w32 & jnp.uint32(0xFFFF0000)) if odd else (w32 << 16)
    return pltpu.bitcast(bits, _F32).astype(_BF)


def _stage(ref, first, w):
    for n in range(w.shape[0] // _T):
        ref[first + n] = pltpu.bitcast(w[n * _T:(n + 1) * _T], jnp.uint32)


def _staged(ref, first, count):
    tiles = [pltpu.bitcast(ref[first + n], _BF) for n in range(count)]
    return tiles[0] if count == 1 else jnp.concatenate(tiles, axis=0)


def _merge(a, b):
    out, ia, ib = [], 0, 0
    while ia < len(a) or ib < len(b):
        if ib >= len(b) or (ia < len(a) and ia * len(b) <= ib * len(a)):
            out.append(a[ia])
            ia += 1
        else:
            out.append(b[ib])
            ib += 1
    return out


def _kernel(x_hbm, k_hbm, v_hbm, shift_hbm, ssmk_hbm, ssmd_hbm, c_hbm, wq_hbm, wuk_hbm,
            wuv_hbm, wo_hbm, gate_hbm, dft_hbm, out_hbm,
            x_v, c_v, wq_v, wuk_v, wuv_v, wo_v, ak_v, av_v, sk_v, ctx_v,
            w0, w1, wo_b, q0, k0, v0, q1, k1, v1, g_v, spec_v, o_v,
            shift_v, ssmd_v, gate_v, dft_v, ssmd_f, zero_s,
            sem, sem_c, sem_x, *, S, M, H, D):
    NP = H // 2
    NQ = S // _BQ
    TPB = _BQ // _T
    qscale = float(D ** -0.5 * _LOG2E)

    def w_copies(p, sems):
        return [pltpu.make_async_copy(src.bitcast(jnp.uint32).at[:, p, :], dst.at[p], sem.at[n])
                for n, (src, dst) in zip(sems, ((wuk_hbm, wuk_v), (wuv_hbm, wuv_v),
                                                (wq_hbm, wq_v)))]

    cp_gate = pltpu.make_async_copy(gate_hbm, gate_v, sem.at[1])
    cp_w1 = w_copies(1, (2, 2, 2))
    cp_w = [cp for n in range(2, NP) for cp in w_copies(n, (3, 6, 7))]
    cp_late = [pltpu.make_async_copy(src, dst, sem.at[4]) for src, dst in (
        (wo_hbm, wo_v.at[:, :, pl.ds(0, M)]), (k_hbm, ak_v), (v_hbm, av_v), (ssmk_hbm, sk_v),
        (shift_hbm, shift_v), (ssmd_hbm, ssmd_v), (dft_hbm, dft_v))]

    def aligned(n, size):
        return pl.ds(n * size if isinstance(n, int) else pl.multiple_of(n * size, size), size)

    def c_copy(n):
        rows = aligned(n, 2 * _BQ)
        return pltpu.make_async_copy(c_hbm.at[rows], c_v.at[rows], sem_c.at[n])

    def x_copy(n):
        rows = aligned(n, _BQ)
        return pltpu.make_async_copy(x_hbm.at[rows], x_v.at[rows], sem_x.at[n])

    def out_copy(cb, part):
        rows = pl.ds(0, S - _BQ) if part == 0 else pl.ds(S - _BQ, _BQ)
        return pltpu.make_async_copy(o_v.at[cb, rows], out_hbm.at[rows, aligned(cb, _T)],
                                     sem.at[5])

    tri = (lax.broadcasted_iota(jnp.int32, (_T, _T), 1)
           <= lax.broadcasted_iota(jnp.int32, (_T, _T), 0))
    bufs = ((q0, k0, v0, w0), (q1, k1, v1, w1))
    NM, NK = M // _T, c_v.shape[1] // _T

    def prep_kv(p, odd):
        _stage(bufs[odd][3], NM, _unpack_head(wuk_v[p], odd))
        _stage(bufs[odd][3], NM + NK, _unpack_head(wuv_v[p], odd))

    def prep_q(p, odd):
        _stage(bufs[odd][3], 0, _unpack_head(wq_v[p], odd))

    def proj_q(r, odd):
        rows = aligned(r, _BQ)
        q = _dot(x_v[rows, :], _staged(bufs[odd][3], 0, NM)) * qscale
        bufs[odd][0][rows, :] = q.astype(_BF)

    def proj_k(r, odd):
        rows = aligned(r, _BQ)
        bufs[odd][1][rows, :] = _dot(c_v[rows, :], _staged(bufs[odd][3], NM, NK)).astype(_BF)

    def proj_v(r, odd):
        rows = aligned(r, _BQ)
        bufs[odd][2][rows, :] = _dot(c_v[rows, :],
                                     _staged(bufs[odd][3], NM + NK, NK)).astype(_BF)

    def first_row(i, j):
        return max(0, j - TPB * i) * _T

    def accum(old, new, lo, op):
        if old is None:
            return new
        if lo == 0:
            return op(old, new)
        return jnp.concatenate([old[:lo], op(old[lo:], new)], axis=0)

    def head(h, odd, project_next):
        q_b, k_b, v_b, _ = bufs[odd]
        st = {}

        def qk(i, js):
            s = st.setdefault(i, dict(t={}, m=None, l=None, acc=None))
            q = q_b[pl.ds(i * _BQ, _BQ), :]
            for j in js:
                lo = first_row(i, j)
                t = _dot_nt(q[lo:], k_b[pl.ds(j * _T, _T), :])
                if j >= TPB * i:
                    top = jnp.where(tri, t[0:_T], _NEG)
                    t = top if t.shape[0] == _T else jnp.concatenate([top, t[_T:]], axis=0)
                s["t"][j] = t
                s["m"] = accum(s["m"], t, lo, jnp.maximum)
            if js[-1] == TPB * (i + 1) - 1:
                s["m"] = jnp.broadcast_to(jnp.max(s["m"], axis=1, keepdims=True), (_BQ, _T))

        def pv(i, js):
            s = st[i]
            for j in js:
                lo = first_row(i, j)
                p = jnp.exp2(s["t"][j] - s["m"][lo:]).astype(_BF)
                p32 = p.astype(_F32)
                o = _dot(p, v_b[pl.ds(j * _T, _T), :])
                s["l"] = accum(s["l"], p32, lo, jnp.add)
                s["acc"] = accum(s["acc"], o, lo, jnp.add)
            if js[-1] == TPB * (i + 1) - 1:
                l = jnp.broadcast_to(jnp.sum(s["l"], axis=1, keepdims=True), (_BQ, _T))
                r = pltpu.reciprocal(l, approx=True)
                r = r * (2.0 - l * r)
                ctx_v[h, pl.ds(i * _BQ, _BQ), :] = (s["acc"] * r).astype(_BF)

        def groups(fn, i, size):
            n = TPB * (i + 1)
            return [(fn, i, list(range(a, min(a + size, n)))) for a in range(0, n, size)]

        order = list(range(NQ - 1, 1, -1)) + [0, 1]
        att = groups(qk, order[0], 2)
        for n, i in enumerate(order):
            att += _merge(groups(qk, order[n + 1], 2) if n + 1 < NQ else [], groups(pv, i, 2))
        cost = [sum(_BQ - first_row(i, j) for j in js) * (2.0 if fn is qk else 1.0)
                for fn, i, js in att]

        def last_use(fn, blocks):
            return max(n for n, (f, i, _) in enumerate(att) if f is fn and i in blocks)

        side = []
        for r in order if project_next else []:
            side += [(last_use(qk, [r]), proj_q, r, 8), (last_use(qk, range(r, NQ)), proj_k, r, 4),
                     (last_use(pv, range(r, NQ)), proj_v, r, 4)]
        side.sort(key=lambda t: t[0])
        budget = sum(t[3] for t in side[:len(side) - _TAIL])
        tasks = []
        done = spent = 0
        for n, (task, c) in enumerate(zip(att, cost)):
            tasks.append(task)
            done += c
            while (len(side) > _TAIL and side[0][0] <= n
                   and spent + 0.5 * side[0][3] <= budget * (done / sum(cost)) ** 0.8):
                _, f, r, c2 = side.pop(0)
                tasks.append((f, r, odd))
                spent += c2
        return tasks + [(f, r, odd) for _, f, r, _ in side]

    def run(tasks):
        for fn, a, b in tasks:
            fn(a, b)

    def prologue():
        cp_uk, cp_uv, cp_q = w_copies(0, (0, 0, 1))

        def clear(i, carry):
            zero_s[i] = 0
            return carry

        def kv_body(n, carry):
            c_copy(n).wait()
            x_copy(2 * n).start()
            x_copy(2 * n + 1).start()
            for r in (2 * n, 2 * n + 1):
                for odd in range(2):
                    proj_k(r, odd)
                    proj_v(r, odd)
            return carry

        for cp in (cp_uk, cp_uv, c_copy(0)):
            cp.start()
        lax.fori_loop(0, zero_s.shape[0], clear, 0)
        cp_uk.wait()
        cp_uv.wait()
        for cp in [c_copy(n) for n in range(1, NQ // 2)] + [cp_q, cp_gate]:
            cp.start()
        prep_kv(0, 0)
        prep_kv(0, 1)
        lax.fori_loop(0, NQ // 2, kv_body, 0)
        cp_q.wait()
        cp_gate.wait()
        prep_q(0, 0)
        prep_q(0, 1)
        gw = gate_v[...].astype(_F32)
        waits = list(range(0, NQ + 1, 2))
        for lo, hi in zip(waits[:-1], waits[1:]):
            for r in range(lo, hi):
                x_copy(r).wait()
            if lo == NQ // 4 * 2:
                for cp in cp_w1:
                    cp.start()
            for r in range(lo, hi):
                proj_q(r, 0)
                proj_q(r, 1)
                rows = pl.ds(r * _BQ, _BQ)
                z = None
                for n in range(M // _T):
                    t = x_v[rows, pl.ds(n * _T, _T)].astype(_F32) * gw[n:n + 1, :]
                    z = t if z is None else z + t
                g = lax.logistic(jnp.sum(z, axis=1, keepdims=True))
                g_v[rows, :] = jnp.broadcast_to(g, (_BQ, _T))
        for cp in cp_w1:
            cp.wait()
        for cp in cp_w:
            cp.start()

    def pair_body(p, carry):
        @pl.when(p == 1)
        def _():
            for w, n in ((wuk_v, 3), (wuv_v, 6), (wq_v, 7)):
                rest = w.at[pl.ds(2, NP - 2)]
                pltpu.make_async_copy(rest, rest, sem.at[n]).wait()
            for cp in cp_late:
                cp.start()

        for odd in range(2):
            prep_kv(p + 1, odd)
            prep_q(p + 1, odd)
        run(head(2 * p, 0, True) + head(2 * p + 1, 1, True))
        return carry

    prologue()
    lax.fori_loop(0, NP - 1, pair_body, 0)
    t0, t1 = head(H - 2, 0, False), head(H - 1, 1, False)
    run(t0[:8] + _merge(t0[8:], t1[:-8]) + t1[-8:])

    for cp in cp_late:
        cp.wait()
    ssmd_f[...] = ssmd_v[...].astype(_F32)
    NC = S // _T
    NB = M // _T
    HF = _T // 2

    def col_body(cb, carry):
        cols = aligned(cb, _T)
        sh = shift_v[:, cols].astype(_F32)
        dvec = ssmd_f[pl.ds(cb, 1), :]
        flip = 7 - lax.broadcasted_iota(jnp.int32, (8, _T), 0)
        bacc, kvs, yt, state = {}, {}, {}, {"n": 0, "tail": jnp.zeros((8, _T), _F32)}

        def new_step():
            state["z"] = pl.multiple_of(zero_s[state["n"]] * 8, 8)
            state["n"] += 1

        def spec_rows(kind, c, part, lo=0, n=_T):
            return pl.ds(state["z"] + ((kind * NC + c) * 2 + part) * _SPEC_STRIDE + lo, n)

        def spec_load(kind, c, fg):
            return tuple(spec_v[spec_rows(kind, c, part, fg * 8, 8), :] for part in range(2))

        def spec_store(kind, c, val):
            for part in range(2):
                spec_v[spec_rows(kind, c, part), :] = val[part * _T:(part + 1) * _T]

        def out_proj(i, g):
            rows = pl.ds(i * _BQ, _BQ)
            for h in range(4 * g, 4 * g + 4):
                t = _dot(ctx_v[h, rows, :], _staged(wo_b, h, 1))
                bacc[i] = t if h == 0 else bacc[i] + t

        def dft_u(j):
            cur = ak_v[pl.ds(j * _T, _T), cols].astype(_F32)
            ext = jnp.concatenate([state["tail"], cur], axis=0)
            state["tail"] = cur[_T - 8:]
            acc = cur * sh[0:1, :]
            for s in range(1, sh.shape[0]):
                acc = acc + ext[8 - s:8 - s + _T] * sh[s:s + 1, :]
            kv = (acc * av_v[pl.ds(j * _T, _T), cols].astype(_F32)).astype(_BF)
            kvs[j] = kv
            spec_store(0, j, _dot(dft_v[0:2 * _T, :], kv))

        def dft_k(j):
            s = _dot_nt(dft_v[2 * _T:4 * _T, :], sk_v[cols, pl.ds(j * _T, _T)])
            if j == 0:
                spec_store(1, j, s)
            else:
                p = state["prev"]
                spec_store(1, j, jnp.concatenate(
                    [s[0:HF] - p[_T:_T + HF], s[HF:_T] + p[_T + HF:],
                     s[_T:_T + HF] + p[0:HF], s[_T + HF:] - p[HF:_T]], axis=0))
            state["prev"] = s

        def mac(arg):
            fg, a = arg
            new_step()
            kc, y = {}, {}
            for j in range(4 * a + 4):
                ur, ui = spec_load(0, j, fg)
                for i in range(max(4 * a, j), 4 * a + 4):
                    if i - j not in kc:
                        kc[i - j] = spec_load(1, i - j, fg)
                    kr, ki = kc[i - j]
                    tr, ti = kr * ur - ki * ui, kr * ui + ki * ur
                    y[i] = (tr, ti) if i not in y else (y[i][0] + tr, y[i][1] + ti)
            for i, parts in y.items():
                for part in range(2):
                    spec_v[spec_rows(2, i, part, fg * 8, 8), :] = parts[part]

        def idft(c):
            new_step()
            even, odd = [_dot(dft_v[4 * _T + part * HF:4 * _T + (part + 1) * HF, :],
                              spec_v[spec_rows(2, c, part), :].astype(_BF))
                         for part in range(2)]
            mirrored = even + odd
            yt[c] = jnp.concatenate(
                [jnp.take_along_axis(mirrored[lo:lo + 8], flip, axis=0)
                 for lo in range(HF - 8, -8, -8)] + [even - odd], axis=0)

        def combine(c):
            rows = pl.ds(c * _T, _T)
            off = (c % TPB) * _T
            y = yt[c] + kvs[c].astype(_F32) * dvec
            a = x_v[rows, cols].astype(_F32) * y
            g = g_v[rows, :]
            o_v[cb, rows, :] = (g * a + (1.0 - g) * bacc[c // TPB][off:off + _T]).astype(_BF)
            if c + 1 in (NC - TPB, NC):
                out_copy(cb, int(c + 1 == NC)).start()

        for h in range(H):
            _stage(wo_b, h, wo_v[h, :, cols])
        main = [(i, g) for i in range(NQ) for g in range(H // 4)]
        f0, f1, f2, f3 = 0.02, 0.2, 0.75, 0.86
        stage1 = [(dft_k, j) for j in range(NC)] + [(dft_u, j) for j in range(NC)]
        stage2 = [(fg, a) for fg in range(_T // 8) for a in range(NC // 4)]
        side = [(f0 + (f1 - f0) * n / len(stage1), f, a) for n, (f, a) in enumerate(stage1)]
        side += [(f1 + (f2 - f1) * n / len(stage2), mac, a) for n, a in enumerate(stage2)]
        side += [(f2 + (f3 - f2) * c / NC, idft, c) for c in range(NC)]
        side += [(max(f2 + (f3 - f2) * (c + 0.5) / NC, (c // TPB + 1) / NQ), combine, c)
                 for c in range(NC)]
        side.sort(key=lambda t: t[0])
        new_step()
        k = 0
        for n, (i, g) in enumerate(main):
            while k < len(side) and side[k][0] <= n / len(main) + 1e-9:
                side[k][1](side[k][2])
                k += 1
            out_proj(i, g)
        for _, f, a in side[k:]:
            f(a)
        return carry

    lax.fori_loop(0, NB, col_body, 0)
    for cb in range(NB):
        out_copy(cb, 0).wait()
        out_copy(cb, 1).wait()


@jax.jit
def pallas_gated_mix__ssm_conv_h3__compressed_kv_cla__prompt_kernel(
    A_q: jax.Array,
    A_k: jax.Array,
    A_v: jax.Array,
    A_shift_k: jax.Array,
    A_ssm_k: jax.Array,
    A_ssm_D: jax.Array,
    B_x: jax.Array,
    B_c_kv: jax.Array,
    B_w_q: jax.Array,
    B_w_uk: jax.Array,
    B_w_uv: jax.Array,
    B_w_o: jax.Array,
    gate_w: jax.Array,
):
    del B_x
    B, S, M = A_q.shape
    _, H, D = B_w_q.shape
    DC = B_c_kv.shape[-1]
    assert B == 1 and D == _T and H >= 8 and H % 4 == 0 and A_shift_k.shape[1] <= 9
    assert S >= 4 * _BQ and S % (2 * _BQ) == 0 and B_c_kv.shape[1] == S
    NP, NC = H // 2, S // _T

    def body(*refs):
        _kernel(*refs, S=S, M=M, H=H, D=D)

    hbm = pl.BlockSpec(memory_space=pl.ANY)
    scratch = [
        pltpu.VMEM((S, M), _BF),
        pltpu.VMEM((S, DC), _BF),
        pltpu.VMEM((NP, M, D), jnp.uint32),
        pltpu.VMEM((NP, DC, D), jnp.uint32),
        pltpu.VMEM((NP, DC, D), jnp.uint32),
        pltpu.VMEM((H, D, M + _T), _BF),
        pltpu.VMEM((S, M), _BF),
        pltpu.VMEM((S, M), _BF),
        pltpu.VMEM((M, S), _BF),
        pltpu.VMEM((H, S, D), _BF),
        pltpu.VMEM(((M + 2 * DC) // _T, _T // 2, D), jnp.uint32),
        pltpu.VMEM(((M + 2 * DC) // _T, _T // 2, D), jnp.uint32),
        pltpu.VMEM((H, D // 2, _T), jnp.uint32),
    ] + [pltpu.VMEM((S, D), _BF)] * 6 + [
        pltpu.VMEM((S, _T), _F32),
        pltpu.VMEM((3 * 2 * NC * _SPEC_STRIDE, _T), _F32),
        pltpu.VMEM((M // _T, S, _T), _BF),
        pltpu.VMEM((A_shift_k.shape[1], M), _BF),
        pltpu.VMEM((M // _T, _T), _BF),
        pltpu.VMEM((M // _T, _T), _BF),
        pltpu.VMEM(_DFT_NP.shape, _BF),
        pltpu.VMEM((M // _T, _T), _F32),
        pltpu.SMEM((1 + (_T // 8) * (NC // 4) + NC,), jnp.int32),
        pltpu.SemaphoreType.DMA((8,)),
        pltpu.SemaphoreType.DMA((S // (2 * _BQ),)),
        pltpu.SemaphoreType.DMA((S // _BQ,)),
    ]
    out = pl.pallas_call(
        body,
        out_shape=jax.ShapeDtypeStruct((S, M), _BF),
        in_specs=[hbm] * 13,
        out_specs=hbm,
        scratch_shapes=scratch,
        compiler_params=pltpu.CompilerParams(vmem_limit_bytes=112 * 2 ** 20),
    )(
        A_q.reshape(S, M), A_k.reshape(S, M), A_v.reshape(S, M), A_shift_k.T, A_ssm_k,
        A_ssm_D.reshape(M // _T, _T), B_c_kv.reshape(S, DC), B_w_q, B_w_uk, B_w_uv, B_w_o,
        gate_w.reshape(M // _T, _T), _DFT_NP,
    )
    return out.reshape(B, S, M)
```
